```python
import jax
import jax.numpy as jnp

def _softmax(x, axis=-1):
    return jax.nn.softmax(x, axis=axis)
def _gelu(x):
    return jax.nn.gelu(x, approximate=True)
def _silu(x):
    return jax.nn.silu(x)
def _sigmoid(x):
    return jax.nn.sigmoid(x)
def _layernorm(x, axis=-1, eps=1e-5):
    m = jnp.mean(x, axis=axis, keepdims=True)
    v = jnp.var(x, axis=axis, keepdims=True)
    return (x - m) / jnp.sqrt(v + eps)
def _scatter_add(tgt, idx, src, axis=0):
    return tgt.at[idx].add(src)
def _segment_sum(src, seg, n):
    return jax.ops.segment_sum(src, seg, n)
class _Rng:
    def __init__(self, key):
        self._k = key
    def _next(self):
        self._k, sub = jax.random.split(self._k)
        return sub
    def normal(self, shape):
        return jax.random.normal(self._next(), shape, dtype=jnp.bfloat16)
    def randint(self, lo, hi, shape):
        return jax.random.randint(self._next(), shape, lo, hi, dtype=jnp.int32)
    def uniform(self, shape, lo=0.0, hi=1.0):
        return jax.random.uniform(self._next(), shape, jnp.bfloat16, lo, hi)
    def permutation(self, n):
        return jax.random.permutation(self._next(), n)


kernel_name = 'concat_heads__gqa_block_cached__mha_block_cached__near_ridge'

def setup_inputs():
    _rng = _Rng(jax.random.key(int.from_bytes(__import__("os").urandom(4), "little")))
    _w = (lambda a: (lambda t: t.astype(jnp.bfloat16) if jnp.issubdtype(t.dtype, jnp.floating) else t)(jnp.asarray(a)))
    def _A_setup():
        B, Sq, D = 16, 160, 640
        Hq, Hkv, Sk, Dh = 32, 32, 512, 192
        assert Hq % Hkv == 0, (Hq, Hkv)
        return {
            "x": _w((lambda *s: _rng.normal(s) * 0.05)(B, Sq, D)),
            "k_cache": _w((lambda *s: _rng.normal(s) * 0.05)(B, Hkv, Sk, Dh)),
            "v_cache": _w((lambda *s: _rng.normal(s) * 0.05)(B, Hkv, Sk, Dh)),
            "wq": _w((lambda *s: _rng.normal(s) * 0.05)(D, Hq * Dh) * (D ** -0.5)),
            "wo": _w((lambda *s: _rng.normal(s) * 0.05)(Hq * Dh, D) * ((Hq * Dh) ** -0.5)),
        }
    _A_in = _A_setup()

    def _B_setup():
        B, Sq, D = 16, 160, 640
        H, Sk, Dh = 32, 512, 192
        return {
            "x": _w((lambda *s: _rng.normal(s) * 0.05)(B, Sq, D)),
            "k_cache": _w((lambda *s: _rng.normal(s) * 0.05)(B, H, Sk, Dh)),
            "v_cache": _w((lambda *s: _rng.normal(s) * 0.05)(B, H, Sk, Dh)),
            "wq": _w((lambda *s: _rng.normal(s) * 0.05)(D, H * Dh) * (D ** -0.5)),
            "wo": _w((lambda *s: _rng.normal(s) * 0.05)(H * Dh, D) * ((H * Dh) ** -0.5)),
        }
    _B_in = _B_setup()

    return {
        "A_x": _A_in["x"],
        "A_k_cache": _A_in["k_cache"],
        "A_v_cache": _A_in["v_cache"],
        "A_wq": _A_in["wq"],
        "A_wo": _A_in["wo"],
        "B_x": _B_in["x"],
        "B_k_cache": _B_in["k_cache"],
        "B_v_cache": _B_in["v_cache"],
        "B_wq": _B_in["wq"],
        "B_wo": _B_in["wo"],
    }

def reference(A_x, A_k_cache, A_v_cache, A_wq, A_wo, B_x, B_k_cache, B_v_cache, B_wq, B_wo):
    def _A_ref(x, k_cache, v_cache, wq, wo):
        B, Sq, D = x.shape
        Hq, Dh = 32, 192
        Hkv = k_cache.shape[1]
        rep = Hq // Hkv
        q = (lambda x, *d: x.transpose(*d))((x @ wq).reshape(B, Sq, Hq, Dh), 0, 2, 1, 3)
        k = jnp.repeat(k_cache, rep, axis=1)
        v = jnp.repeat(v_cache, rep, axis=1)
        scores = jnp.einsum("bhqd,bhkd->bhqk", q, k) * (Dh ** -0.5)
        p = _softmax(scores, axis=-1)
        o = jnp.einsum("bhqk,bhkd->bhqd", p, v)
        return (lambda x, *d: x.transpose(*d))(o, 0, 2, 1, 3).reshape(B, Sq, Hq * Dh) @ wo

    def _B_ref(x, k_cache, v_cache, wq, wo):
        B, Sq, D = x.shape
        H, Dh = 32, 192
        q = (lambda x, *d: x.transpose(*d))((x @ wq).reshape(B, Sq, H, Dh), 0, 2, 1, 3)
        scores = jnp.einsum("bhqd,bhkd->bhqk", q, k_cache) * (Dh ** -0.5)
        p = _softmax(scores, axis=-1)
        o = jnp.einsum("bhqk,bhkd->bhqd", p, v_cache)
        return (lambda x, *d: x.transpose(*d))(o, 0, 2, 1, 3).reshape(B, Sq, H * Dh) @ wo

    a = _A_ref(A_x, A_k_cache, A_v_cache, A_wq, A_wo)
    b = _B_ref(B_x, B_k_cache, B_v_cache, B_wq, B_wo)
    return jnp.concatenate([a, b], axis=-1)
```

```python
import functools
import math

import jax
import jax.numpy as jnp
import jax.experimental.pallas as pl
import jax.experimental.pallas.tpu as pltpu

_H = 32
_DH = 192
_PAIR = 2 * _DH

_NT = (((1,), (1,)), ((), ()))


def _attn_pair(q, kt, vt):
    sq = q.shape[0]
    lane = jax.lax.broadcasted_iota(jnp.int32, (sq, 128), 1)
    lo = lane < 64
    t0, t1, t2 = q[:, 0:128], q[:, 128:256], q[:, 256:384]
    zero = jnp.zeros_like(t1)
    q1 = jnp.concatenate([t0, jnp.where(lo, t1, zero)], axis=1)
    q2 = jnp.concatenate([jnp.where(lo, zero, t1), t2], axis=1)
    s1 = jnp.dot(q1, kt[0:256], preferred_element_type=jnp.float32)
    s2 = jnp.dot(q2, kt[128:384], preferred_element_type=jnp.float32)

    def soft(s):
        m = jnp.max(s, axis=-1, keepdims=True)
        p = jnp.exp2(s - m)
        l = jnp.sum(p, axis=-1, keepdims=True)
        return p.astype(jnp.bfloat16), 1.0 / l

    p1, r1 = soft(s1)
    p2, r2 = soft(s2)
    o1 = jax.lax.dot_general(p1, vt[0:256], _NT, preferred_element_type=jnp.float32) * r1
    o2 = jax.lax.dot_general(p2, vt[128:384], _NT, preferred_element_type=jnp.float32) * r2
    o = jnp.concatenate(
        [o1[:, 0:128], jnp.where(lo, o1[:, 128:256], o2[:, 0:128]), o2[:, 128:256]],
        axis=1)
    return o.astype(jnp.bfloat16)


def _kernel(xa_ref, ka_ref, va_ref, wqa_ref, woa_ref,
            xb_ref, kb_ref, vb_ref, wqb_ref, wob_ref,
            o_ref, acc_ref, *, bg, hg, n_hg):
    ih = pl.program_id(0)
    ib = pl.program_id(1)
    sq, d = xa_ref.shape[1], xa_ref.shape[2]
    scale = (_DH ** -0.5) * math.log2(math.e)

    @pl.when(ih == 0)
    def _():
        acc_ref[ib] = jnp.zeros(acc_ref.shape[1:], jnp.float32)

    for br, (x_ref, k_ref, v_ref, wq_ref, wo_ref) in enumerate(
            ((xa_ref, ka_ref, va_ref, wqa_ref, woa_ref),
             (xb_ref, kb_ref, vb_ref, wqb_ref, wob_ref))):
        x = x_ref[...].reshape(bg * sq, d)
        q = jnp.dot(x, wq_ref[...], preferred_element_type=jnp.float32) * scale
        q = q.astype(jnp.bfloat16)
        rows = []
        for b in range(bg):
            cols = []
            for p in range(hg // 2):
                sl = slice(p * _PAIR, (p + 1) * _PAIR)
                cols.append(_attn_pair(q[b * sq:(b + 1) * sq, sl],
                                       k_ref[b, sl, :], v_ref[b, sl, :]))
            rows.append(jnp.concatenate(cols, axis=1) if len(cols) > 1 else cols[0])
        o = jnp.concatenate(rows, axis=0) if len(rows) > 1 else rows[0]
        acc_ref[ib, :, br * d:(br + 1) * d] += jnp.dot(
            o, wo_ref[...], preferred_element_type=jnp.float32)

    @pl.when(ih == n_hg - 1)
    def _():
        o_ref[...] = acc_ref[ib].reshape(o_ref.shape).astype(o_ref.dtype)


def _build(A_x, A_k_cache, A_v_cache, A_wq, A_wo,
           B_x, B_k_cache, B_v_cache, B_wq, B_wo, *, bg=1, hg=2):
    nb, sq, d = A_x.shape
    sk = A_k_cache.shape[2]

    def tr(c):
        return jnp.swapaxes(c, 2, 3).reshape(nb, _H * _DH, sk)

    n_hg = _H // hg
    n_bg = nb // bg
    x_spec = pl.BlockSpec((bg, sq, d), lambda h, b: (b, 0, 0))
    kv_spec = pl.BlockSpec((bg, hg * _DH, sk), lambda h, b: (b, h, 0))
    wq_spec = pl.BlockSpec((d, hg * _DH), lambda h, b: (0, h))
    wo_spec = pl.BlockSpec((hg * _DH, d), lambda h, b: (h, 0))
    out_spec = pl.BlockSpec(
        (bg, sq, 2 * d), lambda h, b: (jnp.where(h == n_hg - 1, b, 0), 0, 0))
    specs = [x_spec, kv_spec, kv_spec, wq_spec, wo_spec]
    return pl.pallas_call(
        functools.partial(_kernel, bg=bg, hg=hg, n_hg=n_hg),
        grid=(n_hg, n_bg),
        in_specs=specs + specs,
        out_specs=out_spec,
        out_shape=jax.ShapeDtypeStruct((nb, sq, 2 * d), A_x.dtype),
        scratch_shapes=[pltpu.VMEM((n_bg, bg * sq, 2 * d), jnp.float32)],
        compiler_params=pltpu.CompilerParams(
            dimension_semantics=("arbitrary", "arbitrary"),
            vmem_limit_bytes=100 * 1024 * 1024),
    )(A_x, tr(A_k_cache), tr(A_v_cache), A_wq, A_wo,
      B_x, tr(B_k_cache), tr(B_v_cache), B_wq, B_wo)


@jax.jit
def pallas_concat_heads__gqa_block_cached__mha_block_cached__near_ridge_kernel(
    A_x: jax.Array,
    A_k_cache: jax.Array,
    A_v_cache: jax.Array,
    A_wq: jax.Array,
    A_wo: jax.Array,
    B_x: jax.Array,
    B_k_cache: jax.Array,
    B_v_cache: jax.Array,
    B_wq: jax.Array,
    B_wo: jax.Array,
):
    return _build(A_x, A_k_cache, A_v_cache, A_wq, A_wo,
                  B_x, B_k_cache, B_v_cache, B_wq, B_wo)
```

```python
import functools
import math

import jax
import jax.numpy as jnp
import jax.experimental.pallas as pl
import jax.experimental.pallas.tpu as pltpu

_H = 32
_DH = 192
_PAIR = 2 * _DH

_NT = (((1,), (1,)), ((), ()))


def _attn_pair(q, kt, vt):
    sq = q.shape[0]
    lane = jax.lax.broadcasted_iota(jnp.int32, (sq, 128), 1)
    lo = lane < 64
    t0, t1, t2 = q[:, 0:128], q[:, 128:256], q[:, 256:384]
    zero = jnp.zeros_like(t1)
    q1 = jnp.concatenate([t0, jnp.where(lo, t1, zero)], axis=1).astype(jnp.bfloat16)
    q2 = jnp.concatenate([jnp.where(lo, zero, t1), t2], axis=1).astype(jnp.bfloat16)
    s1 = jnp.dot(q1, kt[0:256], preferred_element_type=jnp.float32)
    s2 = jnp.dot(q2, kt[128:384], preferred_element_type=jnp.float32)

    def soft(s):
        m = jnp.max(s, axis=-1, keepdims=True)
        p = jnp.exp2(s - m)
        l = jnp.sum(p, axis=-1, keepdims=True)
        r = pl.reciprocal(l, approx=True)
        r = r * (2.0 - l * r)
        return p.astype(jnp.bfloat16), r

    p1, r1 = soft(s1)
    p2, r2 = soft(s2)
    o1 = jax.lax.dot_general(p1, vt[0:256], _NT, preferred_element_type=jnp.float32) * r1
    o2 = jax.lax.dot_general(p2, vt[128:384], _NT, preferred_element_type=jnp.float32) * r2
    o = jnp.concatenate(
        [o1[:, 0:128], jnp.where(lo, o1[:, 128:256], o2[:, 0:128]), o2[:, 128:256]],
        axis=1)
    return o.astype(jnp.bfloat16)


def _kernel(xa_ref, ka_ref, va_ref, wqa_ref, woa_ref,
            xb_ref, kb_ref, vb_ref, wqb_ref, wob_ref,
            o_ref, acc_ref, *, bg, hg, n_hg):
    ih = pl.program_id(0)
    ib = pl.program_id(1)
    sq, d = xa_ref.shape[1], xa_ref.shape[2]
    scale = (_DH ** -0.5) * math.log2(math.e)

    @pl.when(ih == 0)
    def _():
        acc_ref[ib] = jnp.zeros(acc_ref.shape[1:], jnp.float32)

    for br, (x_ref, k_ref, v_ref, wq_ref, wo_ref) in enumerate(
            ((xa_ref, ka_ref, va_ref, wqa_ref, woa_ref),
             (xb_ref, kb_ref, vb_ref, wqb_ref, wob_ref))):
        x = x_ref[...].reshape(bg * sq, d)
        q = jnp.dot(x, wq_ref[...], preferred_element_type=jnp.float32) * scale
        rows = []
        for b in range(bg):
            cols = []
            for p in range(hg // 2):
                sl = slice(p * _PAIR, (p + 1) * _PAIR)
                cols.append(_attn_pair(q[b * sq:(b + 1) * sq, sl],
                                       k_ref[b, sl, :], v_ref[b, sl, :]))
            rows.append(jnp.concatenate(cols, axis=1) if len(cols) > 1 else cols[0])
        o = jnp.concatenate(rows, axis=0) if len(rows) > 1 else rows[0]
        acc_ref[ib, :, br * d:(br + 1) * d] += jnp.dot(
            o, wo_ref[...], preferred_element_type=jnp.float32)

    @pl.when(ih == n_hg - 1)
    def _():
        o_ref[...] = acc_ref[ib].reshape(o_ref.shape).astype(o_ref.dtype)


def _build(A_x, A_k_cache, A_v_cache, A_wq, A_wo,
           B_x, B_k_cache, B_v_cache, B_wq, B_wo, *, bg=1, hg=2):
    nb, sq, d = A_x.shape
    sk = A_k_cache.shape[2]

    def tr(c):
        return jnp.swapaxes(c, 2, 3).reshape(nb, _H * _DH, sk)

    n_hg = _H // hg
    n_bg = nb // bg
    x_spec = pl.BlockSpec((bg, sq, d), lambda h, b: (b, 0, 0))
    kv_spec = pl.BlockSpec((bg, hg * _DH, sk), lambda h, b: (b, h, 0))
    wq_spec = pl.BlockSpec((d, hg * _DH), lambda h, b: (0, h))
    wo_spec = pl.BlockSpec((hg * _DH, d), lambda h, b: (h, 0))
    out_spec = pl.BlockSpec(
        (bg, sq, 2 * d), lambda h, b: (jnp.where(h == n_hg - 1, b, 0), 0, 0))
    specs = [x_spec, kv_spec, kv_spec, wq_spec, wo_spec]
    return pl.pallas_call(
        functools.partial(_kernel, bg=bg, hg=hg, n_hg=n_hg),
        grid=(n_hg, n_bg),
        in_specs=specs + specs,
        out_specs=out_spec,
        out_shape=jax.ShapeDtypeStruct((nb, sq, 2 * d), A_x.dtype),
        scratch_shapes=[pltpu.VMEM((n_bg, bg * sq, 2 * d), jnp.float32)],
        compiler_params=pltpu.CompilerParams(
            dimension_semantics=("arbitrary", "arbitrary"),
            vmem_limit_bytes=100 * 1024 * 1024),
    )(A_x, tr(A_k_cache), tr(A_v_cache), A_wq, A_wo,
      B_x, tr(B_k_cache), tr(B_v_cache), B_wq, B_wo)


@jax.jit
def pallas_concat_heads__gqa_block_cached__mha_block_cached__near_ridge_kernel(
    A_x: jax.Array,
    A_k_cache: jax.Array,
    A_v_cache: jax.Array,
    A_wq: jax.Array,
    A_wo: jax.Array,
    B_x: jax.Array,
    B_k_cache: jax.Array,
    B_v_cache: jax.Array,
    B_wq: jax.Array,
    B_wo: jax.Array,
):
    return _build(A_x, A_k_cache, A_v_cache, A_wq, A_wo,
                  B_x, B_k_cache, B_v_cache, B_wq, B_wo)
```

```python
import functools
import math

import jax
import jax.numpy as jnp
import jax.experimental.pallas as pl
import jax.experimental.pallas.tpu as pltpu

_H = 32
_DH = 192
_PAIR = 2 * _DH
_NP = _H // 2

_NT = (((1,), (1,)), ((), ()))
_F32 = jnp.float32
_BF16 = jnp.bfloat16
_SCALE = (_DH ** -0.5) * math.log2(math.e)


def _nt(a, b):
    return jax.lax.dot_general(a, b, _NT, preferred_element_type=_F32)


def _lo(n):
    return jax.lax.broadcasted_iota(jnp.int32, (n, 128), 1) < 64


def _qproj(x, wq):
    q = jnp.dot(x, wq, preferred_element_type=_F32) * _SCALE
    lo = _lo(q.shape[0])
    t0, t1, t2 = q[:, 0:128], q[:, 128:256], q[:, 256:384]
    zero = jnp.zeros_like(t1)
    q1 = jnp.concatenate([t0, jnp.where(lo, t1, zero)], axis=1).astype(_BF16)
    q2 = jnp.concatenate([jnp.where(lo, zero, t1), t2], axis=1).astype(_BF16)
    return q1, q2


def _qk(q1, q2, kt):
    s1 = jnp.dot(q1, kt[0:256], preferred_element_type=_F32)
    s2 = jnp.dot(q2, kt[128:384], preferred_element_type=_F32)
    return s1, s2


def _soft(s):
    m = jnp.max(s, axis=-1, keepdims=True)
    p = jnp.exp2(s - m)
    l = jnp.sum(p, axis=-1, keepdims=True)
    r = pl.reciprocal(l, approx=True)
    r = r * (2.0 - l * r)
    return p, r


def _pv(p1, r1, p2, r2, vt):
    sq = p1.shape[0]
    lo = _lo(sq)
    n = sq - 128
    p1t, p1r = p1[0:128].astype(_BF16), p1[128:sq].astype(_BF16)
    p2t, p2r = p2[0:128].astype(_BF16), p2[128:sq].astype(_BF16)
    ot1 = _nt(vt[0:192], p1t)
    ot2 = _nt(vt[192:384], p2t)
    ot = jnp.concatenate([ot1, ot2], axis=0)
    o_top = ot.T
    lo_r = _lo(n)
    ra = _nt(p1r, vt[0:128])
    p12r = jnp.concatenate([p1[128:sq], p2[128:sq]], axis=0).astype(_BF16)
    rm = _nt(p12r, vt[128:256])
    rc = _nt(p2r, vt[256:384])
    o_r = jnp.concatenate([ra, jnp.where(lo_r, rm[0:n], rm[n:2 * n]), rc], axis=1)
    o = jnp.concatenate([o_top, o_r], axis=0)
    rr = jnp.concatenate([jnp.broadcast_to(r1, (sq, 128)),
                          jnp.where(lo, r1, r2),
                          jnp.broadcast_to(r2, (sq, 128))], axis=1)
    return (o * rr).astype(_BF16)


def _order0(T, refill, q, qk, sm, pv, o):
    for k in range(T):
        refill(k)
        q(k + 1); sm(k); o(k - 1); pv(k); qk(k + 1)


_ORDERS = [_order0]


def _kernel(xa, ka, va, wqa, woa, xb, kb, vb, wqb, wob, out,
            x_res, wq_res, wo_res, acc, ostage, kv, s_scr, o_scr,
            g_sem, w_sem, p_sem, o_sem, *, nb, n_pair, ring, sched, g_init, w_pos, late, order):
    emit = _ORDERS[order]
    lg = nb.bit_length() - 1
    assert nb == 1 << lg
    n_pos = n_pair * nb
    sq, d = x_res.shape[2], x_res.shape[3]
    wqs, wos = (wqa, wqb), (woa, wob)

    def static(v):
        return isinstance(v, int)

    def bp(u):
        if static(u):
            return u & (nb - 1), u >> lg
        return u & (nb - 1), jax.lax.shift_right_logical(u, lg)

    def clamp(u, hi=n_pos - 1):
        return min(max(u, 0), hi) if static(u) else jnp.clip(u, 0, hi)

    def when(cond):
        if isinstance(cond, bool):
            return (lambda f: f()) if cond else (lambda f: None)
        return pl.when(cond)

    def pair_ds(p):
        return pl.ds(p * _PAIR if static(p) else pl.multiple_of(p * _PAIR, _PAIR), _PAIR)

    def chunk(ref, u):
        b, p = bp(u)
        return ref.at[b, pair_ds(p), :]

    n_last = sched[-1][0]
    u_last = n_pos - n_last * sched[-1][1]
    lg_last = n_last.bit_length() - 1
    n_par = ring // n_last
    merged = u_last >= nb and n_last > 1

    def sem_of(u):
        if not merged:
            return u & (ring - 1)
        if static(u):
            return u & (ring - 1) if u < u_last else ring + ((u >> lg_last) & (n_par - 1))
        big = ring + (jax.lax.shift_right_logical(u, lg_last) & (n_par - 1))
        if all_last[0]:
            return big
        return jnp.where(u < u_last, u & (ring - 1), big)

    def issue(u, h, enable=True):
        uc = clamp(u)
        slot = uc & (ring - 1)
        sem = g_sem.at[sem_of(uc)]

        def both(c):
            if isinstance(enable, bool):
                return c if enable else False
            return enable if c is True else jnp.logical_and(enable, c)

        if x_possible[0]:
            ux = clamp(u + h, nb - 1)

            @when(both(u + h < nb))
            def _():
                src, br = (xb, 1) if h == 0 else (xa, 0)
                pltpu.make_async_copy(src.at[ux], x_res.at[br, ux], sem).start()
        srcs = (chunk(va, uc), chunk(kb, uc)) if h == 0 else (chunk(vb, uc), chunk(ka, clamp(u + 1)))
        for i, s in enumerate(srcs):
            @when(both(u < n_pos))
            def _():
                pltpu.make_async_copy(s, kv.at[slot, 2 * h + i], sem).start()
        if x_possible[0] and h == 1:
            @when(both(u == nb - 1))
            def _():
                w_start(1)

    def wq_copy(p, br, sem):
        return pltpu.make_async_copy(wqs[br].at[:, pair_ds(p)], wq_res.at[p, br], sem)

    def wo_copy(p, br, sem):
        return pltpu.make_async_copy(wos[br].at[pair_ds(p), :], wo_res.at[p, br], sem)

    def w_start(p):
        sem = w_sem.at[p & 1]
        for br in range(2):
            wq_copy(p, br, sem).start()
            wo_copy(p, br, sem).start()

    def w_wait(p):
        sem = w_sem.at[p & 1]
        pltpu.make_async_copy(wq_res.at[p], wq_res.at[p], sem).wait()
        pltpu.make_async_copy(wo_res.at[p], wo_res.at[p], sem).wait()

    def out_copy(b):
        return pltpu.make_async_copy(ostage.at[b], out.at[b], o_sem.at[b])

    def oproj(o, br, b, p):
        new = acc[br, b] + jnp.dot(o, wo_res[p, br], preferred_element_type=_F32)
        acc[br, b] = new
        ostage[b, :, br * d:(br + 1) * d] = new.astype(ostage.dtype)

    def waits_for(u0, n, maybe_first):
        if merged and all_last[0]:
            slot = u0 & (ring - 1)
            blk = kv.at[pl.ds(slot if static(slot) else pl.multiple_of(slot, n), n)]
            pltpu.make_async_copy(blk, blk, g_sem.at[sem_of(u0)]).wait()
        for i in range(0 if merged and all_last[0] else n):
            u = u0 + i
            sem = g_sem.at[u & (ring - 1)]
            slot = u & (ring - 1)
            pltpu.make_async_copy(kv.at[slot], kv.at[slot], sem).wait()
            if maybe_first:
                for h in range(2):
                    @when(u + h < nb)
                    def _():
                        pltpu.make_async_copy(x_res.at[0, 0], x_res.at[0, 0], sem).wait()
        u1 = u0 + n
        b1, p1 = bp(u1)

        @when((b1 == 0 and p1 < n_pair) if static(u1)
              else jnp.logical_and(b1 == 0, p1 < n_pair))
        def _():
            w_wait(p1)

    x_possible = [True]
    all_last = [False]
    assert g_init < ring
    first = [pltpu.make_async_copy(xa.at[0], x_res.at[0, 0], p_sem.at[0]),
             wq_copy(0, 0, p_sem.at[0]),
             pltpu.make_async_copy(chunk(ka, 0), kv.at[ring - 1, 3], p_sem.at[0])]
    for c in first:
        c.start()
    second = [wq_copy(0, 1, p_sem.at[1]), wo_copy(0, 0, p_sem.at[1]), wo_copy(0, 1, p_sem.at[1])]

    def start_rest():
        second[0].start()
        second[1].start()
        for g in range(g_init):
            issue(g, 0)
            issue(g, 1)
            if g == 0:
                second[2].start()

    if not late:
        start_rest()

    def zero(b, carry):
        for br in range(2):
            acc[br, b] = jnp.zeros((sq, d), _F32)
        return carry
    jax.lax.fori_loop(0, nb, zero, 0)
    o_scr[...] = jnp.zeros(o_scr.shape, o_scr.dtype)

    for c in first:
        c.wait()
    if late:
        start_rest()
    s1, s2 = _qk(*_qproj(x_res[0, 0], wq_res[0, 0]), kv[ring - 1, 3])
    s_scr[0] = s1
    s_scr[1] = s2
    for c in second:
        c.wait()

    def run_phase(u_start, n, cnt, g0, dbl):
        T = 2 * n
        maybe_first = u_start < nb
        maybe_last = u_start + n * cnt > n_pos - nb
        x_possible[0] = g0 < nb
        all_last[0] = u_start >= u_last

        def body(j, carry):
            u0 = u_start + j * n

            def task(k):
                if k == -1:
                    br, u = 1, clamp(u0 - 1)
                elif k == T:
                    br, u = 0, clamp(u0 + n)
                else:
                    br, u = k % 2, u0 + k // 2
                return (br,) + bp(u)

            def slot(k):
                return (u0 + k // 2) & (ring - 1)

            Q, S, P, O = {}, {}, {}, {}
            S[0] = (s_scr[0], s_scr[1])
            O[-1] = o_scr[...]

            def do_q(k):
                br, b, p = task(k)
                Q[k] = _qproj(x_res[br, b], wq_res[p, br])

            def do_qk(k):
                S[k] = _qk(*Q.pop(k), kv[slot(k - 1), 1 if k % 2 == 1 else 3])

            def do_sm(k):
                s1, s2 = S.pop(k)
                P[k] = _soft(s1) + _soft(s2)

            def do_pv(k):
                O[k] = _pv(*P.pop(k), kv[slot(k), 0 if k % 2 == 0 else 2])

            def do_o(k):
                br, b, p = task(k)
                oproj(O.pop(k), br, b, p)
                if br == 1 and maybe_last:
                    last = (p == n_pair - 1) if k >= 0 else (u0 - 1 >= n_pos - nb)

                    @pl.when(last)
                    def _():
                        out_copy(b).start()

            def refill(k):
                i = j * n + k // 2
                h = k % 2
                if dbl:
                    fast = i < dbl // 2
                    g = g0 + i + jnp.minimum(i, dbl // 2)
                    if h == 0:
                        issue(g, 0)
                        issue(g, 1, fast)
                    else:
                        g = g + fast.astype(jnp.int32)
                        issue(g, 0, fast)
                        issue(g, 1)
                else:
                    issue(g0 + i, h)

            emit(T, refill, do_q, do_qk, do_sm, do_pv, do_o)
            b0, p0 = bp(u0)

            @pl.when(jnp.logical_and(b0 == (w_pos // n) * n, p0 + 2 < n_pair))
            def _():
                w_start(p0 + 2)
            s1, s2 = S.pop(T)
            s_scr[0] = s1
            s_scr[1] = s2
            o_scr[...] = O.pop(T - 1)

            @pl.when(j + 1 < cnt)
            def _():
                waits_for(u0 + n, n, maybe_first)
            return carry

        waits_for(u_start, n, maybe_first)
        jax.lax.fori_loop(0, cnt, body, 0)

    issued = {(g, h): -1 for g in range(g_init) for h in range(2)}
    u_start, g0 = 0, g_init
    plan = []
    for n, cnt, dbl in sched:
        assert dbl % 2 == 0 and nb % n == 0 and u_start % n == 0
        plan.append((u_start, n, cnt, g0, dbl))
        for t in range(2 * n * cnt):
            i, h, tg = t // 2, t % 2, 2 * u_start + t
            if i < dbl // 2:
                gs = [(g0 + 2 * i + h, 0), (g0 + 2 * i + h, 1)]
            else:
                gs = [(g0 + i + dbl // 2, h)]
            for g, hh in gs:
                assert (g, hh) not in issued
                issued[(g, hh)] = tg
                assert 2 * (g - ring) + hh < tg
            if t % (2 * n) == 0:
                for u in range(u_start + i, u_start + i + n):
                    assert issued[(u, 0)] < tg and issued[(u, 1)] < tg
        g0 += n * cnt + dbl // 2
        u_start += n * cnt
    assert u_start == n_pos
    for u_start, n, cnt, g0, dbl in plan:
        assert w_pos < nb
        run_phase(u_start, n, cnt, g0, dbl)

    oproj(o_scr[...], 1, nb - 1, n_pair - 1)
    out_copy(nb - 1).start()
    for b in range(nb):
        out_copy(b).wait()


def _build(A_x, A_k_cache, A_v_cache, A_wq, A_wo,
           B_x, B_k_cache, B_v_cache, B_wq, B_wo, *,
           sched=((1, 32, 14), (8, 28, 8)), g_init=1, w_pos=12, late=False, order=0, nobc=True, ring=16, interpret=False):
    nb, sq, d = A_x.shape
    n_head, sk = A_k_cache.shape[1], A_k_cache.shape[2]
    n_pair = n_head // 2

    def tr(c):
        return jnp.swapaxes(c, 2, 3).reshape(nb, n_head * _DH, sk)

    any_spec = pl.BlockSpec(memory_space=pl.ANY)
    return pl.pallas_call(
        functools.partial(_kernel, nb=nb, n_pair=n_pair, ring=ring, sched=sched,
                          g_init=g_init, w_pos=w_pos, late=late, order=order),
        in_specs=[any_spec] * 10,
        out_specs=any_spec,
        out_shape=jax.ShapeDtypeStruct((nb, sq, 2 * d), A_x.dtype),
        scratch_shapes=[
            pltpu.VMEM((2, nb, sq, d), _BF16),
            pltpu.VMEM((n_pair, 2, d, _PAIR), _BF16),
            pltpu.VMEM((n_pair, 2, _PAIR, d), _BF16),
            pltpu.VMEM((2, nb, sq, d), _F32),
            pltpu.VMEM((nb, sq, 2 * d), _BF16),
            pltpu.VMEM((ring, 4, _PAIR, sk), _BF16),
            pltpu.VMEM((2, sq, sk), _F32),
            pltpu.VMEM((sq, _PAIR), _BF16),
            pltpu.SemaphoreType.DMA((2 * ring,)),
            pltpu.SemaphoreType.DMA((2,)),
            pltpu.SemaphoreType.DMA((2,)),
            pltpu.SemaphoreType.DMA((nb,)),
        ],
        compiler_params=pltpu.CompilerParams(
            vmem_limit_bytes=120 * 1024 * 1024,
            disable_bounds_checks=nobc),
        interpret=interpret,
    )(A_x, tr(A_k_cache), tr(A_v_cache), A_wq, A_wo,
      B_x, tr(B_k_cache), tr(B_v_cache), B_wq, B_wo)


@jax.jit
def pallas_concat_heads__gqa_block_cached__mha_block_cached__near_ridge_kernel(
    A_x: jax.Array,
    A_k_cache: jax.Array,
    A_v_cache: jax.Array,
    A_wq: jax.Array,
    A_wo: jax.Array,
    B_x: jax.Array,
    B_k_cache: jax.Array,
    B_v_cache: jax.Array,
    B_wq: jax.Array,
    B_wo: jax.Array,
):
    return _build(A_x, A_k_cache, A_v_cache, A_wq, A_wo,
                  B_x, B_k_cache, B_v_cache, B_wq, B_wo)
```

```python
import functools
import math

import jax
import jax.numpy as jnp
import jax.experimental.pallas as pl
import jax.experimental.pallas.tpu as pltpu

_H = 32
_DH = 192
_PAIR = 2 * _DH
_NP = _H // 2

_NT = (((1,), (1,)), ((), ()))
_F32 = jnp.float32
_BF16 = jnp.bfloat16
_SCALE = (_DH ** -0.5) * math.log2(math.e)

_ALG_Q = (
    (((0, 0, 1),), ((0, 0, 1),), ((0, 0, 1),)),
    (((1, 0, 1),), ((0, 0, 1),), ((1, 0, 1),)),
    (((0, 1, 1),), ((1, 0, 1),), ((0, 0, 1),)),
    (((1, 1, 1),), ((1, 0, 1),), ((1, 0, 1),)),
    (((0, 2, 1), (1, 2, -1)), ((2, 0, 1), (2, 1, -1), (2, 2, -1)), ((0, 0, 1),)),
    (((1, 2, 1),), ((2, 0, 1), (3, 0, 1), (4, 0, 1)), ((0, 0, 1), (1, 0, 1))),
    (((0, 0, 1), (1, 0, -1)), ((0, 1, 1), (0, 2, 1)), ((0, 1, 1),)),
    (((1, 0, 1),), ((0, 1, 1), (4, 1, -1)), ((0, 1, 1), (1, 1, 1))),
    (((0, 3, -1), (1, 3, 1)), ((3, 0, -1), (3, 1, 1), (3, 2, 1)), ((1, 1, 1),)),
    (((0, 3, 1),), ((1, 1, 1), (2, 1, 1), (3, 1, 1)), ((0, 1, 1), (1, 1, 1))),
    (((0, 1, 1), (1, 1, -1)), ((1, 1, 1), (1, 2, 1)), ((0, 2, 1),)),
    (((1, 1, 1),), ((1, 2, 1), (3, 2, 1)), ((0, 2, 1), (1, 2, 1))),
    (((0, 4, -1), (1, 4, 1)), ((4, 0, -1), (4, 1, 1), (4, 2, 1)), ((1, 2, 1),)),
    (((0, 4, 1),), ((0, 2, -1), (2, 2, 1), (4, 2, 1)), ((0, 2, 1), (1, 2, 1))),
    (((0, 3, -1), (1, 2, 1)), ((2, 1, -1), (3, 0, -1)), ((0, 0, 1), (1, 1, -1))),
    (((1, 2, 1), (1, 3, -1)), ((3, 0, 1),), ((1, 0, -1), (1, 1, -1))),
    (((0, 2, 1), (0, 3, -1)), ((2, 1, 1),), ((0, 0, 1), (0, 1, 1))),
    (((0, 4, -1), (1, 2, 1)), ((2, 2, -1), (4, 0, -1)), ((0, 0, 1), (1, 2, -1))),
    (((1, 2, 1), (1, 4, -1)), ((4, 0, 1),), ((1, 0, -1), (1, 2, -1))),
    (((0, 2, 1), (0, 4, -1)), ((2, 2, 1),), ((0, 0, 1), (0, 2, 1))),
    (((0, 3, 1), (1, 1, -1)), ((1, 1, -1), (3, 2, 1)), ((0, 2, 1), (1, 1, 1))),
    (((0, 1, -1), (0, 3, 1)), ((1, 1, 1),), ((0, 1, -1), (0, 2, 1))),
    (((1, 1, -1), (1, 3, 1)), ((3, 2, 1),), ((1, 1, -1), (1, 2, 1))),
    (((0, 4, 1), (1, 0, 1)), ((0, 2, 1), (4, 1, 1)), ((0, 1, 1), (1, 2, 1))),
    (((1, 0, 1), (1, 4, 1)), ((4, 1, 1),), ((1, 1, 1), (1, 2, -1))),
    (((0, 0, 1), (0, 4, 1)), ((0, 2, 1),), ((0, 1, -1), (0, 2, 1))),
)
_ALG_O = (
    (((0, 0, 1),), ((0, 0, 1),), ((0, 0, 1),)),
    (((1, 0, 1),), ((0, 0, 1),), ((1, 0, 1),)),
    (((0, 1, 1), (1, 1, -1)), ((1, 0, 1), (1, 4, -1)), ((0, 0, 1),)),
    (((1, 1, 1),), ((1, 0, 1), (2, 0, 1)), ((0, 0, 1), (1, 0, 1))),
    (((0, 0, 1),), ((0, 1, 1),), ((0, 1, 1),)),
    (((1, 0, 1),), ((0, 1, 1),), ((1, 1, 1),)),
    (((0, 2, 1), (1, 2, -1)), ((2, 1, 1), (2, 3, -1)), ((0, 1, 1),)),
    (((1, 2, 1),), ((1, 1, 1), (2, 1, 1)), ((0, 1, 1), (1, 1, 1))),
    (((0, 0, 1), (1, 0, -1)), ((0, 2, 1), (0, 3, -1), (0, 4, -1)), ((0, 2, 1),)),
    (((1, 0, 1),), ((0, 2, 1), (1, 2, 1), (2, 2, 1)), ((0, 2, 1), (1, 2, 1))),
    (((0, 1, -1), (1, 1, 1)), ((1, 1, -1), (1, 2, -1), (1, 3, 1)), ((1, 3, 1),)),
    (((0, 1, 1),), ((0, 3, 1), (1, 3, 1), (2, 3, 1)), ((0, 3, 1), (1, 3, 1))),
    (((0, 2, -1), (1, 2, 1)), ((2, 0, -1), (2, 2, -1), (2, 4, 1)), ((1, 4, 1),)),
    (((0, 2, 1),), ((0, 4, 1), (1, 4, 1), (2, 4, 1)), ((0, 4, 1), (1, 4, 1))),
    (((0, 2, -1), (1, 1, 1)), ((1, 4, -1), (2, 0, -1)), ((0, 0, 1), (1, 4, -1))),
    (((1, 1, 1), (1, 2, -1)), ((2, 0, 1),), ((1, 0, -1), (1, 4, -1))),
    (((0, 1, 1), (0, 2, -1)), ((1, 4, 1),), ((0, 0, 1), (0, 4, 1))),
    (((0, 1, -1), (1, 2, 1)), ((1, 1, -1), (2, 3, -1)), ((0, 1, 1), (1, 3, -1))),
    (((1, 1, -1), (1, 2, 1)), ((1, 1, 1),), ((1, 1, -1), (1, 3, -1))),
    (((0, 1, -1), (0, 2, 1)), ((2, 3, 1),), ((0, 1, 1), (0, 3, 1))),
    (((0, 1, -1), (1, 0, 1)), ((0, 3, -1), (1, 2, -1)), ((0, 2, 1), (1, 3, -1))),
    (((1, 0, 1), (1, 1, -1)), ((1, 2, 1),), ((1, 2, -1), (1, 3, -1))),
    (((0, 0, 1), (0, 1, -1)), ((0, 3, 1),), ((0, 2, 1), (0, 3, 1))),
    (((0, 2, -1), (1, 0, 1)), ((0, 4, -1), (2, 2, -1)), ((0, 2, 1), (1, 4, -1))),
    (((1, 0, 1), (1, 2, -1)), ((2, 2, 1),), ((1, 2, -1), (1, 4, -1))),
    (((0, 0, 1), (0, 2, -1)), ((0, 4, 1),), ((0, 2, 1), (0, 4, 1))),
)


_ORD_Q = (6, 8, 7, 9, 13, 25, 21, 11, 23, 17, 16, 12, 18, 24, 22, 15, 4, 1, 5, 3, 20, 19, 10, 14, 0, 2)
_ORD_O = (4, 1, 19, 6, 15, 3, 14, 16, 20, 9, 22, 11, 8, 25, 23, 13, 24, 12, 10, 21, 17, 7, 18, 5, 0, 2)


def _plain(nk, nn):
    return tuple((((m, k, 1),), ((k, n, 1),), ((m, n, 1),))
                 for n in range(nn) for k in range(nk) for m in range(2))


class _Alg:
    def __init__(self, table, order=None, round=4, allf=0):
        self.round = round
        if order is not None:
            table = [table[r] for r in order]
        def norm(t):
            sg = t[0][2]
            return tuple((i, j, c * sg) for i, j, c in t), sg
        self.a_forms, self.b_forms, self.prods = [], [], []
        for a, b, c in table:
            (a, sa), (b, sb) = norm(a), norm(b)
            if a not in self.a_forms:
                self.a_forms.append(a)
            if b not in self.b_forms:
                self.b_forms.append(b)
            self.prods.append((a, b, tuple((i, j, v * sa * sb) for i, j, v in c)))
        self.a_multi = [f for f in self.a_forms if len(f) > 1 or allf & 1]
        self.b_multi = [f for f in self.b_forms if len(f) > 1 or allf & 2]


def _combine(form, get):
    r = get(form[0][0], form[0][1])
    for i, j, c in form[1:]:
        r = r + get(i, j) if c > 0 else r - get(i, j)
    return r


def _bilinear(alg, a_of, b_of, init=None):
    out = dict(init or {})

    def acc(d, key, v, sg):
        if key not in d:
            d[key] = (v, sg)
        else:
            w, sw = d[key]
            d[key] = (w + v if sg == sw else w - v, sw)

    for r0 in range(0, len(alg.prods), alg.round):
        groups = {}
        for a, b, c in alg.prods[r0:r0 + alg.round]:
            sg = c[0][2]
            m = jnp.dot(a_of(a), b_of(b), preferred_element_type=_F32)
            acc(groups, tuple((i, j, v * sg) for i, j, v in c), m, sg)
        part = {}
        for c, (tot, tsg) in groups.items():
            for i, j, v in c:
                acc(part, (i, j), tot, v * tsg)
        for key, (v, sg) in part.items():
            if key not in out:
                out[key] = v if sg > 0 else -v
            else:
                out[key] = out[key] + v if sg > 0 else out[key] - v
    return out


def _pack(v):
    return pltpu.bitcast(v, jnp.uint32)


def _unpack(v):
    return pltpu.bitcast(v, _BF16)


def _split(v):
    u = _pack(v)
    return tuple(pltpu.unpack_elementwise(u, index=i, packed_dtype=_BF16, unpacked_dtype=_F32)
                 for i in range(2))


def _form(f, get):
    halves = [_combine(f, lambda i, j: get(i, j)[h]) for h in range(2)]
    r = pltpu.pack_elementwise(halves, packed_dtype=_BF16)
    return r if r.dtype == jnp.uint32 else pltpu.bitcast(r, jnp.uint32)


def _nt(a, b):
    return jax.lax.dot_general(a, b, _NT, preferred_element_type=_F32)


def _lo(n):
    return jax.lax.broadcasted_iota(jnp.int32, (n, 128), 1) < 64


def _qfin(c):
    t0, t1, t2 = [jnp.concatenate([c[0, n], c[1, n]], axis=0) * _SCALE for n in range(3)]
    lo = _lo(t1.shape[0])
    zero = jnp.zeros_like(t1)
    q1 = jnp.concatenate([t0, jnp.where(lo, t1, zero)], axis=1).astype(_BF16)
    q2 = jnp.concatenate([jnp.where(lo, zero, t1), t2], axis=1).astype(_BF16)
    return q1, q2


def _qk(q1, q2, kt):
    s1 = jnp.dot(q1, kt[0:256], preferred_element_type=_F32)
    s2 = jnp.dot(q2, kt[128:384], preferred_element_type=_F32)
    return s1, s2


def _soft(s, ch, raw=False, sumb=False):
    if sumb:
        ps, rs = [], []
        for c in (s[0:128], s[128:]):
            m = jnp.max(c, axis=-1, keepdims=True)
            p = jnp.exp2(c - m).astype(_BF16)
            l = jnp.sum(p.astype(_F32), axis=-1, keepdims=True)
            r = pl.reciprocal(l, approx=True)
            rs.append(r * (2.0 - l * r))
            ps.append(p)
        return tuple(ps), rs
    m = jnp.max(s, axis=-1, keepdims=True)
    p = jnp.exp2(s - m)
    l = jnp.sum(p, axis=-1, keepdims=True)
    r = pl.reciprocal(l, approx=True)
    rs = [r * (2.0 - l * r)]
    if raw:
        return (p, None), rs
    return (p[0:128].astype(_BF16), p[128:].astype(_BF16)), rs


def _pv_top(p, vt_h):
    return _nt(vt_h, p[0])


def _pv_rem(p1, p2, vt):
    p1r, p2r = p1[1], p2[1]
    n = p1r.shape[0]
    ra = _nt(p1r, vt[0:128])
    rm = _nt(jnp.concatenate([p1r, p2r], axis=0), vt[128:256])
    rc = _nt(p2r, vt[256:384])
    return jnp.concatenate([ra, jnp.where(_lo(n), rm[0:n], rm[n:2 * n]), rc], axis=1)


def _pv_fin(ot1, ot2, o_r, r1, r2):
    o_top = jnp.concatenate([ot1, ot2], axis=0).T
    o = jnp.concatenate([o_top, o_r], axis=0)
    outs = []
    i0 = 0
    for a, b in zip(r1, r2):
        ch = a.shape[0]
        rr = jnp.concatenate([jnp.broadcast_to(a, (ch, 128)),
                              jnp.where(_lo(ch), a, b),
                              jnp.broadcast_to(b, (ch, 128))], axis=1)
        outs.append(o[i0:i0 + ch] * rr)
        i0 += ch
    return jnp.concatenate(outs, axis=0) if len(outs) > 1 else outs[0]


def _kernel(xa, ka, va, wqa, woa, xb, kb, vb, wqb, wob, out,
            x_res, wq_res, wo_res, acc, ostage, kv, s_scr, o_scr, xc, wqc, woc, p_scr, q_scr, f_scr, zero_ref,
            g_sem, w_sem, p_sem, o_sem, *, nb, n_pair, ring, sched, g_init, w_pos, late, order, order1, aq, ao, w1_at, ch, mat, noost, wstat, wmerge, gate, walign):
    lg = nb.bit_length() - 1
    assert nb == 1 << lg
    n_pos = n_pair * nb
    sq, d = x_res.shape[2], x_res.shape[3]
    wqs, wos = (wqa, wqb), (woa, wob)

    def static(v):
        return isinstance(v, int)

    def bp(u):
        if static(u):
            return u & (nb - 1), u >> lg
        return u & (nb - 1), jax.lax.shift_right_logical(u, lg)

    def clamp(u, hi=n_pos - 1):
        return min(max(u, 0), hi) if static(u) else jnp.clip(u, 0, hi)

    def when(cond):
        if isinstance(cond, bool):
            return (lambda f: f()) if cond else (lambda f: None)
        return pl.when(cond)

    def pair_ds(p):
        return pl.ds(p * _PAIR if static(p) else pl.multiple_of(p * _PAIR, _PAIR), _PAIR)

    def chunk(ref, u):
        b, p = bp(u)
        return ref.at[b, pair_ds(p), :]

    n_last = sched[-1][0]
    u_last = n_pos - n_last * sched[-1][1]
    lg_last = n_last.bit_length() - 1
    n_par = ring // n_last
    merged = u_last >= nb and n_last > 1

    def sem_of(u):
        if not merged:
            return u & (ring - 1)
        if static(u):
            return u & (ring - 1) if u < u_last else ring + ((u >> lg_last) & (n_par - 1))
        big = ring + (jax.lax.shift_right_logical(u, lg_last) & (n_par - 1))
        if all_last[0]:
            return big
        return jnp.where(u < u_last, u & (ring - 1), big)

    def issue(u, h, enable=True):
        uc = clamp(u)
        slot = uc & (ring - 1)
        sem = g_sem.at[sem_of(uc)]

        def both(c):
            if isinstance(enable, bool):
                return c if enable else False
            return enable if c is True else jnp.logical_and(enable, c)

        if x_possible[0]:
            ux = clamp(u + h, nb - 1)

            @when(both(u + h < nb))
            def _():
                src, br = (xb, 1) if h == 0 else (xa, 0)
                pltpu.make_async_copy(src.at[ux], x_res.at[br, ux], sem).start()
        srcs = (chunk(va, uc), chunk(kb, uc)) if h == 0 else (chunk(vb, uc), chunk(ka, clamp(u + 1)))
        for i, s in enumerate(srcs):
            @when(both(u < n_pos))
            def _():
                pltpu.make_async_copy(s, kv.at[slot, 2 * h + i], sem).start()
        if x_possible[0] and h == 1:
            @when(both(u == w1_at))
            def _():
                w_start(1)

    def wq_copy(p, br, sem):
        return pltpu.make_async_copy(wqs[br].at[:, pair_ds(p)], wq_res.at[p, br], sem)

    def wo_copy(p, br, sem):
        return pltpu.make_async_copy(wos[br].at[pair_ds(p), :], wo_res.at[p, br], sem)

    def w_start(p):
        sem = w_sem.at[p & 1]
        for br in range(2):
            wq_copy(p, br, sem).start()
            wo_copy(p, br, sem).start()

    def w_wait(p):
        sem = w_sem.at[p & 1]
        pltpu.make_async_copy(wq_res.at[p], wq_res.at[p], sem).wait()
        pltpu.make_async_copy(wo_res.at[p], wo_res.at[p], sem).wait()

    def out_copy(b):
        return pltpu.make_async_copy(ostage.at[b], out.at[b], o_sem.at[b])

    hm = sq // 2
    wo_off = 0
    if wmerge:
        woc, wo_off = wqc, len(aq.b_multi)

    def tile(ref, i, j, rows):
        return ref[i * rows:(i + 1) * rows, j * 128:(j + 1) * 128]

    def qproj(br, b, p):
        x, w = x_res.at[br, b], wq_res.at[p, br]

        def a_of(f):
            if f not in aq.a_multi:
                return tile(x, f[0][0], f[0][1], hm)
            return _unpack(xc[br, b, aq.a_multi.index(f)])

        def b_of(f):
            if f not in aq.b_multi:
                return tile(w, f[0][0], f[0][1], 128)
            return _unpack(wqc[p & 1, br, aq.b_multi.index(f)])
        return _qfin(_bilinear(aq, a_of, b_of))

    def o_forms(o):
        return [_combine(f, lambda i, j: tile(o, i, j, hm)).astype(_BF16) for f in ao.a_forms]

    def oproj(forms, br, b, p, stage_out=True):
        w = wo_res.at[p, br]

        def b_of(f):
            if f not in ao.b_multi:
                return tile(w, f[0][0], f[0][1], 128)
            return _unpack(woc[p & 1, br, wo_off + ao.b_multi.index(f)])
        a = acc.at[br, b]
        init = {(i, j): tile(a, i, j, hm) for i in range(2) for j in range(d // 128)}
        c = _bilinear(ao, lambda f: forms[ao.a_forms.index(f)], b_of, init)
        for (i, j), v in c.items():
            a[i * hm:(i + 1) * hm, j * 128:(j + 1) * 128] = v
        if stage_out:
            for i in range(2):
                row = jnp.concatenate([c[i, j] for j in range(d // 128)], axis=1)
                ostage[b, i * hm:(i + 1) * hm, br * d:(br + 1) * d] = row.astype(ostage.dtype)

    def x_forms(br, b):
        x = x_res.at[br, b]
        blk = {}

        def get(i, j):
            if (i, j) not in blk:
                blk[i, j] = _split(tile(x, i, j, hm))
            return blk[i, j]
        for r, f in enumerate(aq.a_multi):
            xc[br, b, r] = (_pack(tile(x, f[0][0], f[0][1], hm)) if len(f) == 1
                            else _form(f, get))

    def w_forms(br, p, si, which=(0, 1), lo=0):
        for t in which:
            raw, dst, alg = ((wq_res, wqc, aq), (wo_res, woc, ao))[t]
            rows = raw.shape[2]
            ext = 16 * (lo + 1)
            if static(si):
                view = raw.at[p, br, pl.ds(si * 16, rows - 128 + ext)]
                off2 = (si + lo) * 8
            else:
                view = raw.at[p, br, pl.ds(pl.multiple_of(si * 16, 16), rows - 128 + ext)]
                off2 = pl.multiple_of((si + lo) * 8, 8)
            blk = {}

            def src(i, j):
                return view[i * 128 + lo * 16:i * 128 + lo * 16 + 16, j * 128:(j + 1) * 128]

            def get(i, j):
                if (i, j) not in blk:
                    blk[i, j] = _split(src(i, j))
                return blk[i, j]
            for r, f in enumerate(alg.b_multi):
                dst[p & 1, br, r + t * wo_off, pl.ds(off2, 8), :] = (
                    _pack(src(f[0][0], f[0][1])) if len(f) == 1 else _form(f, get))

    def waits_for(u0, n, maybe_first):
        if merged and all_last[0]:
            slot = u0 & (ring - 1)
            blk = kv.at[pl.ds(slot if static(slot) else pl.multiple_of(slot, n), n)]
            pltpu.make_async_copy(blk, blk, g_sem.at[sem_of(u0)]).wait()
        for i in range(0 if merged and all_last[0] else n):
            u = u0 + i
            sem = g_sem.at[u & (ring - 1)]
            slot = u & (ring - 1)
            pltpu.make_async_copy(kv.at[slot], kv.at[slot], sem).wait()
            if maybe_first:
                for h in range(2):
                    @when(u + h < nb)
                    def _():
                        pltpu.make_async_copy(x_res.at[0, 0], x_res.at[0, 0], sem).wait()
        b0, p0 = bp(u0)

        @when((b0 == nb // 2 and p0 + 1 < n_pair) if static(u0)
              else jnp.logical_and(b0 == nb // 2, p0 + 1 < n_pair))
        def _():
            w_wait(p0 + 1)

    zero_ref[0] = 0
    x_possible = [True]
    all_last = [False]
    assert g_init < ring
    first = [pltpu.make_async_copy(xa.at[0], x_res.at[0, 0], p_sem.at[0]),
             wq_copy(0, 0, p_sem.at[0]),
             pltpu.make_async_copy(chunk(ka, 0), kv.at[ring - 1, 3], p_sem.at[0])]
    for c in first:
        c.start()
    second = [wq_copy(0, 1, p_sem.at[1]), wo_copy(0, 0, p_sem.at[1]), wo_copy(0, 1, p_sem.at[1])]

    def start_rest():
        second[0].start()
        second[1].start()
        for g in range(g_init):
            issue(g, 0)
            issue(g, 1)
            if g == 0:
                second[2].start()

    if not late:
        start_rest()

    def zero(b, carry):
        for br in range(2):
            acc[br, b] = jnp.zeros((sq, d), _F32)
        return carry
    jax.lax.fori_loop(0, nb, zero, 0)
    o_scr[...] = jnp.zeros(o_scr.shape, o_scr.dtype)

    for c in first:
        c.wait()
    if late:
        start_rest()

    def w0a(si, carry):
        w_forms(0, 0, si, (0,))
        return carry
    jax.lax.fori_loop(0, 8, w0a, 0)
    x_forms(0, 0)
    s1, s2 = _qk(*qproj(0, 0, 0), kv[ring - 1, 3])
    s_scr[0] = s1
    s_scr[1] = s2
    for c in second:
        c.wait()

    def w0b(si, carry):
        w_forms(0, 0, si, (1,))
        w_forms(1, 0, si)
        return carry
    jax.lax.fori_loop(0, 8, w0b, 0)

    def run_phase(u_start, n, cnt, g0, dbl):
        T = 2 * n
        maybe_first = u_start < nb
        maybe_last = u_start + n * cnt > n_pos - nb
        x_possible[0] = g0 < nb
        all_last[0] = u_start >= u_last

        def body(j, carry):
            u0 = u_start + j * n

            def task(k):
                if k == -1:
                    br, u = 1, clamp(u0 - 1)
                elif k == T:
                    br, u = 0, clamp(u0 + n)
                else:
                    br, u = k % 2, u0 + k // 2
                return (br,) + bp(u)

            def slot(k):
                return (u0 + k // 2) & (ring - 1)

            Q, S, P, O, OT, OR, G = {}, {}, {}, {}, {}, {}, {}
            S[0, 0] = s_scr[0]
            S[0, 1] = s_scr[1]
            O[-1] = [_unpack(o_scr[r]) for r in range(len(ao.a_forms))]

            def kref(k):
                return kv.at[slot(k - 1), 1 if k % 2 == 1 else 3]

            def vref(k):
                return kv.at[slot(k), 0 if k % 2 == 0 else 2]

            def do_q(k):
                Q[k, 0], Q[k, 1] = qproj(*task(k))
                if mat & 2:
                    for h in range(2):
                        q_scr[k % 2, h] = _pack(Q[k, h])
                        Q[k, h] = _unpack(q_scr[k % 2, h])

            def do_x(k):
                br, b, _ = task(k)
                x_forms(br, b)

            def do_w(k):
                br, b, p = task(k)
                half = nb // 2
                pc = jnp.minimum(p + jax.lax.shift_right_logical(b, lg - 1), n_pair - 1)
                bh = k // 2 if n == half and wstat is True else (b + (carry if wstat == 2 else 0)) & (half - 1)
                if gate:
                    v = G.pop(k)
                    bh = bh + (pltpu.bitcast(v[0:8, 0:128], jnp.int32)[0, 0] & carry)
                if walign and n >= 4 and half == 8:
                    w_forms(br, pc, b & 4, lo=(k // 2) & 3)
                    return
                for i in range(8 // half):
                    w_forms(br, pc, bh * (8 // half) + i)

            def do_qk(k, h):
                S[k, h] = jnp.dot(Q.pop((k, h)), kref(k)[128 * h:128 * h + 256, :],
                                  preferred_element_type=_F32)
                if gate == 1 + h:
                    G[k - 1] = S[k, h]

            def do_sm(k, h):
                (pt, pr), r = _soft(S.pop((k, h)), ch, mat & 1, mat & 8)
                if mat & 1:
                    for c in range(4):
                        p_scr[k % 2, h, c] = _pack(pt[:, c * 128:(c + 1) * 128].astype(_BF16))
                    pt = jnp.concatenate([_unpack(p_scr[k % 2, h, c, 0:64]) for c in range(4)], axis=1)
                    pr = jnp.concatenate([_unpack(p_scr[k % 2, h, c, 64:sq // 2]) for c in range(4)], axis=1)
                P[k, h] = (pt, pr), r

            def do_pt(k, h):
                OT[k, h] = _pv_top(P[k, h][0], vref(k)[192 * h:192 * h + 192, :])
                if gate == 3 + h:
                    G[k] = OT[k, h]

            def do_pr(k):
                OR[k] = _pv_rem(P[k, 0][0], P[k, 1][0], vref(k)[...])

            def do_pf(k):
                O[k] = o_forms(_pv_fin(OT.pop((k, 0)), OT.pop((k, 1)), OR.pop(k),
                                       P.pop((k, 0))[1], P.pop((k, 1))[1]))
                if mat & 4 and k < T - 1:
                    for r, v in enumerate(O[k]):
                        f_scr[k % 2, r] = _pack(v)
                    O[k] = [_unpack(f_scr[k % 2, r]) for r in range(len(ao.a_forms))]

            def do_o(k):
                br, b, p = task(k)
                oproj(O.pop(k), br, b, p, maybe_last and not noost)
                if br == 1 and maybe_last:
                    last = (p == n_pair - 1) if k >= 0 else (u0 - 1 >= n_pos - nb)

                    @pl.when(last)
                    def _():
                        out_copy(b).start()

            def refill(k):
                i = j * n + k // 2
                h = k % 2
                if dbl:
                    fast = i < dbl // 2
                    g = g0 + i + jnp.minimum(i, dbl // 2)
                    if h == 0:
                        issue(g, 0)
                        issue(g, 1, fast)
                    else:
                        g = g + fast.astype(jnp.int32)
                        issue(g, 0, fast)
                        issue(g, 1)
                else:
                    issue(g0 + i, h)

            ops = {"q": lambda k: do_q(k + 1), "a": lambda k: do_qk(k + 1, 0),
                   "b": lambda k: do_qk(k + 1, 1), "s": lambda k: do_sm(k, 0),
                   "t": lambda k: do_sm(k, 1), "u": lambda k: do_pt(k, 0),
                   "v": lambda k: do_pt(k, 1), "r": do_pr, "f": do_pf,
                   "o": lambda k: do_o(k - 1), "d": refill,
                   "x": lambda k: do_x(k + 1), "w": do_w,
                   "Q": lambda k: do_q(k + 2), "X": lambda k: do_x(k + 2),
                   "B": lambda k: do_qk(k, 1), "R": lambda k: do_pr(k - 1),
                   "V": lambda k: do_pt(k - 1, 1), "F": lambda k: do_pf(k - 1)}
            od = order1 if maybe_first else order
            for k in range(T):
                of, om, ol = (od.split("/") * 3)[:3] if "/" not in od else od.split("/")
                for c in (ol if k == T - 1 else of if k == 0 else om):
                    ops[c](k)
            b0, p0 = bp(u0)

            @pl.when(jnp.logical_and(b0 == (w_pos // n) * n, p0 + 2 < n_pair))
            def _():
                w_start(p0 + 2)
            s_scr[0] = S.pop((T, 0))
            s_scr[1] = S.pop((T, 1))
            for r, v in enumerate(O.pop(T - 1)):
                o_scr[r] = _pack(v)

            @pl.when(j + 1 < cnt)
            def _():
                waits_for(u0 + n, n, maybe_first)
            return carry

        waits_for(u_start, n, maybe_first)
        jax.lax.fori_loop(0, cnt, body, zero_ref[0])

    issued = {(g, h): -1 for g in range(g_init) for h in range(2)}
    u_start, g0 = 0, g_init
    plan = []
    for n, cnt, dbl in sched:
        assert dbl % 2 == 0 and nb % n == 0 and u_start % n == 0
        plan.append((u_start, n, cnt, g0, dbl))
        for t in range(2 * n * cnt):
            i, h, tg = t // 2, t % 2, 2 * u_start + t
            if i < dbl // 2:
                gs = [(g0 + 2 * i + h, 0), (g0 + 2 * i + h, 1)]
            else:
                gs = [(g0 + i + dbl // 2, h)]
            for g, hh in gs:
                assert (g, hh) not in issued
                issued[(g, hh)] = tg
                assert 2 * (g - ring) + hh + 1 < tg
            if t % (2 * n) == 0:
                for u in range(u_start + i, u_start + i + n):
                    assert issued[(u, 0)] < tg and issued[(u, 1)] < tg
        g0 += n * cnt + dbl // 2
        u_start += n * cnt
    assert u_start == n_pos
    for u_start, n, cnt, g0, dbl in plan:
        assert w_pos < nb
        run_phase(u_start, n, cnt, g0, dbl)

    oproj([_unpack(o_scr[r]) for r in range(len(ao.a_forms))], 1, nb - 1, n_pair - 1)
    out_copy(nb - 1).start()
    for b in range(nb):
        out_copy(b).wait()


def _build(A_x, A_k_cache, A_v_cache, A_wq, A_wo,
           B_x, B_k_cache, B_v_cache, B_wq, B_wo, *,
           sched=((1, 32, 16), (8, 28, 0)), g_init=1, w_pos=12, late=False,
           order='stqdwouvrfab/dstqwouvrfab/dstqwouvrfab',
           order1='stxouqdvrfabw/dstxouqvrfabw/dstxouqvrfabw', fq=True, fo=True, w1_at=7, rnd=4, ch=160, mat=8, noost=False, allf=3, opad=20, wstat=False, wmerge=False, gate=0, walign=True, nobc=True, ring=16, interpret=False):
    nb, sq, d = A_x.shape
    n_head, sk = A_k_cache.shape[1], A_k_cache.shape[2]
    n_pair = n_head // 2

    def tr(c):
        return jnp.swapaxes(c, 2, 3).reshape(nb, n_head * _DH, sk)

    any_spec = pl.BlockSpec(memory_space=pl.ANY)
    aq = _Alg(_ALG_Q, _ORD_Q, rnd, allf) if fq else _Alg(_plain(5, 3), None, rnd, allf)
    ao = _Alg(_ALG_O, _ORD_O, rnd, allf) if fo else _Alg(_plain(3, 5), None, rnd, allf)
    return pl.pallas_call(
        functools.partial(_kernel, nb=nb, n_pair=n_pair, ring=ring, sched=sched,
                          g_init=g_init, w_pos=w_pos, late=late, order=order,
                          order1=order1, aq=aq, ao=ao, w1_at=w1_at, ch=ch, mat=mat, noost=noost, wstat=wstat, wmerge=wmerge, gate=gate, walign=walign),
        in_specs=[any_spec] * 10,
        out_specs=any_spec,
        out_shape=jax.ShapeDtypeStruct((nb, sq, 2 * d), A_x.dtype),
        scratch_shapes=[
            pltpu.VMEM((2, nb, sq, d), _BF16),
            pltpu.VMEM((n_pair, 2, d, _PAIR), _BF16),
            pltpu.VMEM((n_pair, 2, _PAIR, d), _BF16),
            pltpu.VMEM((2, nb, sq, d), _F32),
            pltpu.VMEM((nb, sq, 2 * d), _BF16),
            pltpu.VMEM((ring, 4, _PAIR, sk), _BF16),
            pltpu.VMEM((2, sq, sk), _F32),
            pltpu.VMEM((opad, sq // 4, 128), jnp.uint32),
            pltpu.VMEM((2, nb, max(len(aq.a_multi), 1), sq // 4, 128), jnp.uint32),
            pltpu.VMEM((2, 2, max(len(aq.b_multi), 1) + (len(ao.b_multi) if wmerge else 0), 64, 128),
                       jnp.uint32),
            pltpu.VMEM((2, 2, 1 if wmerge else max(len(ao.b_multi), 1), 64, 128), jnp.uint32),
            pltpu.VMEM((2, 2, 4, sq // 2, 128), jnp.uint32),
            pltpu.VMEM((2, 2, sq // 2, 256), jnp.uint32),
            pltpu.VMEM((2, len(ao.a_forms), sq // 4, 128), jnp.uint32),
            pltpu.SMEM((1,), jnp.int32),
            pltpu.SemaphoreType.DMA((2 * ring,)),
            pltpu.SemaphoreType.DMA((2,)),
            pltpu.SemaphoreType.DMA((2,)),
            pltpu.SemaphoreType.DMA((nb,)),
        ],
        compiler_params=pltpu.CompilerParams(
            vmem_limit_bytes=120 * 1024 * 1024,
            disable_bounds_checks=nobc),
        interpret=interpret,
    )(A_x, tr(A_k_cache), tr(A_v_cache), A_wq, A_wo,
      B_x, tr(B_k_cache), tr(B_v_cache), B_wq, B_wo)


@jax.jit
def pallas_concat_heads__gqa_block_cached__mha_block_cached__near_ridge_kernel(
    A_x: jax.Array,
    A_k_cache: jax.Array,
    A_v_cache: jax.Array,
    A_wq: jax.Array,
    A_wo: jax.Array,
    B_x: jax.Array,
    B_k_cache: jax.Array,
    B_v_cache: jax.Array,
    B_wq: jax.Array,
    B_wo: jax.Array,
):
    return _build(A_x, A_k_cache, A_v_cache, A_wq, A_wo,
                  B_x, B_k_cache, B_v_cache, B_wq, B_wo)
```

```python
import functools
import math

import jax
import jax.numpy as jnp
import jax.experimental.pallas as pl
import jax.experimental.pallas.tpu as pltpu

_H = 32
_DH = 192
_PAIR = 2 * _DH
_NP = _H // 2

_NT = (((1,), (1,)), ((), ()))
_F32 = jnp.float32
_BF16 = jnp.bfloat16
_SCALE = (_DH ** -0.5) * math.log2(math.e)

_ALG_Q = (
    (((0, 0, 1),), ((0, 0, 1),), ((0, 0, 1),)),
    (((1, 0, 1),), ((0, 0, 1),), ((1, 0, 1),)),
    (((0, 1, 1),), ((1, 0, 1),), ((0, 0, 1),)),
    (((1, 1, 1),), ((1, 0, 1),), ((1, 0, 1),)),
    (((0, 2, 1), (1, 2, -1)), ((2, 0, 1), (2, 1, -1), (2, 2, -1)), ((0, 0, 1),)),
    (((1, 2, 1),), ((2, 0, 1), (3, 0, 1), (4, 0, 1)), ((0, 0, 1), (1, 0, 1))),
    (((0, 0, 1), (1, 0, -1)), ((0, 1, 1), (0, 2, 1)), ((0, 1, 1),)),
    (((1, 0, 1),), ((0, 1, 1), (4, 1, -1)), ((0, 1, 1), (1, 1, 1))),
    (((0, 3, -1), (1, 3, 1)), ((3, 0, -1), (3, 1, 1), (3, 2, 1)), ((1, 1, 1),)),
    (((0, 3, 1),), ((1, 1, 1), (2, 1, 1), (3, 1, 1)), ((0, 1, 1), (1, 1, 1))),
    (((0, 1, 1), (1, 1, -1)), ((1, 1, 1), (1, 2, 1)), ((0, 2, 1),)),
    (((1, 1, 1),), ((1, 2, 1), (3, 2, 1)), ((0, 2, 1), (1, 2, 1))),
    (((0, 4, -1), (1, 4, 1)), ((4, 0, -1), (4, 1, 1), (4, 2, 1)), ((1, 2, 1),)),
    (((0, 4, 1),), ((0, 2, -1), (2, 2, 1), (4, 2, 1)), ((0, 2, 1), (1, 2, 1))),
    (((0, 3, -1), (1, 2, 1)), ((2, 1, -1), (3, 0, -1)), ((0, 0, 1), (1, 1, -1))),
    (((1, 2, 1), (1, 3, -1)), ((3, 0, 1),), ((1, 0, -1), (1, 1, -1))),
    (((0, 2, 1), (0, 3, -1)), ((2, 1, 1),), ((0, 0, 1), (0, 1, 1))),
    (((0, 4, -1), (1, 2, 1)), ((2, 2, -1), (4, 0, -1)), ((0, 0, 1), (1, 2, -1))),
    (((1, 2, 1), (1, 4, -1)), ((4, 0, 1),), ((1, 0, -1), (1, 2, -1))),
    (((0, 2, 1), (0, 4, -1)), ((2, 2, 1),), ((0, 0, 1), (0, 2, 1))),
    (((0, 3, 1), (1, 1, -1)), ((1, 1, -1), (3, 2, 1)), ((0, 2, 1), (1, 1, 1))),
    (((0, 1, -1), (0, 3, 1)), ((1, 1, 1),), ((0, 1, -1), (0, 2, 1))),
    (((1, 1, -1), (1, 3, 1)), ((3, 2, 1),), ((1, 1, -1), (1, 2, 1))),
    (((0, 4, 1), (1, 0, 1)), ((0, 2, 1), (4, 1, 1)), ((0, 1, 1), (1, 2, 1))),
    (((1, 0, 1), (1, 4, 1)), ((4, 1, 1),), ((1, 1, 1), (1, 2, -1))),
    (((0, 0, 1), (0, 4, 1)), ((0, 2, 1),), ((0, 1, -1), (0, 2, 1))),
)
_ALG_O = (
    (((0, 0, 1),), ((0, 0, 1),), ((0, 0, 1),)),
    (((1, 0, 1),), ((0, 0, 1),), ((1, 0, 1),)),
    (((0, 1, 1), (1, 1, -1)), ((1, 0, 1), (1, 4, -1)), ((0, 0, 1),)),
    (((1, 1, 1),), ((1, 0, 1), (2, 0, 1)), ((0, 0, 1), (1, 0, 1))),
    (((0, 0, 1),), ((0, 1, 1),), ((0, 1, 1),)),
    (((1, 0, 1),), ((0, 1, 1),), ((1, 1, 1),)),
    (((0, 2, 1), (1, 2, -1)), ((2, 1, 1), (2, 3, -1)), ((0, 1, 1),)),
    (((1, 2, 1),), ((1, 1, 1), (2, 1, 1)), ((0, 1, 1), (1, 1, 1))),
    (((0, 0, 1), (1, 0, -1)), ((0, 2, 1), (0, 3, -1), (0, 4, -1)), ((0, 2, 1),)),
    (((1, 0, 1),), ((0, 2, 1), (1, 2, 1), (2, 2, 1)), ((0, 2, 1), (1, 2, 1))),
    (((0, 1, -1), (1, 1, 1)), ((1, 1, -1), (1, 2, -1), (1, 3, 1)), ((1, 3, 1),)),
    (((0, 1, 1),), ((0, 3, 1), (1, 3, 1), (2, 3, 1)), ((0, 3, 1), (1, 3, 1))),
    (((0, 2, -1), (1, 2, 1)), ((2, 0, -1), (2, 2, -1), (2, 4, 1)), ((1, 4, 1),)),
    (((0, 2, 1),), ((0, 4, 1), (1, 4, 1), (2, 4, 1)), ((0, 4, 1), (1, 4, 1))),
    (((0, 2, -1), (1, 1, 1)), ((1, 4, -1), (2, 0, -1)), ((0, 0, 1), (1, 4, -1))),
    (((1, 1, 1), (1, 2, -1)), ((2, 0, 1),), ((1, 0, -1), (1, 4, -1))),
    (((0, 1, 1), (0, 2, -1)), ((1, 4, 1),), ((0, 0, 1), (0, 4, 1))),
    (((0, 1, -1), (1, 2, 1)), ((1, 1, -1), (2, 3, -1)), ((0, 1, 1), (1, 3, -1))),
    (((1, 1, -1), (1, 2, 1)), ((1, 1, 1),), ((1, 1, -1), (1, 3, -1))),
    (((0, 1, -1), (0, 2, 1)), ((2, 3, 1),), ((0, 1, 1), (0, 3, 1))),
    (((0, 1, -1), (1, 0, 1)), ((0, 3, -1), (1, 2, -1)), ((0, 2, 1), (1, 3, -1))),
    (((1, 0, 1), (1, 1, -1)), ((1, 2, 1),), ((1, 2, -1), (1, 3, -1))),
    (((0, 0, 1), (0, 1, -1)), ((0, 3, 1),), ((0, 2, 1), (0, 3, 1))),
    (((0, 2, -1), (1, 0, 1)), ((0, 4, -1), (2, 2, -1)), ((0, 2, 1), (1, 4, -1))),
    (((1, 0, 1), (1, 2, -1)), ((2, 2, 1),), ((1, 2, -1), (1, 4, -1))),
    (((0, 0, 1), (0, 2, -1)), ((0, 4, 1),), ((0, 2, 1), (0, 4, 1))),
)


_ALG25_Q = (
    (((0, 1, 1),), ((0, 1, -1), (1, 1, 1), (2, 0, 1), (2, 1, 1)), ((0, 1, 1), (1, 1, 1))),
    (((0, 1, 1), (1, 0, 1)), ((0, 1, 1), (1, 0, 1)), ((0, 0, 1), (1, 1, 1))),
    (((0, 2, 1), (0, 3, -1)), ((2, 0, 1),), ((0, 0, 1), (0, 1, -1), (1, 0, 1), (1, 1, -1))),
    (((1, 3, 1), (1, 4, 1)), ((4, 1, -1),), ((0, 1, -1), (1, 1, -1))),
    (((0, 2, 1), (0, 3, -1), (1, 2, -1), (1, 3, 1)), ((3, 0, 1), (3, 2, 1)), ((1, 0, 1), (1, 1, -1))),
    (((0, 1, 1), (1, 2, -1)), ((1, 2, -1), (2, 0, -1), (2, 1, -1)), ((0, 2, -1), (1, 1, 1))),
    (((0, 1, -1), (1, 1, 1)), ((1, 0, 1), (1, 1, 1), (1, 2, -1)), ((1, 1, 1),)),
    (((0, 2, 1), (0, 3, -1), (1, 2, -1)), ((2, 0, -1), (3, 0, -1), (3, 2, -1)), ((0, 2, 1), (1, 0, 1), (1, 1, -1))),
    (((0, 4, 1), (1, 0, -1)), ((0, 2, 1), (4, 0, 1), (4, 2, 1)), ((0, 0, 1), (1, 0, 1), (1, 2, -1))),
    (((1, 0, 1),), ((0, 0, 1), (0, 2, 1), (1, 0, -1), (4, 0, 1), (4, 2, 1)), ((0, 0, 1), (1, 0, 1))),
    (((0, 4, -1), (1, 4, 1)), ((3, 0, -1), (3, 1, -1), (4, 0, 1), (4, 1, 1)), ((1, 0, 1), (1, 2, -1))),
    (((0, 4, 1),), ((0, 2, -1), (4, 2, -1)), ((0, 0, 1), (0, 2, -1), (1, 0, 1), (1, 2, -1))),
    (((0, 0, -1), (0, 4, 1)), ((0, 2, -1),), ((0, 2, 1),)),
    (((0, 2, 1), (1, 2, -1)), ((2, 1, -1), (2, 2, 1), (3, 0, 1), (3, 2, 1)), ((0, 2, 1),)),
    (((1, 0, -1), (1, 4, 1)), ((4, 0, 1), (4, 2, 1)), ((1, 2, 1),)),
    (((1, 2, 1),), ((1, 2, 1), (2, 2, 1)), ((0, 2, 1), (1, 2, 1))),
    (((0, 1, 1), (0, 2, -1)), ((2, 0, 1), (2, 1, 1)), ((0, 1, -1), (0, 2, -1))),
    (((0, 3, 1),), ((2, 0, 1), (3, 0, 1)), ((0, 0, 1), (0, 1, -1), (0, 2, -1))),
    (((0, 3, 1), (0, 4, 1), (1, 3, -1), (1, 4, -1)), ((3, 0, 1), (3, 1, 1)), ((0, 1, 1),)),
    (((0, 0, 1), (0, 1, 1)), ((0, 1, 1),), ((0, 0, -1), (0, 1, 1))),
    (((1, 1, 1), (1, 2, -1)), ((1, 2, 1),), ((1, 1, 1), (1, 2, 1))),
    (((1, 3, 1),), ((3, 0, -1), (3, 1, -1), (3, 2, -1), (4, 1, 1)), ((1, 0, 1), (1, 1, -1), (1, 2, -1))),
    (((1, 0, 1), (1, 1, 1)), ((1, 0, 1),), ((1, 0, 1), (1, 1, -1))),
    (((0, 4, -1), (1, 3, 1), (1, 4, 1)), ((3, 0, -1), (3, 1, -1), (4, 1, 1)), ((0, 1, -1), (1, 0, -1), (1, 2, 1))),
    (((0, 0, 1), (1, 0, -1)), ((0, 0, 1), (0, 1, 1)), ((0, 0, 1),)),
)
_ALG25_O = (
    (((1, 0, 1), (1, 2, -1)), ((0, 2, 1), (0, 3, -1), (1, 2, -1)), ((0, 2, 1), (1, 2, 1))),
    (((1, 0, 1), (1, 1, 1), (1, 2, -1)), ((1, 2, 1),), ((1, 1, 1), (1, 2, 1))),
    (((0, 0, 1), (0, 2, -1), (1, 0, -1), (1, 2, 1)), ((2, 1, 1), (2, 2, -1)), ((0, 2, 1),)),
    (((0, 1, 1), (1, 0, 1), (1, 2, -1)), ((1, 2, -1), (2, 1, -1)), ((0, 2, -1), (1, 1, 1))),
    (((0, 0, 1), (0, 1, 1), (0, 2, -1)), ((0, 4, 1),), ((0, 0, -1), (0, 4, 1))),
    (((1, 0, -1), (1, 1, -1), (1, 2, 1)), ((2, 0, -1),), ((1, 0, -1), (1, 4, 1))),
    (((0, 1, 1), (0, 2, -1), (1, 0, 1)), ((0, 4, 1), (2, 0, -1)), ((0, 0, 1), (1, 4, 1))),
    (((0, 1, 1), (0, 2, -1)), ((0, 4, -1), (1, 3, 1), (1, 4, 1)), ((0, 4, 1), (1, 4, 1))),
    (((0, 1, 1), (0, 2, -1), (1, 1, -1), (1, 2, 1)), ((2, 0, -1), (2, 4, -1)), ((1, 4, -1),)),
    (((1, 1, 1),), ((1, 3, 1),), ((0, 3, 1), (0, 4, -1), (1, 3, 1), (1, 4, -1))),
    (((0, 1, -1), (0, 2, 1), (1, 1, 1)), ((1, 3, -1), (1, 4, -1), (2, 4, -1)), ((0, 3, 1), (0, 4, -1), (1, 4, -1))),
    (((0, 1, -1), (1, 1, 1)), ((1, 4, 1), (2, 4, 1)), ((0, 3, 1), (0, 4, -1))),
    (((1, 0, 1), (1, 1, 1)), ((1, 0, 1), (2, 0, 1)), ((1, 0, 1), (1, 1, 1))),
    (((1, 0, 1),), ((0, 0, 1), (1, 0, -1)), ((0, 0, 1), (1, 0, 1))),
    (((0, 1, 1), (1, 0, 1)), ((0, 1, -1), (1, 0, 1), (2, 0, 1), (2, 1, -1)), ((0, 0, 1), (1, 1, -1))),
    (((0, 1, 1), (1, 1, -1)), ((1, 0, -1), (1, 1, 1), (1, 2, -1), (2, 0, -1)), ((1, 1, -1),)),
    (((0, 0, 1),), ((0, 3, 1),), ((0, 2, 1), (0, 3, 1), (1, 2, 1), (1, 3, 1))),
    (((1, 2, 1),), ((0, 2, -1), (0, 3, 1), (2, 2, -1), (2, 3, 1)), ((1, 3, 1),)),
    (((0, 0, 1), (1, 0, -1), (1, 2, 1)), ((0, 2, 1), (0, 3, -1), (2, 2, 1)), ((0, 2, 1), (1, 2, 1), (1, 3, 1))),
    (((0, 0, -1), (1, 0, 1)), ((0, 2, 1), (2, 2, 1)), ((1, 2, 1), (1, 3, 1))),
    (((0, 0, 1), (0, 1, 1), (0, 2, -1)), ((2, 1, -1),), ((0, 1, 1), (0, 2, 1))),
    (((0, 0, 1), (0, 1, 1)), ((0, 1, 1), (2, 1, 1)), ((0, 0, 1), (0, 1, 1))),
    (((0, 0, 1), (1, 0, -1)), ((0, 0, 1), (0, 1, -1), (0, 4, 1), (2, 1, -1)), ((0, 0, 1),)),
    (((0, 1, 1),), ((0, 1, -1), (1, 1, 1)), ((0, 1, 1), (1, 1, 1))),
    (((0, 2, 1),), ((1, 3, 1), (1, 4, 1), (2, 3, 1), (2, 4, 1)), ((0, 3, 1),)),
)
_ORD_Q = (6, 8, 7, 9, 13, 25, 21, 11, 23, 17, 16, 12, 18, 24, 22, 15, 4, 1, 5, 3, 20, 19, 10, 14, 0, 2)
_ORD_O = (4, 1, 19, 6, 15, 3, 14, 16, 20, 9, 22, 11, 8, 25, 23, 13, 24, 12, 10, 21, 17, 7, 18, 5, 0, 2)


def _plain(nk, nn):
    return tuple((((m, k, 1),), ((k, n, 1),), ((m, n, 1),))
                 for n in range(nn) for k in range(nk) for m in range(2))


class _Alg:
    def __init__(self, table, order=None, round=4, allf=0):
        self.round = round
        if order is not None:
            table = [table[r] for r in order]
        def norm(t):
            sg = t[0][2]
            return tuple((i, j, c * sg) for i, j, c in t), sg
        self.a_forms, self.b_forms, self.prods = [], [], []
        for a, b, c in table:
            (a, sa), (b, sb) = norm(a), norm(b)
            if a not in self.a_forms:
                self.a_forms.append(a)
            if b not in self.b_forms:
                self.b_forms.append(b)
            self.prods.append((a, b, tuple((i, j, v * sa * sb) for i, j, v in c)))
        self.a_multi = [f for f in self.a_forms if len(f) > 1 or allf & 1]
        self.b_multi = [f for f in self.b_forms if len(f) > 1 or allf & 2]


def _combine(form, get):
    r = get(form[0][0], form[0][1])
    for i, j, c in form[1:]:
        r = r + get(i, j) if c > 0 else r - get(i, j)
    return r


def _bilinear(alg, a_of, b_of, init=None):
    out = dict(init or {})

    def acc(d, key, v, sg):
        if key not in d:
            d[key] = (v, sg)
        else:
            w, sw = d[key]
            d[key] = (w + v if sg == sw else w - v, sw)

    for r0 in range(0, len(alg.prods), alg.round):
        groups = {}
        for a, b, c in alg.prods[r0:r0 + alg.round]:
            sg = c[0][2]
            m = jnp.dot(a_of(a), b_of(b), preferred_element_type=_F32)
            acc(groups, tuple((i, j, v * sg) for i, j, v in c), m, sg)
        part = {}
        for c, (tot, tsg) in groups.items():
            for i, j, v in c:
                acc(part, (i, j), tot, v * tsg)
        for key, (v, sg) in part.items():
            if key not in out:
                out[key] = v if sg > 0 else -v
            else:
                out[key] = out[key] + v if sg > 0 else out[key] - v
    return out


def _pack(v):
    return pltpu.bitcast(v, jnp.uint32)


def _unpack(v):
    return pltpu.bitcast(v, _BF16)


def _split(v):
    u = _pack(v)
    return tuple(pltpu.unpack_elementwise(u, index=i, packed_dtype=_BF16, unpacked_dtype=_F32)
                 for i in range(2))


def _form(f, get):
    halves = [_combine(f, lambda i, j: get(i, j)[h]) for h in range(2)]
    r = pltpu.pack_elementwise(halves, packed_dtype=_BF16)
    return r if r.dtype == jnp.uint32 else pltpu.bitcast(r, jnp.uint32)


def _nt(a, b):
    return jax.lax.dot_general(a, b, _NT, preferred_element_type=_F32)


def _lo(n):
    return jax.lax.broadcasted_iota(jnp.int32, (n, 128), 1) < 64


def _qfin(c):
    t0, t1, t2 = [jnp.concatenate([c[0, n], c[1, n]], axis=0) * _SCALE for n in range(3)]
    lo = _lo(t1.shape[0])
    zero = jnp.zeros_like(t1)
    q1 = jnp.concatenate([t0, jnp.where(lo, t1, zero)], axis=1).astype(_BF16)
    q2 = jnp.concatenate([jnp.where(lo, zero, t1), t2], axis=1).astype(_BF16)
    return q1, q2


def _qk(q1, q2, kt):
    s1 = jnp.dot(q1, kt[0:256], preferred_element_type=_F32)
    s2 = jnp.dot(q2, kt[128:384], preferred_element_type=_F32)
    return s1, s2


def _soft(s, ch, raw=False, sumb=False):
    if sumb:
        ps, rs = [], []
        for c in (s[0:128], s[128:]):
            m = jnp.max(c, axis=-1, keepdims=True)
            p = jnp.exp2(c - m).astype(_BF16)
            l = jnp.sum(p.astype(_F32), axis=-1, keepdims=True)
            r = pl.reciprocal(l, approx=True)
            rs.append(r if sumb & 16 else r * (2.0 - l * r))
            ps.append(p)
        return tuple(ps), rs
    m = jnp.max(s, axis=-1, keepdims=True)
    p = jnp.exp2(s - m)
    l = jnp.sum(p, axis=-1, keepdims=True)
    r = pl.reciprocal(l, approx=True)
    rs = [r * (2.0 - l * r)]
    if raw:
        return (p, None), rs
    return (p[0:128].astype(_BF16), p[128:].astype(_BF16)), rs


def _pv_top(p, vt_h):
    return _nt(vt_h, p[0])


def _pv_rem(p1, p2, vt):
    p1r, p2r = p1[1], p2[1]
    n = p1r.shape[0]
    ra = _nt(p1r, vt[0:128])
    rm = _nt(jnp.concatenate([p1r, p2r], axis=0), vt[128:256])
    rc = _nt(p2r, vt[256:384])
    return jnp.concatenate([ra, jnp.where(_lo(n), rm[0:n], rm[n:2 * n]), rc], axis=1)


def _pv_fin(ot1, ot2, o_r, r1, r2):
    o_top = jnp.concatenate([ot1, ot2], axis=0).T
    o = jnp.concatenate([o_top, o_r], axis=0)
    outs = []
    i0 = 0
    for a, b in zip(r1, r2):
        ch = a.shape[0]
        rr = jnp.concatenate([jnp.broadcast_to(a, (ch, 128)),
                              jnp.where(_lo(ch), a, b),
                              jnp.broadcast_to(b, (ch, 128))], axis=1)
        outs.append(o[i0:i0 + ch] * rr)
        i0 += ch
    return jnp.concatenate(outs, axis=0) if len(outs) > 1 else outs[0]


def _kernel(xa, ka, va, wqa, woa, xb, kb, vb, wqb, wob, out,
            x_res, wq_res, wo_res, acc, ostage, kv, s_scr, o_scr, xc, wqc, woc, p_scr, q_scr, f_scr, zero_ref,
            g_sem, w_sem, p_sem, o_sem, *, nb, n_pair, ring, sched, g_init, w_pos, late, order, order1, aq, ao, w1_at, ch, mat, noost, wstat, wmerge, gate, walign, pk, whalf):
    lg = nb.bit_length() - 1
    assert nb == 1 << lg
    n_pos = n_pair * nb
    sq, d = x_res.shape[2], x_res.shape[3]
    wqs, wos = (wqa, wqb), (woa, wob)

    def static(v):
        return isinstance(v, int)

    def bp(u):
        if static(u):
            return u & (nb - 1), u >> lg
        return u & (nb - 1), jax.lax.shift_right_logical(u, lg)

    def clamp(u, hi=n_pos - 1):
        return min(max(u, 0), hi) if static(u) else jnp.clip(u, 0, hi)

    def when(cond):
        if isinstance(cond, bool):
            return (lambda f: f()) if cond else (lambda f: None)
        return pl.when(cond)

    def pair_ds(p):
        return pl.ds(p * _PAIR if static(p) else pl.multiple_of(p * _PAIR, _PAIR), _PAIR)

    def chunk(ref, u):
        b, p = bp(u)
        return ref.at[b, pair_ds(p), :]

    n_last = sched[-1][0]
    u_last = n_pos - n_last * sched[-1][1]
    lg_last = n_last.bit_length() - 1
    n_par = ring // n_last
    merged = u_last >= nb and n_last > 1

    def sem_of(u):
        if not merged:
            return u & (ring - 1)
        if static(u):
            return u & (ring - 1) if u < u_last else ring + ((u >> lg_last) & (n_par - 1))
        big = ring + (jax.lax.shift_right_logical(u, lg_last) & (n_par - 1))
        if all_last[0]:
            return big
        return jnp.where(u < u_last, u & (ring - 1), big)

    def issue(u, h, enable=True):
        uc = clamp(u)
        slot = uc & (ring - 1)
        sem = g_sem.at[sem_of(uc)]

        def both(c):
            if isinstance(enable, bool):
                return c if enable else False
            return enable if c is True else jnp.logical_and(enable, c)

        if x_possible[0]:
            ux = clamp(u + h, nb - 1)

            @when(both(u + h < nb))
            def _():
                src, br = (xb, 1) if h == 0 else (xa, 0)
                pltpu.make_async_copy(src.at[ux], x_res.at[br, ux], sem).start()
        srcs = (chunk(va, uc), chunk(kb, uc)) if h == 0 else (chunk(vb, uc), chunk(ka, clamp(u + 1)))
        for i, s in enumerate(srcs):
            @when(both(u < n_pos))
            def _():
                pltpu.make_async_copy(s, kv.at[slot, 2 * h + i], sem).start()
        if x_possible[0] and h == 1:
            @when(both(u == w1_at))
            def _():
                w_start(1)

    def wq_copy(p, br, sem):
        return pltpu.make_async_copy(wqs[br].at[:, pair_ds(p)], wq_res.at[p, br], sem)

    def wo_copy(p, br, sem):
        return pltpu.make_async_copy(wos[br].at[pair_ds(p), :], wo_res.at[p, br], sem)

    def w_start(p):
        sem = w_sem.at[p & 1]
        for br in range(2):
            wq_copy(p, br, sem).start()
            wo_copy(p, br, sem).start()

    def w_wait(p):
        sem = w_sem.at[p & 1]
        pltpu.make_async_copy(wq_res.at[p], wq_res.at[p], sem).wait()
        pltpu.make_async_copy(wo_res.at[p], wo_res.at[p], sem).wait()

    def out_copy(b):
        return pltpu.make_async_copy(ostage.at[b], out.at[b], o_sem.at[b])

    hm = sq // 2
    wo_off = 0
    if wmerge:
        woc, wo_off = wqc, len(aq.b_multi)

    def tile(ref, i, j, rows):
        return ref[i * rows:(i + 1) * rows, j * 128:(j + 1) * 128]

    def qproj(br, b, p):
        x, w = x_res.at[br, b], wq_res.at[p, br]

        def a_of(f):
            if f not in aq.a_multi:
                return tile(x, f[0][0], f[0][1], hm)
            return _unpack(xc[br, b, aq.a_multi.index(f)])

        def b_of(f):
            if f not in aq.b_multi:
                return tile(w, f[0][0], f[0][1], 128)
            return _unpack(wqc[p & 1, br, aq.b_multi.index(f)])
        return _qfin(_bilinear(aq, a_of, b_of))

    def o_forms(o):
        return [_combine(f, lambda i, j: tile(o, i, j, hm)).astype(_BF16) for f in ao.a_forms]

    def oproj(forms, br, b, p, stage_out=True):
        w = wo_res.at[p, br]

        def b_of(f):
            if f not in ao.b_multi:
                return tile(w, f[0][0], f[0][1], 128)
            return _unpack(woc[p & 1, br, wo_off + ao.b_multi.index(f)])
        a = acc.at[br, b]
        init = {(i, j): tile(a, i, j, hm) for i in range(2) for j in range(d // 128)}
        c = _bilinear(ao, lambda f: forms[ao.a_forms.index(f)], b_of, init)
        for (i, j), v in c.items():
            a[i * hm:(i + 1) * hm, j * 128:(j + 1) * 128] = v
        if stage_out:
            for i in range(2):
                row = jnp.concatenate([c[i, j] for j in range(d // 128)], axis=1)
                ostage[b, i * hm:(i + 1) * hm, br * d:(br + 1) * d] = row.astype(ostage.dtype)

    def x_forms(br, b):
        x = x_res.at[br, b]
        blk = {}

        def get(i, j):
            if (i, j) not in blk:
                blk[i, j] = _split(tile(x, i, j, hm)) if pk == 0 else tile(x, i, j, hm).astype(_F32)
            return blk[i, j]
        for r, f in enumerate(aq.a_multi):
            if len(f) == 1:
                xc[br, b, r] = _pack(tile(x, f[0][0], f[0][1], hm))
            elif pk == 0:
                xc[br, b, r] = _form(f, get)
            elif pk == 1:
                xc[br, b, r] = _pack(_combine(f, get).astype(_BF16))
            else:
                xc.bitcast(_BF16)[br, b, r] = _combine(f, get).astype(_BF16)

    def w_forms(br, p, si, which=(0, 1), lo=0):
        for t in which:
            raw, dst, alg = ((wq_res, wqc, aq), (wo_res, woc, ao))[t]
            rows = raw.shape[2]
            ext = 16 * (lo + 1)
            if static(si):
                view = raw.at[p, br, pl.ds(si * 16, rows - 128 + ext)]
                off2 = (si + lo) * 8
            else:
                view = raw.at[p, br, pl.ds(pl.multiple_of(si * 16, 16), rows - 128 + ext)]
                off2 = pl.multiple_of((si + lo) * 8, 8)
            blk = {}

            def src(i, j):
                return view[i * 128 + lo * 16:i * 128 + lo * 16 + 16, j * 128:(j + 1) * 128]

            def get(i, j):
                if (i, j) not in blk:
                    blk[i, j] = _split(src(i, j)) if pk == 0 else src(i, j).astype(_F32)
                return blk[i, j]
            for r, f in enumerate(alg.b_multi):
                if len(f) == 1 or pk < 2:
                    dst[p & 1, br, r + t * wo_off, pl.ds(off2, 8), :] = (
                        _pack(src(f[0][0], f[0][1])) if len(f) == 1
                        else _form(f, get) if pk == 0
                        else _pack(_combine(f, get).astype(_BF16)))
                else:
                    off = off2 * 2 if static(off2) else pl.multiple_of(off2 * 2, 16)
                    dst.bitcast(_BF16)[p & 1, br, r + t * wo_off, pl.ds(off, 16), :] = (
                        _combine(f, get).astype(_BF16))

    def waits_for(u0, n, maybe_first):
        if merged and all_last[0]:
            slot = u0 & (ring - 1)
            blk = kv.at[pl.ds(slot if static(slot) else pl.multiple_of(slot, n), n)]
            pltpu.make_async_copy(blk, blk, g_sem.at[sem_of(u0)]).wait()
        for i in range(0 if merged and all_last[0] else n):
            u = u0 + i
            sem = g_sem.at[u & (ring - 1)]
            slot = u & (ring - 1)
            pltpu.make_async_copy(kv.at[slot], kv.at[slot], sem).wait()
            if maybe_first:
                for h in range(2):
                    @when(u + h < nb)
                    def _():
                        pltpu.make_async_copy(x_res.at[0, 0], x_res.at[0, 0], sem).wait()
        b0, p0 = bp(u0)
        bw = 0 if whalf and all_last[0] else nb // 2

        @when((b0 == bw and p0 + 1 < n_pair) if static(u0)
              else jnp.logical_and(b0 == bw, p0 + 1 < n_pair))
        def _():
            w_wait(p0 + 1)

    zero_ref[0] = 0
    x_possible = [True]
    all_last = [False]
    assert g_init < ring
    first = [pltpu.make_async_copy(xa.at[0], x_res.at[0, 0], p_sem.at[0]),
             wq_copy(0, 0, p_sem.at[0]),
             pltpu.make_async_copy(chunk(ka, 0), kv.at[ring - 1, 3], p_sem.at[0])]
    for c in first:
        c.start()
    second = [wq_copy(0, 1, p_sem.at[1]), wo_copy(0, 0, p_sem.at[1]), wo_copy(0, 1, p_sem.at[1])]

    def start_rest():
        second[0].start()
        second[1].start()
        for g in range(g_init):
            issue(g, 0)
            issue(g, 1)
            if g == 0:
                second[2].start()

    if not late:
        start_rest()

    def zero(b, carry):
        for br in range(2):
            acc[br, b] = jnp.zeros((sq, d), _F32)
        return carry
    jax.lax.fori_loop(0, nb, zero, 0)
    o_scr[...] = jnp.zeros(o_scr.shape, o_scr.dtype)

    for c in first:
        c.wait()
    if late:
        start_rest()

    def w0a(si, carry):
        w_forms(0, 0, si, (0,))
        return carry
    jax.lax.fori_loop(0, 8, w0a, 0)
    x_forms(0, 0)
    s1, s2 = _qk(*qproj(0, 0, 0), kv[ring - 1, 3])
    s_scr[0] = s1
    s_scr[1] = s2
    for c in second:
        c.wait()

    def w0b(si, carry):
        w_forms(0, 0, si, (1,))
        w_forms(1, 0, si)
        return carry
    jax.lax.fori_loop(0, 8, w0b, 0)

    def run_phase(u_start, n, cnt, g0, dbl):
        T = 2 * n
        maybe_first = u_start < nb
        maybe_last = u_start + n * cnt > n_pos - nb
        x_possible[0] = g0 < nb
        all_last[0] = u_start >= u_last

        def body(j, carry):
            u0 = u_start + j * n

            def task(k):
                if k == -1:
                    br, u = 1, clamp(u0 - 1)
                elif k == T:
                    br, u = 0, clamp(u0 + n)
                else:
                    br, u = k % 2, u0 + k // 2
                return (br,) + bp(u)

            def slot(k):
                return (u0 + k // 2) & (ring - 1)

            Q, S, P, O, OT, OR, G = {}, {}, {}, {}, {}, {}, {}
            S[0, 0] = s_scr[0]
            S[0, 1] = s_scr[1]
            O[-1] = [_unpack(o_scr[r]) for r in range(len(ao.a_forms))]

            def kref(k):
                return kv.at[slot(k - 1), 1 if k % 2 == 1 else 3]

            def vref(k):
                return kv.at[slot(k), 0 if k % 2 == 0 else 2]

            def do_q(k):
                Q[k, 0], Q[k, 1] = qproj(*task(k))
                if mat & 2:
                    for h in range(2):
                        q_scr[k % 2, h] = _pack(Q[k, h])
                        Q[k, h] = _unpack(q_scr[k % 2, h])

            def do_x(k):
                br, b, _ = task(k)
                x_forms(br, b)

            def do_w(k):
                br, b, p = task(k)
                half = nb // 2
                pc = jnp.minimum(p + jax.lax.shift_right_logical(b, lg - 1), n_pair - 1)
                bh = k // 2 if n == half and wstat is True else (b + (carry if wstat == 2 else 0)) & (half - 1)
                if gate:
                    v = G.pop(k)
                    bh = bh + (pltpu.bitcast(v[0:8, 0:128], jnp.int32)[0, 0] & carry)
                if whalf and n == half and not maybe_first:
                    pc = jnp.minimum(p + 1, n_pair - 1)
                    per = 16 // nb
                    hi = jax.lax.shift_right_logical(b, lg - 1) * 4
                    for i in range(per):
                        w_forms(br, pc, hi, ((k // 2) & 1,), lo=(k // 4) * per + i)
                    return
                if walign and n >= 4 and half == 8:
                    w_forms(br, pc, b & 4, lo=(k // 2) & 3)
                    return
                for i in range(8 // half):
                    w_forms(br, pc, bh * (8 // half) + i)

            def do_qk(k, h):
                S[k, h] = jnp.dot(Q.pop((k, h)), kref(k)[128 * h:128 * h + 256, :],
                                  preferred_element_type=_F32)
                if gate == 1 + h:
                    G[k - 1] = S[k, h]

            def do_sm(k, h):
                (pt, pr), r = _soft(S.pop((k, h)), ch, mat & 1, mat & 24)
                if mat & 1:
                    for c in range(4):
                        p_scr[k % 2, h, c] = _pack(pt[:, c * 128:(c + 1) * 128].astype(_BF16))
                    pt = jnp.concatenate([_unpack(p_scr[k % 2, h, c, 0:64]) for c in range(4)], axis=1)
                    pr = jnp.concatenate([_unpack(p_scr[k % 2, h, c, 64:sq // 2]) for c in range(4)], axis=1)
                P[k, h] = (pt, pr), r

            def do_pt(k, h):
                OT[k, h] = _pv_top(P[k, h][0], vref(k)[192 * h:192 * h + 192, :])
                if gate == 3 + h:
                    G[k] = OT[k, h]

            def do_pr(k):
                OR[k] = _pv_rem(P[k, 0][0], P[k, 1][0], vref(k)[...])

            def do_pf(k):
                O[k] = o_forms(_pv_fin(OT.pop((k, 0)), OT.pop((k, 1)), OR.pop(k),
                                       P.pop((k, 0))[1], P.pop((k, 1))[1]))
                if mat & 4 and k < T - 1:
                    for r, v in enumerate(O[k]):
                        f_scr[k % 2, r] = _pack(v)
                    O[k] = [_unpack(f_scr[k % 2, r]) for r in range(len(ao.a_forms))]

            def do_o(k):
                br, b, p = task(k)
                oproj(O.pop(k), br, b, p, maybe_last and not noost)
                if br == 1 and maybe_last:
                    last = (p == n_pair - 1) if k >= 0 else (u0 - 1 >= n_pos - nb)

                    @pl.when(last)
                    def _():
                        out_copy(b).start()

            def refill(k):
                i = j * n + k // 2
                h = k % 2
                if dbl:
                    fast = i < dbl // 2
                    g = g0 + i + jnp.minimum(i, dbl // 2)
                    if h == 0:
                        issue(g, 0)
                        issue(g, 1, fast)
                    else:
                        g = g + fast.astype(jnp.int32)
                        issue(g, 0, fast)
                        issue(g, 1)
                else:
                    issue(g0 + i, h)

            ops = {"q": lambda k: do_q(k + 1), "a": lambda k: do_qk(k + 1, 0),
                   "b": lambda k: do_qk(k + 1, 1), "s": lambda k: do_sm(k, 0),
                   "t": lambda k: do_sm(k, 1), "u": lambda k: do_pt(k, 0),
                   "v": lambda k: do_pt(k, 1), "r": do_pr, "f": do_pf,
                   "o": lambda k: do_o(k - 1), "d": refill,
                   "x": lambda k: do_x(k + 1), "w": do_w,
                   "Q": lambda k: do_q(k + 2), "X": lambda k: do_x(k + 2),
                   "B": lambda k: do_qk(k, 1), "R": lambda k: do_pr(k - 1),
                   "V": lambda k: do_pt(k - 1, 1), "F": lambda k: do_pf(k - 1)}
            od = order1 if maybe_first else order
            for k in range(T):
                of, om, ol = (od.split("/") * 3)[:3] if "/" not in od else od.split("/")
                for c in (ol if k == T - 1 else of if k == 0 else om):
                    ops[c](k)
            b0, p0 = bp(u0)

            wp = w_pos if all_last[0] else (3 * nb) // 4

            @pl.when(jnp.logical_and(b0 == (wp // n) * n, p0 + 2 < n_pair))
            def _():
                w_start(p0 + 2)
            s_scr[0] = S.pop((T, 0))
            s_scr[1] = S.pop((T, 1))
            for r, v in enumerate(O.pop(T - 1)):
                o_scr[r] = _pack(v)

            @pl.when(j + 1 < cnt)
            def _():
                waits_for(u0 + n, n, maybe_first)
            return carry

        waits_for(u_start, n, maybe_first)
        jax.lax.fori_loop(0, cnt, body, zero_ref[0])

    issued = {(g, h): -1 for g in range(g_init) for h in range(2)}
    u_start, g0 = 0, g_init
    plan = []
    for n, cnt, dbl in sched:
        assert dbl % 2 == 0 and nb % n == 0 and u_start % n == 0
        plan.append((u_start, n, cnt, g0, dbl))
        for t in range(2 * n * cnt):
            i, h, tg = t // 2, t % 2, 2 * u_start + t
            if i < dbl // 2:
                gs = [(g0 + 2 * i + h, 0), (g0 + 2 * i + h, 1)]
            else:
                gs = [(g0 + i + dbl // 2, h)]
            for g, hh in gs:
                assert (g, hh) not in issued
                issued[(g, hh)] = tg
                assert 2 * (g - ring) + hh + 1 < tg
            if t % (2 * n) == 0:
                for u in range(u_start + i, u_start + i + n):
                    assert issued[(u, 0)] < tg and issued[(u, 1)] < tg
        g0 += n * cnt + dbl // 2
        u_start += n * cnt
    assert u_start == n_pos
    assert not whalf or (u_last % nb == 0 and n_last == nb // 2 and w_pos < nb // 2)
    for u_start, n, cnt, g0, dbl in plan:
        assert w_pos < nb
        run_phase(u_start, n, cnt, g0, dbl)

    oproj([_unpack(o_scr[r]) for r in range(len(ao.a_forms))], 1, nb - 1, n_pair - 1)
    out_copy(nb - 1).start()
    for b in range(nb):
        out_copy(b).wait()


def _build(A_x, A_k_cache, A_v_cache, A_wq, A_wo,
           B_x, B_k_cache, B_v_cache, B_wq, B_wo, *,
           sched=((1, 32, 16), (8, 28, 0)), g_init=1, w_pos=12, late=False,
           order='stqdwouvrfab/dstqwouvrfab/dstqwouvrfab',
           order1='stxouqdvrfabw/dstxouqvrfabw/dstxouqvrfabw', fq=True, fo=True, w1_at=7, rnd=4, ch=160, mat=24, noost=False, allf=3, wstat=False, wmerge=False, gate=0, walign=True, pk=1, whalf=False, nobc=True, ring=16, interpret=False):
    nb, sq, d = A_x.shape
    n_head, sk = A_k_cache.shape[1], A_k_cache.shape[2]
    n_pair = n_head // 2

    def tr(c):
        return jnp.swapaxes(c, 2, 3).reshape(nb, n_head * _DH, sk)

    any_spec = pl.BlockSpec(memory_space=pl.ANY)
    aq = (_Alg(_ALG25_Q, None, rnd, allf) if fq == 25 else
          _Alg(_ALG_Q, _ORD_Q, rnd, allf) if fq else _Alg(_plain(5, 3), None, rnd, allf))
    ao = (_Alg(_ALG25_O, None, rnd, allf) if fo == 25 else
          _Alg(_ALG_O, _ORD_O, rnd, allf) if fo else _Alg(_plain(3, 5), None, rnd, allf))
    up4 = lambda v: -(-v // 4) * 4
    opad = up4(len(ao.a_forms))
    return pl.pallas_call(
        functools.partial(_kernel, nb=nb, n_pair=n_pair, ring=ring, sched=sched,
                          g_init=g_init, w_pos=w_pos, late=late, order=order,
                          order1=order1, aq=aq, ao=ao, w1_at=w1_at, ch=ch, mat=mat, noost=noost, wstat=wstat, wmerge=wmerge, gate=gate, walign=walign, pk=pk, whalf=whalf),
        in_specs=[any_spec] * 10,
        out_specs=any_spec,
        out_shape=jax.ShapeDtypeStruct((nb, sq, 2 * d), A_x.dtype),
        scratch_shapes=[
            pltpu.VMEM((2, nb, sq, d), _BF16),
            pltpu.VMEM((n_pair, 2, d, _PAIR), _BF16),
            pltpu.VMEM((n_pair, 2, _PAIR, d), _BF16),
            pltpu.VMEM((2, nb, sq, d), _F32),
            pltpu.VMEM((nb, sq, 2 * d), _BF16),
            pltpu.VMEM((ring, 4, _PAIR, sk), _BF16),
            pltpu.VMEM((2, sq, sk), _F32),
            pltpu.VMEM((opad, sq // 4, 128), jnp.uint32),
            pltpu.VMEM((2, nb, up4(max(len(aq.a_multi), 1)), sq // 4, 128), jnp.uint32),
            pltpu.VMEM((2, 2, max(len(aq.b_multi), 1) + (len(ao.b_multi) if wmerge else 0), 64, 128),
                       jnp.uint32),
            pltpu.VMEM((2, 2, 1 if wmerge else max(len(ao.b_multi), 1), 64, 128), jnp.uint32),
            pltpu.VMEM((2, 2, 4, sq // 2, 128), jnp.uint32),
            pltpu.VMEM((2, 2, sq // 2, 256), jnp.uint32),
            pltpu.VMEM((2, len(ao.a_forms), sq // 4, 128), jnp.uint32),
            pltpu.SMEM((1,), jnp.int32),
            pltpu.SemaphoreType.DMA((2 * ring,)),
            pltpu.SemaphoreType.DMA((2,)),
            pltpu.SemaphoreType.DMA((2,)),
            pltpu.SemaphoreType.DMA((nb,)),
        ],
        compiler_params=pltpu.CompilerParams(
            vmem_limit_bytes=120 * 1024 * 1024,
            disable_bounds_checks=nobc),
        interpret=interpret,
    )(A_x, tr(A_k_cache), tr(A_v_cache), A_wq, A_wo,
      B_x, tr(B_k_cache), tr(B_v_cache), B_wq, B_wo)


@jax.jit
def pallas_concat_heads__gqa_block_cached__mha_block_cached__near_ridge_kernel(
    A_x: jax.Array,
    A_k_cache: jax.Array,
    A_v_cache: jax.Array,
    A_wq: jax.Array,
    A_wo: jax.Array,
    B_x: jax.Array,
    B_k_cache: jax.Array,
    B_v_cache: jax.Array,
    B_wq: jax.Array,
    B_wo: jax.Array,
):
    return _build(A_x, A_k_cache, A_v_cache, A_wq, A_wo,
                  B_x, B_k_cache, B_v_cache, B_wq, B_wo)
```

```python
import functools
import math

import jax
import jax.numpy as jnp
import jax.experimental.pallas as pl
import jax.experimental.pallas.tpu as pltpu

_DH = 192
_PAIR = 2 * _DH
_NT = (((1,), (1,)), ((), ()))
_F32 = jnp.float32
_BF16 = jnp.bfloat16
_SCALE = (_DH ** -0.5) * math.log2(math.e)

_ALG_Q = (
    (((0, 0, 1),), ((0, 0, 1),), ((0, 0, 1),)),
    (((1, 0, 1),), ((0, 0, 1),), ((1, 0, 1),)),
    (((0, 1, 1),), ((1, 0, 1),), ((0, 0, 1),)),
    (((1, 1, 1),), ((1, 0, 1),), ((1, 0, 1),)),
    (((0, 2, 1), (1, 2, -1)), ((2, 0, 1), (2, 1, -1), (2, 2, -1)), ((0, 0, 1),)),
    (((1, 2, 1),), ((2, 0, 1), (3, 0, 1), (4, 0, 1)), ((0, 0, 1), (1, 0, 1))),
    (((0, 0, 1), (1, 0, -1)), ((0, 1, 1), (0, 2, 1)), ((0, 1, 1),)),
    (((1, 0, 1),), ((0, 1, 1), (4, 1, -1)), ((0, 1, 1), (1, 1, 1))),
    (((0, 3, -1), (1, 3, 1)), ((3, 0, -1), (3, 1, 1), (3, 2, 1)), ((1, 1, 1),)),
    (((0, 3, 1),), ((1, 1, 1), (2, 1, 1), (3, 1, 1)), ((0, 1, 1), (1, 1, 1))),
    (((0, 1, 1), (1, 1, -1)), ((1, 1, 1), (1, 2, 1)), ((0, 2, 1),)),
    (((1, 1, 1),), ((1, 2, 1), (3, 2, 1)), ((0, 2, 1), (1, 2, 1))),
    (((0, 4, -1), (1, 4, 1)), ((4, 0, -1), (4, 1, 1), (4, 2, 1)), ((1, 2, 1),)),
    (((0, 4, 1),), ((0, 2, -1), (2, 2, 1), (4, 2, 1)), ((0, 2, 1), (1, 2, 1))),
    (((0, 3, -1), (1, 2, 1)), ((2, 1, -1), (3, 0, -1)), ((0, 0, 1), (1, 1, -1))),
    (((1, 2, 1), (1, 3, -1)), ((3, 0, 1),), ((1, 0, -1), (1, 1, -1))),
    (((0, 2, 1), (0, 3, -1)), ((2, 1, 1),), ((0, 0, 1), (0, 1, 1))),
    (((0, 4, -1), (1, 2, 1)), ((2, 2, -1), (4, 0, -1)), ((0, 0, 1), (1, 2, -1))),
    (((1, 2, 1), (1, 4, -1)), ((4, 0, 1),), ((1, 0, -1), (1, 2, -1))),
    (((0, 2, 1), (0, 4, -1)), ((2, 2, 1),), ((0, 0, 1), (0, 2, 1))),
    (((0, 3, 1), (1, 1, -1)), ((1, 1, -1), (3, 2, 1)), ((0, 2, 1), (1, 1, 1))),
    (((0, 1, -1), (0, 3, 1)), ((1, 1, 1),), ((0, 1, -1), (0, 2, 1))),
    (((1, 1, -1), (1, 3, 1)), ((3, 2, 1),), ((1, 1, -1), (1, 2, 1))),
    (((0, 4, 1), (1, 0, 1)), ((0, 2, 1), (4, 1, 1)), ((0, 1, 1), (1, 2, 1))),
    (((1, 0, 1), (1, 4, 1)), ((4, 1, 1),), ((1, 1, 1), (1, 2, -1))),
    (((0, 0, 1), (0, 4, 1)), ((0, 2, 1),), ((0, 1, -1), (0, 2, 1))),
)
_ALG_O = (
    (((0, 0, 1),), ((0, 0, 1),), ((0, 0, 1),)),
    (((1, 0, 1),), ((0, 0, 1),), ((1, 0, 1),)),
    (((0, 1, 1), (1, 1, -1)), ((1, 0, 1), (1, 4, -1)), ((0, 0, 1),)),
    (((1, 1, 1),), ((1, 0, 1), (2, 0, 1)), ((0, 0, 1), (1, 0, 1))),
    (((0, 0, 1),), ((0, 1, 1),), ((0, 1, 1),)),
    (((1, 0, 1),), ((0, 1, 1),), ((1, 1, 1),)),
    (((0, 2, 1), (1, 2, -1)), ((2, 1, 1), (2, 3, -1)), ((0, 1, 1),)),
    (((1, 2, 1),), ((1, 1, 1), (2, 1, 1)), ((0, 1, 1), (1, 1, 1))),
    (((0, 0, 1), (1, 0, -1)), ((0, 2, 1), (0, 3, -1), (0, 4, -1)), ((0, 2, 1),)),
    (((1, 0, 1),), ((0, 2, 1), (1, 2, 1), (2, 2, 1)), ((0, 2, 1), (1, 2, 1))),
    (((0, 1, -1), (1, 1, 1)), ((1, 1, -1), (1, 2, -1), (1, 3, 1)), ((1, 3, 1),)),
    (((0, 1, 1),), ((0, 3, 1), (1, 3, 1), (2, 3, 1)), ((0, 3, 1), (1, 3, 1))),
    (((0, 2, -1), (1, 2, 1)), ((2, 0, -1), (2, 2, -1), (2, 4, 1)), ((1, 4, 1),)),
    (((0, 2, 1),), ((0, 4, 1), (1, 4, 1), (2, 4, 1)), ((0, 4, 1), (1, 4, 1))),
    (((0, 2, -1), (1, 1, 1)), ((1, 4, -1), (2, 0, -1)), ((0, 0, 1), (1, 4, -1))),
    (((1, 1, 1), (1, 2, -1)), ((2, 0, 1),), ((1, 0, -1), (1, 4, -1))),
    (((0, 1, 1), (0, 2, -1)), ((1, 4, 1),), ((0, 0, 1), (0, 4, 1))),
    (((0, 1, -1), (1, 2, 1)), ((1, 1, -1), (2, 3, -1)), ((0, 1, 1), (1, 3, -1))),
    (((1, 1, -1), (1, 2, 1)), ((1, 1, 1),), ((1, 1, -1), (1, 3, -1))),
    (((0, 1, -1), (0, 2, 1)), ((2, 3, 1),), ((0, 1, 1), (0, 3, 1))),
    (((0, 1, -1), (1, 0, 1)), ((0, 3, -1), (1, 2, -1)), ((0, 2, 1), (1, 3, -1))),
    (((1, 0, 1), (1, 1, -1)), ((1, 2, 1),), ((1, 2, -1), (1, 3, -1))),
    (((0, 0, 1), (0, 1, -1)), ((0, 3, 1),), ((0, 2, 1), (0, 3, 1))),
    (((0, 2, -1), (1, 0, 1)), ((0, 4, -1), (2, 2, -1)), ((0, 2, 1), (1, 4, -1))),
    (((1, 0, 1), (1, 2, -1)), ((2, 2, 1),), ((1, 2, -1), (1, 4, -1))),
    (((0, 0, 1), (0, 2, -1)), ((0, 4, 1),), ((0, 2, 1), (0, 4, 1))),
)


_ORD_Q = (6, 8, 7, 9, 13, 25, 21, 11, 23, 17, 16, 12, 18, 24, 22, 15, 4, 1, 5, 3, 20, 19, 10, 14, 0, 2)
_ORD_O = (4, 1, 19, 6, 15, 3, 14, 16, 20, 9, 22, 11, 8, 25, 23, 13, 24, 12, 10, 21, 17, 7, 18, 5, 0, 2)


class _Alg:
    def __init__(self, table, order, split):
        def norm(t):
            sg = t[0][2]
            return tuple((i, j, c * sg) for i, j, c in t), sg
        self.split = split
        self.a_forms, self.b_forms, self.prods = [], [], []
        for r in order:
            a, b, c = table[r]
            (a, sa), (b, sb) = norm(a), norm(b)
            if a not in self.a_forms:
                self.a_forms.append(a)
            if b not in self.b_forms:
                self.b_forms.append(b)
            self.prods.append((a, b, tuple((i, j, v * sa * sb) for i, j, v in c)))


def _dot(a, b):
    return jnp.dot(a, b, preferred_element_type=_F32)


def _nt(a, b):
    return jax.lax.dot_general(a, b, _NT, preferred_element_type=_F32)


def _combine(form, get):
    r = get(form[0][0], form[0][1])
    for i, j, c in form[1:]:
        r = r + get(i, j) if c > 0 else r - get(i, j)
    return r


def _signed_add(d, key, v, sg):
    if key not in d:
        d[key] = (v, sg)
    else:
        w, sw = d[key]
        d[key] = (w + v if sg == sw else w - v, sw)


def _round(prods, out):
    groups, part = {}, {}
    for m, c in prods:
        sg = c[0][2]
        _signed_add(groups, tuple((i, j, v * sg) for i, j, v in c), m, sg)
    for c, (tot, tsg) in groups.items():
        for i, j, v in c:
            _signed_add(part, (i, j), tot, v * tsg)
    for key, (v, sg) in part.items():
        if key not in out:
            out[key] = v if sg > 0 else -v
        else:
            out[key] = out[key] + v if sg > 0 else out[key] - v


def _bilinear(alg, a_of, b_of, init=None):
    out = dict(init or {})
    for r0 in range(0, len(alg.prods), 4):
        prods = []
        for a, b, c in alg.prods[r0:r0 + 4]:
            av, bv = a_of(a), b_of(b)
            if alg.split and len(alg.prods) - r0 == 2:
                m = jnp.concatenate([_dot(av[0:alg.split], bv), _dot(av[alg.split:], bv)], axis=0)
            else:
                m = _dot(av, bv)
            prods.append((m, c))
        _round(prods, out)
    return out


def _pack(v):
    return pltpu.bitcast(v, jnp.uint32)


def _unpack(v):
    return pltpu.bitcast(v, _BF16)


def _lo(n):
    return jax.lax.broadcasted_iota(jnp.int32, (n, 128), 1) < 64


def _q_forms(c):
    a, b = [[c[m, n] * _SCALE for n in range(3)] for m in range(2)]
    lo = _lo(a[0].shape[0])
    rolled = pltpu.roll(b[1], 64, 1)
    forms = []
    for t, own in ((0, lo), (2, jnp.logical_not(lo))):
        t3 = jnp.where(own, a[t], b[t]).astype(_BF16)
        t3f = t3.astype(_F32)
        forms.append((t3,
                      jnp.where(own, a[1], a[t] - t3f).astype(_BF16),
                      jnp.where(own, b[t] - t3f, rolled).astype(_BF16)))
    return forms


def _scores(af, kt, h):
    if h == 0:
        w3, w1, w2 = kt[0:128], (kt[128:192], kt[64:128]), (kt[0:64], kt[128:192])
    else:
        w3, w1, w2 = kt[256:384], (kt[256:320], kt[192:256]), (kt[192:256], kt[320:384])
    t3 = _dot(af[0], w3)
    t1 = _dot(af[1], jnp.concatenate(w1, axis=0))
    t2 = _dot(af[2], jnp.concatenate(w2, axis=0))
    return t1 + t3, t2 + t3


def _softmax(s, mode=0):
    ps, us, rs = [], [], []
    for c in s:
        m = jnp.max(c, axis=-1, keepdims=True)
        e = jnp.exp2(c - m)
        p = e.astype(_BF16)
        u = p.astype(_F32)
        rs.append(pl.reciprocal(jnp.sum(e if mode == 2 else u, axis=-1, keepdims=True), approx=True))
        ps.append(p)
        us.append(u if mode == 0 else e)
    return (ps[0], ps[1], (us[0] + us[1]).astype(_BF16)), rs


def _pv(p, vt, h, i):
    lo, hi, e = ((0, 64, 128), (256, 320, 192))[h]
    rows = (((e, hi), (lo, e), (lo, hi)), ((lo, e), (e, hi), (lo, hi)))[h][i]
    if rows == (lo, hi):
        w = vt[lo:lo + 128]
    else:
        w = jnp.concatenate([vt[r:r + 64] for r in rows], axis=0)
    return _nt(p[i], w)


def _pv_finish(t0, t1, r0, r1):
    lo = _lo(t0[0].shape[0])
    d0 = jnp.where(lo, t0[1], t0[0])
    e0 = t0[2] - d0
    d1 = jnp.where(lo, t1[0], t1[1])
    e1 = t1[2] - d1
    return {(0, 0): jnp.where(lo, e0, d0) * r0[0],
            (1, 0): jnp.where(lo, d0, e0) * r0[1],
            (0, 1): jnp.where(lo, t0[0], t1[0]) * jnp.where(lo, r0[0], r1[0]),
            (1, 1): pltpu.roll(jnp.where(lo, t1[1], t0[1]), 64, 1) * jnp.where(lo, r0[1], r1[1]),
            (0, 2): jnp.where(lo, d1, e1) * r1[0],
            (1, 2): jnp.where(lo, e1, d1) * r1[1]}


def _kernel(xa, ka, va, wqa, woa, xb, kb, vb, wqb, wob, out,
            x_res, wq_res, wo_res, acc, ostage, kv, s_scr, o_scr, xc, wqc, woc,
            g_sem, w_sem, p_sem, o_sem, *, nb, n_pair, ring, n_main, u_main, dbl, w1_at,
            aq, ao, orders, only, pv_order, smode):
    lg = nb.bit_length() - 1
    half = nb // 2
    n_pos = n_pair * nb
    sq, d = acc.shape[2], acc.shape[3]
    hm = sq // 2
    wqs, wos = (wqa, wqb), (woa, wob)
    lg_main = n_main.bit_length() - 1
    assert nb == 1 << lg and n_main == 1 << lg_main and half % n_main == 0
    assert u_main >= nb and u_main % n_main == 0 and 8 % half == 0

    def static(v):
        return isinstance(v, int)

    def shr(v, s):
        return v >> s if static(v) else jax.lax.shift_right_logical(v, s)

    def aligned(v, m):
        return v if static(v) else pl.multiple_of(v, m)

    def clamp(u, hi=n_pos - 1):
        return min(max(u, 0), hi) if static(u) else jnp.clip(u, 0, hi)

    def when(*conds):
        dyn = [c for c in conds if not isinstance(c, bool)]
        if not all(c for c in conds if isinstance(c, bool)):
            return lambda f: None
        if not dyn:
            return lambda f: f()
        return pl.when(functools.reduce(jnp.logical_and, dyn))

    def pair_ds(p):
        return pl.ds(aligned(p * _PAIR, _PAIR), _PAIR)

    def chunk(ref, u):
        return ref.at[u & (nb - 1), pair_ds(shr(u, lg)), :]

    def sem_of(u, early):
        late = ring + (shr(u, lg_main) & (ring // n_main - 1))
        if static(u):
            return u & (ring - 1) if u < u_main else late
        return jnp.where(u < u_main, u & (ring - 1), late) if early else late

    def x_copy(br, b, sem):
        return pltpu.make_async_copy((xa, xb)[br].at[b], x_res.at[br, b, 0:sq], sem)

    def issue(u, h, early, may_end, enable=True):
        uc = clamp(u) if may_end else u
        un = clamp(u + 1) if may_end else u + 1
        sem = g_sem.at[sem_of(uc, early)]
        if early:
            ux = clamp(u + h, nb - 1)

            @when(enable, u + h < nb)
            def _():
                x_copy(1 - h, ux, sem).start()
        srcs = (chunk(va, uc), chunk(kb, uc)) if h == 0 else (chunk(vb, uc), chunk(ka, un))
        for i, s in enumerate(srcs):
            @when(enable, (u < n_pos) if may_end else True)
            def _():
                pltpu.make_async_copy(s, kv.at[uc & (ring - 1), 2 * h + i], sem).start()
        if early and h == 1:
            @when(enable, u == w1_at)
            def _():
                w_start(1)

    def wq_copy(p, br, sem):
        return pltpu.make_async_copy(wqs[br].at[:, pair_ds(p)], wq_res.at[p, br], sem)

    def wo_copy(p, br, sem):
        return pltpu.make_async_copy(wos[br].at[pair_ds(p), :], wo_res.at[p, br], sem)

    def w_start(p):
        for br in range(2):
            wq_copy(p, br, w_sem.at[p & 1]).start()
            wo_copy(p, br, w_sem.at[p & 1]).start()

    def waits_for(u0, n, early):
        blk = kv.at[pl.ds(aligned(u0 & (ring - 1), n), n)]
        sem = g_sem.at[u0 & (ring - 1) if early else sem_of(u0, False)]
        pltpu.make_async_copy(blk, blk, sem).wait()
        if early:
            for h in range(2):
                @when(u0 + h < nb)
                def _():
                    x_copy(0, 0, sem).wait()
        p1 = shr(u0, lg) + 1

        @when((u0 & (nb - 1)) == half, p1 < n_pair)
        def _():
            for ref in (wq_res, wo_res):
                pltpu.make_async_copy(ref.at[p1], ref.at[p1], w_sem.at[p1 & 1]).wait()

    def tile(ref, i, j, rows):
        return ref[i * rows:(i + 1) * rows, j * 128:(j + 1) * 128]

    def qproj(br, b, p):
        c = _bilinear(aq, lambda f: _unpack(xc[br, b, aq.a_forms.index(f)]),
                      lambda f: _unpack(wqc[p & 1, br, aq.b_forms.index(f)]))
        return _q_forms(c)

    def o_forms(o):
        return [_combine(f, lambda i, j: o[i, j]).astype(_BF16) for f in ao.a_forms]

    def oproj(forms, br, b, p, keep, emit):
        a = acc.at[br, b]
        init = {(i, j): tile(a, i, j, hm) for i in range(2) for j in range(d // 128)}
        c = _bilinear(ao, lambda f: forms[ao.a_forms.index(f)],
                      lambda f: _unpack(woc[p & 1, br, ao.b_forms.index(f)]), init)
        if keep:
            for (i, j), v in c.items():
                a[i * hm:(i + 1) * hm, j * 128:(j + 1) * 128] = v
        if emit is not False:
            for i in range(2):
                row = jnp.concatenate([c[i, j] for j in range(d // 128)], axis=1)
                ostage[b, i * hm:(i + 1) * hm, br * d:(br + 1) * d] = row.astype(ostage.dtype)
            if br == 1:
                @when(emit)
                def _():
                    pltpu.make_async_copy(ostage.at[b], out.at[b], o_sem.at[0]).start()

    def store_forms(forms, src, put):
        blk = {}

        def get(i, j):
            if (i, j) not in blk:
                blk[i, j] = src(i, j).astype(_F32)
            return blk[i, j]
        for r, f in enumerate(forms):
            put(r, _pack(src(f[0][0], f[0][1]) if len(f) == 1
                         else _combine(f, get).astype(_BF16)))

    def x_forms(br, b):
        def put(r, v):
            xc[br, b, r] = v
        store_forms(aq.a_forms, lambda i, j: tile(x_res.at[br, b], i, j, hm), put)

    def w_forms(br, p, si, lo=0, which=(0, 1)):
        for t in which:
            raw, dst, alg = ((wq_res, wqc, aq), (wo_res, woc, ao))[t]
            view = raw.at[p, br, pl.ds(aligned(si * 16, 16), raw.shape[2] - 112 + 16 * lo)]
            rows = pl.ds(aligned((si + lo) * 8, 8), 8)

            def put(r, v):
                dst[p & 1, br, r, rows, :] = v
            store_forms(alg.b_forms, lambda i, j: view[i * 128 + lo * 16:i * 128 + lo * 16 + 16,
                                                       j * 128:(j + 1) * 128], put)

    def block(u0, n, kind, order, refill, emit_prev=False):
        T = 2 * n
        last = kind in ('last', 'end')

        def task(k):
            u = u0 + k // 2
            if k == -1 and kind == 'ramp':
                u = clamp(u)
            return k % 2, u & (nb - 1), shr(u, lg)

        def kv_ref(k, i):
            return kv.at[(u0 + k // 2) & (ring - 1), 2 * (k % 2) + i]

        Q, S, P, O, OT, OR = {}, {}, {}, {}, {}, {}
        for h in range(2):
            S[0, h] = (s_scr[h, 0], s_scr[h, 1])
        O[-1] = o_forms({(i, j): o_scr[i, j] for i in range(2) for j in range(3)})

        def do_q(k):
            Q[k, 0], Q[k, 1] = qproj(*task(k))

        def do_qk(k, h):
            S[k, h] = _scores(Q.pop((k, h)), kv_ref(k - 1, 1), h)

        def do_sm(k, h):
            P[k, h] = _softmax(S.pop((k, h)), smode)

        def do_pv(k, h, passes=(0, 1, 2)):
            for i in passes:
                OT[k, h, i] = _pv(P[k, h][0], kv_ref(k, 0), h, i)

        def do_pf(k):
            t0, t1 = [[OT.pop((k, h, i)) for i in range(3)] for h in range(2)]
            o = _pv_finish(t0, t1, P.pop((k, 0))[1], P.pop((k, 1))[1])
            if k == T - 1 and kind != 'end':
                for (i, j), v in o.items():
                    o_scr[i, j] = v
            else:
                O[k] = o_forms(o)

        def do_o(k):
            if k == -1:
                oproj(O.pop(k), *task(k), emit_prev is not True, emit_prev if last else False)
            else:
                oproj(O.pop(k), *task(k), not last, last)

        def do_w(k):
            br, b, p = task(k)
            pc = jnp.minimum(p + shr(b, lg - 1), n_pair - 1)
            per = 8 // half
            if n >= 4:
                w_forms(br, pc, b & 4, (k // 2) & 3)
            else:
                for i in range(per):
                    w_forms(br, pc, (b & (half - 1)) * per + i)

        def do_x(k):
            x_forms(*task(k)[:2])

        ops = {"q": lambda k: do_q(k + 1), "a": lambda k: do_qk(k + 1, 0),
               "b": lambda k: do_qk(k + 1, 1), "s": lambda k: do_sm(k, 0),
               "t": lambda k: do_sm(k, 1), "u": lambda k: do_pv(k, 0, pv_order),
               "v": lambda k: do_pv(k, 1, pv_order), "r": lambda k: None, "f": do_pf,
               "o": lambda k: do_o(k - 1), "d": refill, "x": lambda k: do_x(k + 1), "w": do_w}
        first, mid, final = order.split("/")
        for k in range(T):
            for c in (final if k == T - 1 else first if k == 0 else mid):
                ops[c](k)
        if kind == 'end':
            do_o(T - 1)
        else:
            for h in range(2):
                s_scr[h, 0], s_scr[h, 1] = S.pop((T, h))
        if not last:
            p2 = shr(u0, lg) + 2

            @when((u0 & (nb - 1)) == (3 * nb // 4 // n) * n, p2 < n_pair)
            def _():
                w_start(p2)

    first = [x_copy(0, 0, p_sem.at[0]), wq_copy(0, 0, p_sem.at[0]),
             pltpu.make_async_copy(chunk(ka, 0), kv.at[ring - 1, 3], p_sem.at[0])]
    second = [wq_copy(0, 1, p_sem.at[1]), wo_copy(0, 0, p_sem.at[1]), wo_copy(0, 1, p_sem.at[1])]
    for c in first + second[:2]:
        c.start()
    issue(0, 0, True, False)
    issue(0, 1, True, False)
    second[2].start()

    def zero(b, carry):
        for br in range(2):
            acc[br, b] = jnp.zeros((sq, d), _F32)
        return carry
    jax.lax.fori_loop(0, nb, zero, 0)
    o_scr[...] = jnp.zeros(o_scr.shape, o_scr.dtype)
    for c in first:
        c.wait()

    def w0a(si, carry):
        w_forms(0, 0, si, which=(0,))
        return carry
    jax.lax.fori_loop(0, 8, w0a, 0)
    x_forms(0, 0)
    for h, af in enumerate(qproj(0, 0, 0)):
        s_scr[h, 0], s_scr[h, 1] = _scores(af, kv.at[ring - 1, 3], h)
    for c in second:
        c.wait()

    def w0b(si, carry):
        w_forms(0, 0, si, which=(1,))
        w_forms(1, 0, si)
        return carry
    jax.lax.fori_loop(0, 8, w0b, 0)

    lead = 1 + dbl // 2
    assert dbl % 2 == 0 and dbl // 2 <= u_main and n_main < lead < ring and w1_at < half

    def ramp(u, carry):
        fast = u < dbl // 2
        g = u + 1 + jnp.minimum(u, dbl // 2)

        def refill(k):
            if k == 0:
                issue(g, 0, True, False)
                issue(g, 1, True, False, fast)
            else:
                g1 = g + fast.astype(jnp.int32)
                issue(g1, 0, True, False, fast)
                issue(g1, 1, True, False)
        block(u, 1, 'ramp', orders[0], refill)

        @pl.when(u + 1 < u_main)
        def _():
            waits_for(u + 1, 1, True)
        return carry

    waits_for(0, 1, True)
    if only in (None, 0):
        jax.lax.fori_loop(0, u_main, ramp, 0)

    def steady(u_start, cnt, kind, order):
        may_end = u_start + cnt * n_main + lead + 1 > n_pos

        def body(j, carry):
            u0 = u_start + j * n_main
            block(u0, n_main, kind, order,
                  lambda k: issue(u0 + k // 2 + lead, k % 2, False, may_end),
                  emit_prev=(j > 0) if kind == 'last' else False)
            waits_for(u0 + n_main, n_main, False)
            return carry
        if cnt:
            jax.lax.fori_loop(0, cnt, body, 0)

    u_last = n_pos - nb
    waits_for(u_main, n_main, False)
    if only in (None, 1):
        steady(u_main, (u_last - u_main) // n_main, 'main', orders[1])
    if only in (None, 2):
        steady(u_last, nb // n_main - 1, 'last', orders[2])
    if only in (None, 3):
        block(n_pos - n_main, n_main, 'end', orders[3], lambda k: None, emit_prev=True)
    pltpu.make_async_copy(ostage, out, o_sem.at[0]).wait()


def _build(A_x, A_k_cache, A_v_cache, A_wq, A_wo, B_x, B_k_cache, B_v_cache, B_wq, B_wo, *,
           n_main=4, u_main=24, dbl=10, w1_at=7, ring=16, split=(0, 0),
           algq=None, algo=None,
           o_ramp="stxqdwouvfab/-/dstxuvfqwoab",
           o_main="stqdwouvfab/dstuvfqwoab/dstuvfqwoab",
           o_last="stqdouvfab/dstuvfqoab/dstuvfqoab",
           o_end="stqouvfab/stuvfqoab/stuvfo",
           interpret=False, only=None, pv_order=(0, 2, 1), smode=2):
    nb, sq, d = A_x.shape
    n_head, sk = A_k_cache.shape[1], A_k_cache.shape[2]
    n_pair = n_head // 2

    def tr(c):
        return jnp.swapaxes(c, 2, 3).reshape(nb, n_head * _DH, sk)

    aq = _Alg(*(algq or (_ALG_Q, _ORD_Q)), split[0])
    ao = _Alg(*(algo or (_ALG_O, _ORD_O)), split[1])
    u32 = jnp.uint32
    n_xf = -(-len(aq.a_forms) // 4) * 4
    return pl.pallas_call(
        functools.partial(_kernel, nb=nb, n_pair=n_pair, ring=ring, n_main=n_main,
                          u_main=u_main, dbl=dbl, w1_at=w1_at, aq=aq, ao=ao,
                          orders=(o_ramp, o_main, o_last, o_end), only=only, pv_order=pv_order, smode=smode),
        in_specs=[pl.BlockSpec(memory_space=pl.ANY)] * 10,
        out_specs=pl.BlockSpec(memory_space=pl.ANY),
        out_shape=jax.ShapeDtypeStruct((nb, sq, 2 * d), A_x.dtype),
        scratch_shapes=[
            pltpu.VMEM((2, nb, 192, d), _BF16),
            pltpu.VMEM((n_pair, 2, d, _PAIR), _BF16),
            pltpu.VMEM((n_pair, 2, _PAIR, d), _BF16),
            pltpu.VMEM((2, nb, sq, d), _F32),
            pltpu.VMEM((nb, sq, 2 * d), _BF16),
            pltpu.VMEM((ring, 4, _PAIR, sk), _BF16),
            pltpu.VMEM((2, 2, sq // 2, sk), _F32),
            pltpu.VMEM((2, 3, sq // 2, 128), _F32),
            pltpu.VMEM((2, nb, n_xf, sq // 4, 128), u32),
            pltpu.VMEM((2, 2, len(aq.b_forms), 64, 128), u32),
            pltpu.VMEM((2, 2, len(ao.b_forms), 64, 128), u32),
            pltpu.SemaphoreType.DMA((ring + ring // n_main,)),
            pltpu.SemaphoreType.DMA((2,)),
            pltpu.SemaphoreType.DMA((2,)),
            pltpu.SemaphoreType.DMA((1,)),
        ],
        compiler_params=pltpu.CompilerParams(
            vmem_limit_bytes=122 * 1024 * 1024, disable_bounds_checks=True),
        interpret=interpret,
    )(A_x, tr(A_k_cache), tr(A_v_cache), A_wq, A_wo,
      B_x, tr(B_k_cache), tr(B_v_cache), B_wq, B_wo)


@jax.jit
def pallas_concat_heads__gqa_block_cached__mha_block_cached__near_ridge_kernel(
    A_x: jax.Array,
    A_k_cache: jax.Array,
    A_v_cache: jax.Array,
    A_wq: jax.Array,
    A_wo: jax.Array,
    B_x: jax.Array,
    B_k_cache: jax.Array,
    B_v_cache: jax.Array,
    B_wq: jax.Array,
    B_wo: jax.Array,
):
    return _build(A_x, A_k_cache, A_v_cache, A_wq, A_wo,
                  B_x, B_k_cache, B_v_cache, B_wq, B_wo)
```

```python
import functools
import math

import jax
import jax.numpy as jnp
import jax.experimental.pallas as pl
import jax.experimental.pallas.tpu as pltpu

_DH = 192
_PAIR = 2 * _DH
_NT = (((1,), (1,)), ((), ()))
_F32 = jnp.float32
_BF16 = jnp.bfloat16
_SCALE = (_DH ** -0.5) * math.log2(math.e)

_ALG_Q = (
    (((0, 0, 1),), ((0, 0, 1),), ((0, 0, 1),)),
    (((1, 0, 1),), ((0, 0, 1),), ((1, 0, 1),)),
    (((0, 1, 1),), ((1, 0, 1),), ((0, 0, 1),)),
    (((1, 1, 1),), ((1, 0, 1),), ((1, 0, 1),)),
    (((0, 2, 1), (1, 2, -1)), ((2, 0, 1), (2, 1, -1), (2, 2, -1)), ((0, 0, 1),)),
    (((1, 2, 1),), ((2, 0, 1), (3, 0, 1), (4, 0, 1)), ((0, 0, 1), (1, 0, 1))),
    (((0, 0, 1), (1, 0, -1)), ((0, 1, 1), (0, 2, 1)), ((0, 1, 1),)),
    (((1, 0, 1),), ((0, 1, 1), (4, 1, -1)), ((0, 1, 1), (1, 1, 1))),
    (((0, 3, -1), (1, 3, 1)), ((3, 0, -1), (3, 1, 1), (3, 2, 1)), ((1, 1, 1),)),
    (((0, 3, 1),), ((1, 1, 1), (2, 1, 1), (3, 1, 1)), ((0, 1, 1), (1, 1, 1))),
    (((0, 1, 1), (1, 1, -1)), ((1, 1, 1), (1, 2, 1)), ((0, 2, 1),)),
    (((1, 1, 1),), ((1, 2, 1), (3, 2, 1)), ((0, 2, 1), (1, 2, 1))),
    (((0, 4, -1), (1, 4, 1)), ((4, 0, -1), (4, 1, 1), (4, 2, 1)), ((1, 2, 1),)),
    (((0, 4, 1),), ((0, 2, -1), (2, 2, 1), (4, 2, 1)), ((0, 2, 1), (1, 2, 1))),
    (((0, 3, -1), (1, 2, 1)), ((2, 1, -1), (3, 0, -1)), ((0, 0, 1), (1, 1, -1))),
    (((1, 2, 1), (1, 3, -1)), ((3, 0, 1),), ((1, 0, -1), (1, 1, -1))),
    (((0, 2, 1), (0, 3, -1)), ((2, 1, 1),), ((0, 0, 1), (0, 1, 1))),
    (((0, 4, -1), (1, 2, 1)), ((2, 2, -1), (4, 0, -1)), ((0, 0, 1), (1, 2, -1))),
    (((1, 2, 1), (1, 4, -1)), ((4, 0, 1),), ((1, 0, -1), (1, 2, -1))),
    (((0, 2, 1), (0, 4, -1)), ((2, 2, 1),), ((0, 0, 1), (0, 2, 1))),
    (((0, 3, 1), (1, 1, -1)), ((1, 1, -1), (3, 2, 1)), ((0, 2, 1), (1, 1, 1))),
    (((0, 1, -1), (0, 3, 1)), ((1, 1, 1),), ((0, 1, -1), (0, 2, 1))),
    (((1, 1, -1), (1, 3, 1)), ((3, 2, 1),), ((1, 1, -1), (1, 2, 1))),
    (((0, 4, 1), (1, 0, 1)), ((0, 2, 1), (4, 1, 1)), ((0, 1, 1), (1, 2, 1))),
    (((1, 0, 1), (1, 4, 1)), ((4, 1, 1),), ((1, 1, 1), (1, 2, -1))),
    (((0, 0, 1), (0, 4, 1)), ((0, 2, 1),), ((0, 1, -1), (0, 2, 1))),
)
_ALG_O = (
    (((0, 0, 1),), ((0, 0, 1),), ((0, 0, 1),)),
    (((1, 0, 1),), ((0, 0, 1),), ((1, 0, 1),)),
    (((0, 1, 1), (1, 1, -1)), ((1, 0, 1), (1, 4, -1)), ((0, 0, 1),)),
    (((1, 1, 1),), ((1, 0, 1), (2, 0, 1)), ((0, 0, 1), (1, 0, 1))),
    (((0, 0, 1),), ((0, 1, 1),), ((0, 1, 1),)),
    (((1, 0, 1),), ((0, 1, 1),), ((1, 1, 1),)),
    (((0, 2, 1), (1, 2, -1)), ((2, 1, 1), (2, 3, -1)), ((0, 1, 1),)),
    (((1, 2, 1),), ((1, 1, 1), (2, 1, 1)), ((0, 1, 1), (1, 1, 1))),
    (((0, 0, 1), (1, 0, -1)), ((0, 2, 1), (0, 3, -1), (0, 4, -1)), ((0, 2, 1),)),
    (((1, 0, 1),), ((0, 2, 1), (1, 2, 1), (2, 2, 1)), ((0, 2, 1), (1, 2, 1))),
    (((0, 1, -1), (1, 1, 1)), ((1, 1, -1), (1, 2, -1), (1, 3, 1)), ((1, 3, 1),)),
    (((0, 1, 1),), ((0, 3, 1), (1, 3, 1), (2, 3, 1)), ((0, 3, 1), (1, 3, 1))),
    (((0, 2, -1), (1, 2, 1)), ((2, 0, -1), (2, 2, -1), (2, 4, 1)), ((1, 4, 1),)),
    (((0, 2, 1),), ((0, 4, 1), (1, 4, 1), (2, 4, 1)), ((0, 4, 1), (1, 4, 1))),
    (((0, 2, -1), (1, 1, 1)), ((1, 4, -1), (2, 0, -1)), ((0, 0, 1), (1, 4, -1))),
    (((1, 1, 1), (1, 2, -1)), ((2, 0, 1),), ((1, 0, -1), (1, 4, -1))),
    (((0, 1, 1), (0, 2, -1)), ((1, 4, 1),), ((0, 0, 1), (0, 4, 1))),
    (((0, 1, -1), (1, 2, 1)), ((1, 1, -1), (2, 3, -1)), ((0, 1, 1), (1, 3, -1))),
    (((1, 1, -1), (1, 2, 1)), ((1, 1, 1),), ((1, 1, -1), (1, 3, -1))),
    (((0, 1, -1), (0, 2, 1)), ((2, 3, 1),), ((0, 1, 1), (0, 3, 1))),
    (((0, 1, -1), (1, 0, 1)), ((0, 3, -1), (1, 2, -1)), ((0, 2, 1), (1, 3, -1))),
    (((1, 0, 1), (1, 1, -1)), ((1, 2, 1),), ((1, 2, -1), (1, 3, -1))),
    (((0, 0, 1), (0, 1, -1)), ((0, 3, 1),), ((0, 2, 1), (0, 3, 1))),
    (((0, 2, -1), (1, 0, 1)), ((0, 4, -1), (2, 2, -1)), ((0, 2, 1), (1, 4, -1))),
    (((1, 0, 1), (1, 2, -1)), ((2, 2, 1),), ((1, 2, -1), (1, 4, -1))),
    (((0, 0, 1), (0, 2, -1)), ((0, 4, 1),), ((0, 2, 1), (0, 4, 1))),
)


_ORD_Q = (6, 8, 7, 9, 13, 25, 21, 11, 23, 17, 16, 12, 18, 24, 22, 15, 4, 1, 5, 3, 20, 19, 10, 14, 0, 2)
_ORD_O = (4, 1, 19, 6, 15, 3, 14, 16, 20, 9, 22, 11, 8, 25, 23, 13, 24, 12, 10, 21, 17, 7, 18, 5, 0, 2)


class _Alg:
    def __init__(self, table, order, split, lead=4):
        def norm(t):
            sg = t[0][2]
            return tuple((i, j, c * sg) for i, j, c in t), sg
        self.split = split
        self.starts = [0] + list(range(lead, len(order), 4)) + [len(order)]
        self.a_forms, self.b_forms, self.prods = [], [], []
        for r in order:
            a, b, c = table[r]
            (a, sa), (b, sb) = norm(a), norm(b)
            if a not in self.a_forms:
                self.a_forms.append(a)
            if b not in self.b_forms:
                self.b_forms.append(b)
            self.prods.append((a, b, tuple((i, j, v * sa * sb) for i, j, v in c)))


def _dot(a, b):
    return jnp.dot(a, b, preferred_element_type=_F32)


def _nt(a, b):
    return jax.lax.dot_general(a, b, _NT, preferred_element_type=_F32)


def _combine(form, get):
    r = get(form[0][0], form[0][1])
    for i, j, c in form[1:]:
        r = r + get(i, j) if c > 0 else r - get(i, j)
    return r


def _signed_add(d, key, v, sg):
    if key not in d:
        d[key] = (v, sg)
    else:
        w, sw = d[key]
        d[key] = (w + v if sg == sw else w - v, sw)


def _round(prods, out):
    groups, part = {}, {}
    for m, c in prods:
        sg = c[0][2]
        _signed_add(groups, tuple((i, j, v * sg) for i, j, v in c), m, sg)
    for c, (tot, tsg) in groups.items():
        for i, j, v in c:
            _signed_add(part, (i, j), tot, v * tsg)
    for key, (v, sg) in part.items():
        if key not in out:
            out[key] = v if sg > 0 else -v
        else:
            out[key] = out[key] + v if sg > 0 else out[key] - v


def _bilinear(alg, a_of, b_of, out, rounds):
    spans = list(zip(alg.starts[:-1], alg.starts[1:]))
    for r0, r1 in spans[rounds]:
        prods = []
        for a, b, c in alg.prods[r0:r1]:
            av, bv = a_of(a), b_of(b)
            if alg.split and len(alg.prods) - r0 == 2:
                m = jnp.concatenate([_dot(av[0:alg.split], bv), _dot(av[alg.split:], bv)], axis=0)
            else:
                m = _dot(av, bv)
            prods.append((m, c))
        _round(prods, out)


def _pack(v):
    return pltpu.bitcast(v, jnp.uint32)


def _unpack(v):
    return pltpu.bitcast(v, _BF16)


def _lo(n):
    return jax.lax.broadcasted_iota(jnp.int32, (n, 128), 1) < 64


def _q_forms(c):
    a, b = [[c[m, n] * _SCALE for n in range(3)] for m in range(2)]
    lo = _lo(a[0].shape[0])
    rolled = pltpu.roll(b[1], 64, 1)
    forms = []
    for t, own in ((0, lo), (2, jnp.logical_not(lo))):
        t3 = jnp.where(own, a[t], b[t]).astype(_BF16)
        t3f = t3.astype(_F32)
        forms.append((t3,
                      jnp.where(own, a[1], a[t] - t3f).astype(_BF16),
                      jnp.where(own, b[t] - t3f, rolled).astype(_BF16)))
    return forms


def _qk_pass(af, kt, h, i):
    rows = (((0, 64), (128, 64), (0, 128)), ((256, 320), (256, 192), (192, 320)))[h][i]
    if i == 0:
        w = kt[rows[0]:rows[0] + 128]
    else:
        w = jnp.concatenate([kt[r:r + 64] for r in rows], axis=0)
    return _dot(af[i], w)


def _scores(af, kt, h):
    t = [_qk_pass(af, kt, h, i) for i in range(3)]
    return t[1] + t[0], t[2] + t[0]


def _softmax(s):
    es = [jnp.exp2(c - jnp.max(c, axis=-1, keepdims=True)) for c in s]
    parts = [(e[:, 0:128] + e[:, 128:256]) + (e[:, 256:384] + e[:, 384:512]) for e in es]
    return (es[0].astype(_BF16), es[1].astype(_BF16), (es[0] + es[1]).astype(_BF16)), parts


def _pv(p, vt, h, i):
    lo, hi, e = ((0, 64, 128), (256, 320, 192))[h]
    rows = (((e, hi), (lo, e), (lo, hi)), ((lo, e), (e, hi), (lo, hi)))[h][i]
    if rows == (lo, hi):
        w = vt[lo:lo + 128]
    else:
        w = jnp.concatenate([vt[r:r + 64] for r in rows], axis=0)
    return _nt(p[i], w)


def _pv_finish(t0, t1, l0, l1):
    r0, r1 = [[pl.reciprocal(jnp.sum(v, axis=-1, keepdims=True), approx=True) for v in l]
              for l in (l0, l1)]
    lo = _lo(t0[0].shape[0])
    d0 = jnp.where(lo, t0[1], t0[0])
    e0 = t0[2] - d0
    d1 = jnp.where(lo, t1[0], t1[1])
    e1 = t1[2] - d1
    return {(0, 0): jnp.where(lo, e0, d0) * r0[0],
            (1, 0): jnp.where(lo, d0, e0) * r0[1],
            (0, 1): jnp.where(lo, t0[0], t1[0]) * jnp.where(lo, r0[0], r1[0]),
            (1, 1): pltpu.roll(jnp.where(lo, t1[1], t0[1]), 64, 1) * jnp.where(lo, r0[1], r1[1]),
            (0, 2): jnp.where(lo, d1, e1) * r1[0],
            (1, 2): jnp.where(lo, e1, d1) * r1[1]}


def _kernel(xa, ka, va, wqa, woa, xb, kb, vb, wqb, wob, out,
            x_res, wq_res, wo_res, acc, ostage, kv, o_scr, xc, wqc, woc,
            g_sem, w_sem, p_sem, o_sem, *, nb, n_pair, ring, n_main, u_main, dbl, w1_at,
            aq, ao, orders, only, pv_order, raw, u_big, extra):
    lg = nb.bit_length() - 1
    half = nb // 2
    n_pos = n_pair * nb
    sq, d = acc.shape[2], acc.shape[3]
    hm = sq // 2
    wqs, wos = (wqa, wqb), (woa, wob)
    lg_main = n_main.bit_length() - 1
    assert nb == 1 << lg and n_main == 1 << lg_main and half % n_main == 0 and (u_big is None or half % (2 * n_main) == 0)
    assert u_main >= nb and u_main % n_main == 0 and 8 % half == 0

    def static(v):
        return isinstance(v, int)

    def shr(v, s):
        return v >> s if static(v) else jax.lax.shift_right_logical(v, s)

    def aligned(v, m):
        return v if static(v) else pl.multiple_of(v, m)

    def clamp(u, hi=n_pos - 1):
        return min(max(u, 0), hi) if static(u) else jnp.clip(u, 0, hi)

    def when(*conds):
        dyn = [c for c in conds if not isinstance(c, bool)]
        if not all(c for c in conds if isinstance(c, bool)):
            return lambda f: None
        if not dyn:
            return lambda f: f()
        return pl.when(functools.reduce(jnp.logical_and, dyn))

    def pair_ds(p):
        return pl.ds(aligned(p * _PAIR, _PAIR), _PAIR)

    def chunk(ref, u):
        return ref.at[u & (nb - 1), pair_ds(shr(u, lg)), :]

    def sem_of(u, early):
        late = ring + (shr(u, lg_main) & (ring // n_main - 1))
        if static(u):
            return u & (ring - 1) if u < u_main else late
        return jnp.where(u < u_main, u & (ring - 1), late) if early else late

    def x_copy(br, b, sem):
        return pltpu.make_async_copy((xa, xb)[br].at[b], x_res.at[br, b, 0:sq], sem)

    def issue(u, h, early, may_end, enable=True):
        uc = clamp(u) if may_end else u
        sem = g_sem.at[sem_of(uc, early)]
        if early:
            ux = clamp(u, nb - 1)

            @when(enable, u < nb)
            def _():
                x_copy(h, ux, sem).start()
        for i, src in enumerate(((ka, va), (kb, vb))[h]):
            s = chunk(src, uc)

            @when(enable, (u < n_pos) if may_end else True)
            def _():
                pltpu.make_async_copy(s, kv.at[uc & (ring - 1), 2 * h + i], sem).start()
        if early and h == 1:
            @when(enable, u == w1_at)
            def _():
                w_start(1)

    def wq_copy(p, br, sem):
        return pltpu.make_async_copy(wqs[br].at[:, pair_ds(p)], wq_res.at[p, br], sem)

    def wo_copy(p, br, sem):
        return pltpu.make_async_copy(wos[br].at[pair_ds(p), :], wo_res.at[p, br], sem)

    def w_start(p):
        for br in range(2):
            wq_copy(p, br, w_sem.at[p & 1]).start()
            wo_copy(p, br, w_sem.at[p & 1]).start()

    def waits_for(u0, n, early):
        g = min(n, n_main)
        for u in [u0 + i for i in range(0, n, g)]:
            blk = kv.at[pl.ds(aligned(u & (ring - 1), g), g)]
            sem = g_sem.at[u & (ring - 1) if early else sem_of(u, False)]
            pltpu.make_async_copy(blk, blk, sem).wait()
        if early:
            @when(u0 < nb)
            def _():
                for h in range(2):
                    x_copy(0, 0, sem).wait()
        p1 = shr(u0, lg) + 1

        @when((u0 & (nb - 1)) == half, p1 < n_pair)
        def _():
            for ref in (wq_res, wo_res):
                pltpu.make_async_copy(ref.at[p1], ref.at[p1], w_sem.at[p1 & 1]).wait()

    def tile(ref, i, j, rows):
        return ref[i * rows:(i + 1) * rows, j * 128:(j + 1) * 128]

    def qproj(br, b, p, c, rounds=slice(None)):
        _bilinear(aq, lambda f: _unpack(xc[br, b, aq.a_forms.index(f)]),
                  lambda f: _unpack(wqc[p & 1, br, aq.b_forms.index(f)]), c, rounds)
        return c

    def o_forms(o):
        return [_combine(f, lambda i, j: o[i, j]).astype(_BF16) for f in ao.a_forms]

    def oproj(forms, br, b, p, c, rounds):
        if not c:
            c.update({(i, j): tile(acc.at[br, b], i, j, hm)
                      for i in range(2) for j in range(d // 128)})
        _bilinear(ao, lambda f: forms[ao.a_forms.index(f)],
                  lambda f: _unpack(woc[p & 1, br, ao.b_forms.index(f)]), c, rounds)

    def o_store(c, br, b, keep, emit):
        a = acc.at[br, b]
        if keep:
            for (i, j), v in c.items():
                a[i * hm:(i + 1) * hm, j * 128:(j + 1) * 128] = v
        if emit is not False:
            for i in range(2):
                row = jnp.concatenate([c[i, j] for j in range(d // 128)], axis=1)
                ostage[b, i * hm:(i + 1) * hm, br * d:(br + 1) * d] = row.astype(ostage.dtype)
            if br == 1:
                @when(emit)
                def _():
                    pltpu.make_async_copy(ostage.at[b], out.at[b], o_sem.at[0]).start()

    def store_forms(forms, src, put):
        blk = {}

        def get(i, j):
            if (i, j) not in blk:
                blk[i, j] = src(i, j).astype(_F32)
            return blk[i, j]
        for r, f in enumerate(forms):
            put(r, _pack(src(f[0][0], f[0][1]) if len(f) == 1
                         else _combine(f, get).astype(_BF16)))

    def x_forms(br, b):
        def put(r, v):
            xc[br, b, r] = v
        store_forms(aq.a_forms, lambda i, j: tile(x_res.at[br, b], i, j, hm), put)

    def w_forms(br, p, si, lo=0, which=(0, 1)):
        for t in which:
            raw, dst, alg = ((wq_res, wqc, aq), (wo_res, woc, ao))[t]
            view = raw.at[p, br, pl.ds(aligned(si * 16, 16), raw.shape[2] - 112 + 16 * lo)]
            rows = pl.ds(aligned((si + lo) * 8, 8), 8)

            def put(r, v):
                dst[p & 1, br, r, rows, :] = v
            store_forms(alg.b_forms, lambda i, j: view[i * 128 + lo * 16:i * 128 + lo * 16 + 16,
                                                       j * 128:(j + 1) * 128], put)

    def block(u0, n, kind, order, refill, emit_prev=False):
        T = 2 * n
        last = kind in ('last', 'end')

        def task(k):
            u = u0 + k // 2
            if k == -1 and kind == 'ramp':
                u = clamp(u)
            return k % 2, u & (nb - 1), shr(u, lg)

        def kv_ref(k, i):
            return kv.at[(u0 + k // 2) & (ring - 1), 2 * (k % 2) + i]

        Q, S, P, O, OT = {}, {}, {}, {}, {}
        if raw:
            O[-1] = o_forms(_pv_finish(*[[o_scr[r] for r in rr]
                                         for rr in ((0, 1, 2), (3, 4, 5), (6, 7), (8, 9))]))
        else:
            O[-1] = o_forms({(i, j): o_scr[3 * i + j] for i in range(2) for j in range(3)})

        def do_q(k):
            Q[k, 0], Q[k, 1] = _q_forms(qproj(*task(k), {}))

        def do_qk(k, h):
            S[k, h] = _scores(Q.pop((k, h)), kv_ref(k, 0), h)

        def do_pv(k, h):
            P[k, h] = _softmax(S.pop((k, h)))
            for i in pv_order:
                OT[k, h, i] = _pv(P[k, h][0], kv_ref(k, 1), h, i)

        def do_pf(k):
            t0, t1 = [[OT.pop((k, h, i)) for i in range(3)] for h in range(2)]
            l0, l1 = P.pop((k, 0))[1], P.pop((k, 1))[1]
            if k == T - 1 and kind != 'end':
                if raw:
                    for r, v in enumerate(t0 + t1 + l0 + l1):
                        o_scr[r] = v
                else:
                    for (i, j), v in _pv_finish(t0, t1, l0, l1).items():
                        o_scr[3 * i + j] = v
            else:
                O[k] = o_forms(_pv_finish(t0, t1, l0, l1))

        def do_o(k):
            c = {}
            oproj(O.pop(k), *task(k), c, slice(None))
            if k == -1:
                o_store(c, *task(k)[:2], emit_prev is not True, emit_prev if last else False)
            else:
                o_store(c, *task(k)[:2], not last, last)

        def do_w(k):
            br, b, p = task(k)
            pc = jnp.minimum(p + shr(b, lg - 1), n_pair - 1)
            per = 8 // half
            if n >= 4 and half == 8:
                w_forms(br, pc, b & 4, (k // 2) & 3)
            else:
                for i in range(per):
                    w_forms(br, pc, (b & (half - 1)) * per + i)

        ops = {"q": do_q, "a": lambda k: do_qk(k, 0), "b": lambda k: do_qk(k, 1),
               "u": lambda k: do_pv(k, 0), "v": lambda k: do_pv(k, 1), "f": do_pf,
               "o": lambda k: do_o(k - 1), "d": refill, "w": do_w,
               "x": lambda k: x_forms(*task(k)[:2])}
        first, mid, final = order.split("/")
        for k in range(T):
            for c in (final if k == T - 1 else first if k == 0 else mid):
                ops[c](k)
        if kind == 'end':
            do_o(T - 1)
        if not last:
            p2 = shr(u0, lg) + 2

            @when((u0 & (nb - 1)) == (3 * nb // 4 // n) * n, p2 < n_pair)
            def _():
                w_start(p2)

    w0 = [wq_copy(0, 0, p_sem.at[0]), wq_copy(0, 1, p_sem.at[0]),
          wo_copy(0, 0, p_sem.at[0]), wo_copy(0, 1, p_sem.at[0])]
    for c in w0:
        c.start()
    issue(0, 0, True, False)
    issue(0, 1, True, False)

    def zero(b, carry):
        for br in range(2):
            acc[br, b] = jnp.zeros((sq, d), _F32)
        return carry
    jax.lax.fori_loop(0, nb, zero, 0)
    o_scr[0:6] = jnp.zeros((6,) + o_scr.shape[1:], _F32)
    o_scr[6:10] = jnp.ones((4,) + o_scr.shape[1:], _F32)
    for c in w0:
        c.wait()

    def w_first(si, carry):
        for br in range(2):
            w_forms(br, 0, si)
        return carry
    jax.lax.fori_loop(0, 8, w_first, 0)

    lead = 1 + dbl // 2
    assert dbl % 2 == 0 and dbl // 2 <= u_main and n_main < lead < ring and w1_at < half

    def ramp(u, carry):
        fast = u < dbl // 2
        g = u + 1 + jnp.minimum(u, dbl // 2)

        def refill(k):
            if k == 0:
                issue(g, 0, True, False)
                issue(g, 1, True, False, fast)
            else:
                g1 = g + fast.astype(jnp.int32)
                issue(g1, 0, True, False, fast)
                issue(g1, 1, True, False)
        block(u, 1, 'ramp', orders[0], refill)

        @pl.when(u + 1 < u_main)
        def _():
            waits_for(u + 1, 1, True)
        return carry

    waits_for(0, 1, True)
    if only in (None, 0):
        jax.lax.fori_loop(0, u_main, ramp, 0)

    def steady(u_start, n, cnt, n_next, lead, extra, kind, order):
        may_end = u_start + cnt * n + lead + extra > n_pos

        def body(j, carry):
            u0 = u_start + j * n

            def refill(k):
                u, h = u0 + k // 2 + lead, k % 2
                if extra and k // 2 < extra:
                    fast = j == 1
                    g = u + jnp.where(j > 1, extra, jnp.where(fast, k // 2 + h, 0))
                    issue(g, 0, False, may_end, fast if h == 1 else True)
                    issue(g, 1, False, may_end, fast if h == 0 else True)
                else:
                    issue(u + (jnp.where(j >= 1, extra, 0) if extra else 0), h, False, may_end)
            block(u0, n, kind, order, refill, emit_prev=(j > 0) if kind == 'last' else False)
            if n == n_next:
                waits_for(u0 + n, n, False)
            else:
                @pl.when(j + 1 < cnt)
                def _():
                    waits_for(u0 + n, n, False)
            return carry
        jax.lax.fori_loop(0, cnt, body, 0)
        if n != n_next:
            waits_for(u_start + cnt * n, n_next, False)

    u_last = n_pos - nb
    waits_for(u_main, n_main, False)
    if u_big is None:
        if only in (None, 1):
            steady(u_main, n_main, (u_last - u_main) // n_main, n_main, lead, 0, 'main', orders[1])
    else:
        n_big = 2 * n_main
        cnt = (u_big - u_main) // n_main
        assert cnt >= 2 and extra <= n_main and n_big < lead + extra < ring and u_big % n_big == 0
        if only in (None, 1):
            steady(u_main, n_main, cnt, n_big, lead, extra, 'main', orders[1])
        lead += extra
        if only in (None, 4):
            steady(u_big, n_big, (u_last - u_big) // n_big, n_main, lead, 0, 'main', orders[4])
    if only in (None, 2):
        steady(u_last, n_main, nb // n_main - 1, n_main, lead, 0, 'last', orders[2])
    if only in (None, 3):
        block(n_pos - n_main, n_main, 'end', orders[3], lambda k: None, emit_prev=True)
    pltpu.make_async_copy(ostage, out, o_sem.at[0]).wait()


def _build(A_x, A_k_cache, A_v_cache, A_wq, A_wo, B_x, B_k_cache, B_v_cache, B_wq, B_wo, *,
           n_main=4, u_main=24, dbl=10, w1_at=7, ring=16, split=(0, 0),
           algq=None, algo=None, olead=4,
           o_ramp="xqdwoabuvf/-/dxqwoabuvf",
           o_main="qdwoabuvf/dqwoabuvf/dqwoabuvf",
           o_last="qdoabuvf/dqoabuvf/dqoabuvf",
           o_end="qoabuvf/qoabuvf/qoabuvf",
           interpret=False, only=None, pv_order=(0, 2, 1), raw=True, u_big=40, extra=4,
           o_big="qdwoabuvf/dqwoabuvf/dqwoabuvf"):
    nb, sq, d = A_x.shape
    n_head, sk = A_k_cache.shape[1], A_k_cache.shape[2]
    n_pair = n_head // 2

    def tr(c):
        return jnp.swapaxes(c, 2, 3).reshape(nb, n_head * _DH, sk)

    aq = _Alg(*(algq or (_ALG_Q, _ORD_Q)), split[0])
    ao = _Alg(*(algo or (_ALG_O, _ORD_O)), split[1], olead)
    u32 = jnp.uint32
    n_xf = -(-len(aq.a_forms) // 4) * 4
    return pl.pallas_call(
        functools.partial(_kernel, nb=nb, n_pair=n_pair, ring=ring, n_main=n_main,
                          u_main=u_main, dbl=dbl, w1_at=w1_at, aq=aq, ao=ao,
                          orders=(o_ramp, o_main, o_last, o_end, o_big), only=only, pv_order=pv_order, raw=raw, u_big=u_big, extra=extra),
        in_specs=[pl.BlockSpec(memory_space=pl.ANY)] * 10,
        out_specs=pl.BlockSpec(memory_space=pl.ANY),
        out_shape=jax.ShapeDtypeStruct((nb, sq, 2 * d), A_x.dtype),
        scratch_shapes=[
            pltpu.VMEM((2, nb, 192, d), _BF16),
            pltpu.VMEM((n_pair, 2, d, _PAIR), _BF16),
            pltpu.VMEM((n_pair, 2, _PAIR, d), _BF16),
            pltpu.VMEM((2, nb, sq, d), _F32),
            pltpu.VMEM((nb, sq, 2 * d), _BF16),
            pltpu.VMEM((ring, 4, _PAIR, sk), _BF16),
            pltpu.VMEM((10, sq // 2, 128), _F32),
            pltpu.VMEM((2, nb, n_xf, sq // 4, 128), u32),
            pltpu.VMEM((2, 2, len(aq.b_forms), 64, 128), u32),
            pltpu.VMEM((2, 2, len(ao.b_forms), 64, 128), u32),
            pltpu.SemaphoreType.DMA((ring + ring // n_main,)),
            pltpu.SemaphoreType.DMA((2,)),
            pltpu.SemaphoreType.DMA((1,)),
            pltpu.SemaphoreType.DMA((1,)),
        ],
        compiler_params=pltpu.CompilerParams(
            vmem_limit_bytes=122 * 1024 * 1024, disable_bounds_checks=True),
        interpret=interpret,
    )(A_x, tr(A_k_cache), tr(A_v_cache), A_wq, A_wo,
      B_x, tr(B_k_cache), tr(B_v_cache), B_wq, B_wo)


@jax.jit
def pallas_concat_heads__gqa_block_cached__mha_block_cached__near_ridge_kernel(
    A_x: jax.Array,
    A_k_cache: jax.Array,
    A_v_cache: jax.Array,
    A_wq: jax.Array,
    A_wo: jax.Array,
    B_x: jax.Array,
    B_k_cache: jax.Array,
    B_v_cache: jax.Array,
    B_wq: jax.Array,
    B_wo: jax.Array,
):
    return _build(A_x, A_k_cache, A_v_cache, A_wq, A_wo,
                  B_x, B_k_cache, B_v_cache, B_wq, B_wo)
```

```python
import functools
import math

import jax
import jax.numpy as jnp
import jax.experimental.pallas as pl
import jax.experimental.pallas.tpu as pltpu

_DH = 192
_PAIR = 2 * _DH
_NT = (((1,), (1,)), ((), ()))
_F32 = jnp.float32
_BF16 = jnp.bfloat16
_SCALE = (_DH ** -0.5) * math.log2(math.e)

_ALG_Q = (
    (((1, 2, 1), (1, 3, -1)), ((2, 0, 1),), ((1, 0, 1),)),
    (((0, 0, -1), (1, 0, 1)), ((0, 0, 1), (0, 1, -1), (4, 0, 1), (4, 2, 1)), ((1, 0, 1),)),
    (((0, 2, 1), (0, 3, -1)), ((3, 0, 1), (3, 2, 1)), ((0, 0, -1),)),
    (((0, 0, 1),), ((0, 0, 1), (1, 0, -1)), ((0, 0, 1), (1, 0, 1))),
    (((0, 3, 1), (1, 3, -1)), ((3, 1, -1), (3, 2, -1), (4, 1, 1), (4, 2, 1)), ((0, 0, 1), (0, 2, -1))),
    (((0, 0, 1), (0, 1, 1)), ((1, 0, 1),), ((0, 0, 1), (0, 1, 1))),
    (((0, 4, 1),), ((3, 1, -1), (4, 0, 1), (4, 1, 1), (4, 2, 1)), ((0, 0, 1), (0, 1, 1), (0, 2, -1))),
    (((0, 1, 1), (1, 1, -1)), ((1, 0, -1), (1, 1, 1), (1, 2, 1)), ((0, 1, 1),)),
    (((0, 0, -1), (0, 4, 1), (1, 0, 1), (1, 4, -1)), ((4, 0, 1), (4, 2, 1)), ((0, 1, -1), (0, 2, 1))),
    (((0, 0, 1), (1, 0, -1), (1, 4, 1)), ((0, 2, -1), (4, 0, -1), (4, 2, -1)), ((0, 1, 1), (0, 2, -1), (1, 0, -1))),
    (((0, 1, 1), (0, 2, -1)), ((1, 2, 1),), ((0, 1, -1), (0, 2, 1))),
    (((0, 0, 1), (1, 1, 1)), ((0, 1, -1), (0, 2, -1), (1, 0, 1)), ((0, 1, -1), (1, 0, 1))),
    (((0, 2, -1), (1, 1, 1)), ((1, 2, 1), (2, 1, -1)), ((0, 1, 1), (1, 2, 1))),
    (((0, 3, 1), (0, 4, 1)), ((3, 1, 1),), ((0, 1, 1), (1, 1, 1))),
    (((1, 1, 1),), ((0, 1, -1), (0, 2, -1), (1, 1, 1), (2, 1, 1)), ((0, 1, 1), (1, 1, 1))),
    (((1, 0, -1), (1, 4, 1)), ((0, 2, -1),), ((0, 1, -1), (0, 2, 1), (1, 1, -1), (1, 2, 1))),
    (((1, 0, 1), (1, 1, 1)), ((0, 1, 1), (0, 2, 1)), ((1, 0, 1), (1, 1, 1))),
    (((1, 4, 1),), ((0, 2, -1), (4, 2, -1)), ((1, 0, 1), (1, 1, 1), (1, 2, -1))),
    (((1, 1, 1), (1, 2, -1)), ((2, 1, 1),), ((1, 1, -1), (1, 2, 1))),
    (((0, 3, 1), (0, 4, 1), (1, 3, -1), (1, 4, -1)), ((4, 1, -1), (4, 2, -1)), ((1, 1, 1),)),
    (((0, 2, 1), (1, 3, -1)), ((2, 0, -1), (3, 0, -1), (3, 2, -1)), ((0, 0, -1), (0, 2, 1), (1, 2, 1))),
    (((0, 2, 1),), ((1, 2, 1), (2, 0, 1), (2, 2, 1), (3, 0, 1), (3, 2, 1)), ((0, 2, 1), (1, 2, 1))),
    (((0, 3, 1), (0, 4, 1), (1, 3, -1)), ((3, 1, 1), (4, 1, -1), (4, 2, -1)), ((0, 0, 1), (0, 2, -1), (1, 1, -1))),
    (((1, 3, 1),), ((2, 0, 1), (3, 0, 1)), ((0, 0, 1), (0, 2, -1), (1, 0, 1), (1, 2, -1))),
    (((0, 2, -1), (1, 2, 1)), ((2, 1, 1), (2, 2, 1)), ((1, 2, 1),)),
)
_ALG_O = (
    (((1, 0, 1), (1, 1, -1), (1, 2, 1)), ((0, 4, 1),), ((1, 0, -1), (1, 4, 1))),
    (((0, 0, -1), (1, 1, 1), (1, 2, -1)), ((0, 4, -1), (2, 0, -1)), ((0, 4, 1), (1, 0, 1))),
    (((0, 0, 1), (1, 0, -1)), ((0, 0, 1), (0, 1, 1), (0, 4, 1), (2, 1, -1)), ((1, 0, -1),)),
    (((1, 1, 1), (1, 2, -1)), ((0, 4, 1), (1, 3, -1), (1, 4, 1)), ((0, 4, 1), (1, 4, 1))),
    (((0, 1, 1),), ((1, 3, 1),), ((0, 3, 1), (0, 4, 1), (1, 3, 1), (1, 4, 1))),
    (((0, 1, -1), (1, 1, 1)), ((1, 4, 1), (2, 4, 1)), ((1, 3, 1), (1, 4, 1))),
    (((0, 1, 1), (1, 1, -1), (1, 2, 1)), ((1, 3, -1), (1, 4, 1), (2, 4, 1)), ((0, 4, 1), (1, 3, 1), (1, 4, 1))),
    (((0, 0, 1), (1, 1, -1)), ((0, 1, 1), (1, 0, -1), (2, 0, -1), (2, 1, -1)), ((0, 1, 1), (1, 0, 1))),
    (((0, 0, 1),), ((0, 0, 1), (1, 0, 1)), ((0, 0, 1), (1, 0, 1))),
    (((1, 0, -1), (1, 1, 1)), ((0, 1, 1), (2, 1, -1)), ((1, 0, 1), (1, 1, -1))),
    (((0, 0, -1), (0, 1, 1)), ((1, 0, 1), (2, 0, 1)), ((0, 0, 1), (0, 1, -1))),
    (((1, 0, 1), (1, 1, -1), (1, 2, 1)), ((2, 1, 1),), ((1, 1, 1), (1, 2, -1))),
    (((1, 1, 1),), ((0, 1, 1), (1, 1, 1)), ((0, 1, 1), (1, 1, 1))),
    (((0, 0, 1), (0, 2, 1), (1, 0, -1), (1, 2, -1)), ((2, 1, 1), (2, 2, 1)), ((1, 2, -1),)),
    (((0, 0, -1), (0, 2, -1), (1, 1, 1)), ((1, 2, 1), (2, 1, -1)), ((0, 1, 1), (1, 2, 1))),
    (((0, 2, 1),), ((0, 2, -1), (0, 3, -1), (2, 2, 1), (2, 3, 1)), ((0, 3, 1),)),
    (((0, 1, 1), (1, 1, -1)), ((1, 0, 1), (1, 1, 1), (1, 2, 1), (2, 0, 1)), ((0, 1, 1),)),
    (((0, 0, 1), (0, 1, -1), (0, 2, 1)), ((1, 2, 1),), ((0, 1, 1), (0, 2, -1))),
    (((0, 0, -1), (1, 0, 1)), ((0, 2, -1), (2, 2, 1)), ((0, 2, 1), (0, 3, -1))),
    (((1, 0, -1),), ((0, 3, 1),), ((0, 2, 1), (0, 3, -1), (1, 2, 1), (1, 3, -1))),
    (((0, 0, 1), (0, 2, 1), (1, 0, -1)), ((0, 2, -1), (0, 3, -1), (2, 2, 1)), ((0, 2, 1), (0, 3, -1), (1, 2, 1))),
    (((0, 0, 1), (0, 2, 1)), ((0, 2, 1), (0, 3, 1), (1, 2, 1)), ((0, 2, 1), (1, 2, 1))),
    (((1, 2, 1),), ((1, 3, 1), (1, 4, -1), (2, 3, 1), (2, 4, -1)), ((1, 3, 1),)),
    (((0, 1, 1), (0, 2, -1), (1, 1, -1), (1, 2, 1)), ((2, 0, -1), (2, 4, -1)), ((0, 4, 1),)),
    (((0, 0, 1), (0, 1, -1), (0, 2, 1)), ((2, 0, -1),), ((0, 0, -1), (0, 4, 1))),
)


class _Alg:
    def __init__(self, table, order, split, lead=4):
        def norm(t):
            sg = t[0][2]
            return tuple((i, j, c * sg) for i, j, c in t), sg
        self.split = split
        self.starts = [0] + list(range(lead, len(order), 4)) + [len(order)]
        self.a_forms, self.b_forms, self.prods = [], [], []
        for r in order:
            a, b, c = table[r]
            (a, sa), (b, sb) = norm(a), norm(b)
            if a not in self.a_forms:
                self.a_forms.append(a)
            if b not in self.b_forms:
                self.b_forms.append(b)
            self.prods.append((a, b, tuple((i, j, v * sa * sb) for i, j, v in c)))


def _dot(a, b):
    return jnp.dot(a, b, preferred_element_type=_F32)


def _nt(a, b):
    return jax.lax.dot_general(a, b, _NT, preferred_element_type=_F32)


def _combine(form, get):
    r = get(form[0][0], form[0][1])
    for i, j, c in form[1:]:
        r = r + get(i, j) if c > 0 else r - get(i, j)
    return r


def _signed_add(d, key, v, sg):
    if key not in d:
        d[key] = (v, sg)
    else:
        w, sw = d[key]
        d[key] = (w + v if sg == sw else w - v, sw)


def _round(prods, out):
    groups, part = {}, {}
    for m, c in prods:
        sg = c[0][2]
        _signed_add(groups, tuple((i, j, v * sg) for i, j, v in c), m, sg)
    for c, (tot, tsg) in groups.items():
        for i, j, v in c:
            _signed_add(part, (i, j), tot, v * tsg)
    for key, (v, sg) in part.items():
        if key not in out:
            out[key] = v if sg > 0 else -v
        else:
            out[key] = out[key] + v if sg > 0 else out[key] - v


def _bilinear(alg, a_of, b_of, out, rounds, tie=None):
    spans = list(zip(alg.starts[:-1], alg.starts[1:]))
    for r0, r1 in spans[rounds]:
        prods = []
        for a, b, c in alg.prods[r0:r1]:
            av, bv = a_of(a), b_of(b)
            if tie is not None and r0 == 4 * tie[0] and not prods:
                bv = _tie(bv, tie[1]())
            if alg.split and len(alg.prods) - r0 == 2:
                m = jnp.concatenate([_dot(av[0:alg.split], bv), _dot(av[alg.split:], bv)], axis=0)
            else:
                m = _dot(av, bv)
            prods.append((m, c))
        _round(prods, out)


def _pack(v):
    return pltpu.bitcast(v, jnp.uint32)


def _unpack(v):
    return pltpu.bitcast(v, _BF16)


def _tie(v, words):
    u = _pack(v)
    return _unpack(jnp.concatenate([u[0:8] | words, u[8:]], axis=0))


def _lo(n):
    return jax.lax.broadcasted_iota(jnp.int32, (n, 128), 1) < 64


def _q_forms(c):
    a, b = [[c[m, n] * _SCALE for n in range(3)] for m in range(2)]
    lo = _lo(a[0].shape[0])
    rolled = pltpu.roll(b[1], 64, 1)
    forms = []
    for t, own in ((0, lo), (2, jnp.logical_not(lo))):
        t3 = jnp.where(own, a[t], b[t]).astype(_BF16)
        t3f = t3.astype(_F32)
        forms.append((t3,
                      jnp.where(own, a[1], a[t] - t3f).astype(_BF16),
                      jnp.where(own, b[t] - t3f, rolled).astype(_BF16)))
    return forms


def _qk_pass(af, kt, h, i):
    rows = (((0, 64), (128, 64), (0, 128)), ((256, 320), (256, 192), (192, 320)))[h][i]
    if i == 0:
        w = kt[rows[0]:rows[0] + 128]
    else:
        w = jnp.concatenate([kt[r:r + 64] for r in rows], axis=0)
    return _dot(af[i], w)


def _scores(af, kt, h):
    t = [_qk_pass(af, kt, h, i) for i in range(3)]
    return t[1] + t[0], t[2] + t[0]


def _softmax(s):
    es = [jnp.exp2(c - jnp.max(c, axis=-1, keepdims=True)) for c in s]
    parts = [(e[:, 0:128] + e[:, 128:256]) + (e[:, 256:384] + e[:, 384:512]) for e in es]
    return (es[0].astype(_BF16), es[1].astype(_BF16), (es[0] + es[1]).astype(_BF16)), parts


def _pv(p, vt, h, i):
    lo, hi, e = ((0, 64, 128), (256, 320, 192))[h]
    rows = (((e, hi), (lo, e), (lo, hi)), ((lo, e), (e, hi), (lo, hi)))[h][i]
    if rows == (lo, hi):
        w = vt[lo:lo + 128]
    else:
        w = jnp.concatenate([vt[r:r + 64] for r in rows], axis=0)
    return _nt(p[i], w)


def _pv_finish(t0, t1, l0, l1):
    r0, r1 = [[pl.reciprocal(jnp.sum(v, axis=-1, keepdims=True), approx=True) for v in l]
              for l in (l0, l1)]
    lo = _lo(t0[0].shape[0])
    d0 = jnp.where(lo, t0[1], t0[0])
    e0 = t0[2] - d0
    d1 = jnp.where(lo, t1[0], t1[1])
    e1 = t1[2] - d1
    return {(0, 0): jnp.where(lo, e0, d0) * r0[0],
            (1, 0): jnp.where(lo, d0, e0) * r0[1],
            (0, 1): jnp.where(lo, t0[0], t1[0]) * jnp.where(lo, r0[0], r1[0]),
            (1, 1): pltpu.roll(jnp.where(lo, t1[1], t0[1]), 64, 1) * jnp.where(lo, r0[1], r1[1]),
            (0, 2): jnp.where(lo, d1, e1) * r1[0],
            (1, 2): jnp.where(lo, e1, d1) * r1[1]}


def _kernel(xa, ka, va, wqa, woa, xb, kb, vb, wqb, wob, out,
            x_res, wq_res, wo_res, acc, ostage, kv, o_scr, xc, wqc, woc, f_scr, zero_ref,
            g_sem, w_sem, p_sem, o_sem, *, nb, n_pair, ring, n_main, u_main, dbl, w1_at,
            aq, ao, orders, only, pv_order, raw, u_big, extra, pre, g_init, tie_w, tie_f, tie_f0):
    lg = nb.bit_length() - 1
    half = nb // 2
    n_pos = n_pair * nb
    sq, d = acc.shape[2], acc.shape[3]
    hm = sq // 2
    wqs, wos = (wqa, wqb), (woa, wob)
    lg_main = n_main.bit_length() - 1
    assert nb == 1 << lg and n_main == 1 << lg_main and half % n_main == 0 and (u_big is None or half % (2 * n_main) == 0)
    assert u_main >= nb and u_main % n_main == 0 and 8 % half == 0

    def static(v):
        return isinstance(v, int)

    def shr(v, s):
        return v >> s if static(v) else jax.lax.shift_right_logical(v, s)

    def aligned(v, m):
        return v if static(v) else pl.multiple_of(v, m)

    def clamp(u, hi=n_pos - 1):
        return min(max(u, 0), hi) if static(u) else jnp.clip(u, 0, hi)

    def when(*conds):
        dyn = [c for c in conds if not isinstance(c, bool)]
        if not all(c for c in conds if isinstance(c, bool)):
            return lambda f: None
        if not dyn:
            return lambda f: f()
        return pl.when(functools.reduce(jnp.logical_and, dyn))

    def pair_ds(p):
        return pl.ds(aligned(p * _PAIR, _PAIR), _PAIR)

    def chunk(ref, u):
        return ref.at[u & (nb - 1), pair_ds(shr(u, lg)), :]

    def sem_of(u, early):
        late = ring + (shr(u, lg_main) & (ring // n_main - 1))
        if static(u):
            return u & (ring - 1) if u < u_main else late
        return jnp.where(u < u_main, u & (ring - 1), late) if early else late

    def x_copy(br, b, sem):
        return pltpu.make_async_copy((xa, xb)[br].at[b], x_res.at[br, b, 0:sq], sem)

    def issue(u, h, early, may_end, enable=True):
        uc = clamp(u) if may_end else u
        sem = g_sem.at[sem_of(uc, early)]
        if early:
            ux = clamp(u, nb - 1)

            @when(enable, u < nb)
            def _():
                x_copy(h, ux, sem).start()
        for i, src in enumerate(((ka, va), (kb, vb))[h]):
            s = chunk(src, uc)

            @when(enable, (u < n_pos) if may_end else True)
            def _():
                pltpu.make_async_copy(s, kv.at[uc & (ring - 1), 2 * h + i], sem).start()
        if early and h == 1:
            @when(enable, u == w1_at)
            def _():
                w_start(1)

    def wq_copy(p, br, sem):
        return pltpu.make_async_copy(wqs[br].at[:, pair_ds(p)], wq_res.at[p, br], sem)

    def wo_copy(p, br, sem):
        return pltpu.make_async_copy(wos[br].at[pair_ds(p), :], wo_res.at[p, br], sem)

    def w_start(p):
        for br in range(2):
            wq_copy(p, br, w_sem.at[p & 1]).start()
            wo_copy(p, br, w_sem.at[p & 1]).start()

    def waits_for(u0, n, early):
        g = min(n, n_main)
        for u in [u0 + i for i in range(0, n, g)]:
            blk = kv.at[pl.ds(aligned(u & (ring - 1), g), g)]
            sem = g_sem.at[u & (ring - 1) if early else sem_of(u, False)]
            pltpu.make_async_copy(blk, blk, sem).wait()
        if early:
            @when(u0 < nb)
            def _():
                for h in range(2):
                    x_copy(0, 0, sem).wait()
        p1 = shr(u0, lg) + 1

        @when((u0 & (nb - 1)) == half, p1 < n_pair)
        def _():
            for ref in (wq_res, wo_res):
                pltpu.make_async_copy(ref.at[p1], ref.at[p1], w_sem.at[p1 & 1]).wait()

    def tile(ref, i, j, rows):
        return ref[i * rows:(i + 1) * rows, j * 128:(j + 1) * 128]

    def qproj(br, b, p, c, rounds=slice(None), tie=None):
        _bilinear(aq, lambda f: _unpack(xc[br, b, aq.a_forms.index(f)]),
                  lambda f: _unpack(wqc[p & 1, br, aq.b_forms.index(f)]), c, rounds, tie)
        return c

    def o_forms(o):
        return [_combine(f, lambda i, j: o[i, j]).astype(_BF16) for f in ao.a_forms]

    def oproj(forms, br, b, p, c, rounds):
        if not c:
            c.update({(i, j): tile(acc.at[br, b], i, j, hm)
                      for i in range(2) for j in range(d // 128)})
        _bilinear(ao, lambda f: forms[ao.a_forms.index(f)],
                  lambda f: _unpack(woc[p & 1, br, ao.b_forms.index(f)]), c, rounds)

    def o_store(c, br, b, keep, emit):
        a = acc.at[br, b]
        if keep:
            for (i, j), v in c.items():
                a[i * hm:(i + 1) * hm, j * 128:(j + 1) * 128] = v
        if emit is not False:
            for i in range(2):
                row = jnp.concatenate([c[i, j] for j in range(d // 128)], axis=1)
                ostage[b, i * hm:(i + 1) * hm, br * d:(br + 1) * d] = row.astype(ostage.dtype)
            if br == 1:
                @when(emit)
                def _():
                    pltpu.make_async_copy(ostage.at[b], out.at[b], o_sem.at[0]).start()

    def store_forms(forms, src, put):
        blk = {}

        def get(i, j):
            if (i, j) not in blk:
                blk[i, j] = src(i, j).astype(_F32)
            return blk[i, j]
        for r, f in enumerate(forms):
            put(r, _pack(src(f[0][0], f[0][1]) if len(f) == 1
                         else _combine(f, get).astype(_BF16)))

    def x_forms(br, b):
        def put(r, v):
            xc[br, b, r] = v
        store_forms(aq.a_forms, lambda i, j: tile(x_res.at[br, b], i, j, hm), put)

    def w_forms(br, p, si, lo=0, which=(0, 1)):
        for t in which:
            raw, dst, alg = ((wq_res, wqc, aq), (wo_res, woc, ao))[t]
            view = raw.at[p, br, pl.ds(aligned(si * 16, 16), raw.shape[2] - 112 + 16 * lo)]
            rows = pl.ds(aligned((si + lo) * 8, 8), 8)

            def put(r, v):
                dst[p & 1, br, r, rows, :] = v
            store_forms(alg.b_forms, lambda i, j: view[i * 128 + lo * 16:i * 128 + lo * 16 + 16,
                                                       j * 128:(j + 1) * 128], put)

    def block(u0, n, kind, order, refill, emit_prev=False):
        T = 2 * n
        last = kind in ('last', 'end')
        zero_idx = zero_ref[0]
        zero_vec = jnp.full((8, 128), zero_idx, jnp.int32).astype(jnp.uint32)

        def task(k):
            u = u0 + k // 2
            if k == -1 and kind == 'ramp':
                u = clamp(u)
            return k % 2, u & (nb - 1), shr(u, lg)

        def kv_ref(k, i):
            return kv.at[(u0 + k // 2) & (ring - 1), 2 * (k % 2) + i]

        Q, S, P, O, OT = {}, {}, {}, {}, {}
        if raw:
            o = _pv_finish(*[[o_scr[r] for r in rr]
                             for rr in ((0, 1, 2), (3, 4, 5), (6, 7), (8, 9))])
            if tie_f is not None:
                for (i, j), v in o.items():
                    f_scr[3 * i + j] = v
                O[-1] = None
            else:
                O[-1] = o_forms(o)
        else:
            O[-1] = o_forms({(i, j): o_scr[3 * i + j] for i in range(2) for j in range(3)})

        def do_q(k):
            tie = None
            if tie_f is not None:
                tie = (tie_f if k > 0 else tie_f0, lambda: pltpu.bitcast(f_scr[zero_idx, 0:8], jnp.uint32) & zero_vec)
            Q[k, 0], Q[k, 1] = _q_forms(qproj(*task(k), {}, tie=tie))

        def do_qk(k, h):
            af = Q.pop((k, h))
            if tie_w is not None and tie_w // 3 == h and 'w' in order:
                br, _, p = task(k)
                words = (wqc[p & 1, br, 0, 0:8] | woc[p & 1, br, 0, 0:8]) & zero_vec
                af = tuple(_tie(v, words) if i == tie_w % 3 else v for i, v in enumerate(af))
            S[k, h] = _scores(af, kv_ref(k, 0), h)

        def do_pv(k, h):
            P[k, h] = _softmax(S.pop((k, h)))
            for i in pv_order:
                OT[k, h, i] = _pv(P[k, h][0], kv_ref(k, 1), h, i)

        def do_pf(k):
            t0, t1 = [[OT.pop((k, h, i)) for i in range(3)] for h in range(2)]
            l0, l1 = P.pop((k, 0))[1], P.pop((k, 1))[1]
            if k == T - 1 and kind != 'end':
                if raw:
                    for r, v in enumerate(t0 + t1 + l0 + l1):
                        o_scr[r] = v
                else:
                    for (i, j), v in _pv_finish(t0, t1, l0, l1).items():
                        o_scr[3 * i + j] = v
            elif tie_f is not None and k < T - 1:
                for (i, j), v in _pv_finish(t0, t1, l0, l1).items():
                    f_scr[3 * i + j] = v
                O[k] = None
            else:
                O[k] = o_forms(_pv_finish(t0, t1, l0, l1))

        def do_o(k):
            c = {}
            forms = O.pop(k)
            if forms is None:
                forms = o_forms({(i, j): f_scr[3 * i + j] for i in range(2) for j in range(3)})
            oproj(forms, *task(k), c, slice(None))
            if k == -1:
                o_store(c, *task(k)[:2], emit_prev is not True, emit_prev if last else False)
            else:
                o_store(c, *task(k)[:2], not last, last)

        def do_w(k):
            br, b, p = task(k)
            pc = jnp.minimum(p + shr(b, lg - 1), n_pair - 1)
            per = 8 // half
            if n >= 4 and half == 8:
                w_forms(br, pc, b & 4, (k // 2) & 3)
            else:
                for i in range(per):
                    w_forms(br, pc, (b & (half - 1)) * per + i)

        ops = {"q": do_q, "a": lambda k: do_qk(k, 0), "b": lambda k: do_qk(k, 1),
               "u": lambda k: do_pv(k, 0), "v": lambda k: do_pv(k, 1), "f": do_pf,
               "o": lambda k: do_o(k - 1), "d": refill, "w": do_w,
               "x": lambda k: x_forms(*task(k)[:2])}
        first, mid, final = order.split("/")
        for k in range(T):
            for c in (final if k == T - 1 else first if k == 0 else mid):
                ops[c](k)
        if kind == 'end':
            do_o(T - 1)
        if not last:
            p2 = shr(u0, lg) + 2

            @when((u0 & (nb - 1)) == (3 * nb // 4 // n) * n, p2 < n_pair)
            def _():
                w_start(p2)

    zero_ref[0] = 0
    w0 = [wq_copy(0, 0, p_sem.at[0]), wq_copy(0, 1, p_sem.at[0]),
          wo_copy(0, 0, p_sem.at[0]), wo_copy(0, 1, p_sem.at[0])]
    for c in w0:
        c.start()
    if pre >= 1:
        issue(0, 0, True, False)
    if pre >= 2:
        issue(0, 1, True, False)

    def zero(b, carry):
        for br in range(2):
            acc[br, b] = jnp.zeros((sq, d), _F32)
        return carry
    jax.lax.fori_loop(0, nb, zero, 0)
    o_scr[0:6] = jnp.zeros((6,) + o_scr.shape[1:], _F32)
    o_scr[6:10] = jnp.ones((4,) + o_scr.shape[1:], _F32)
    for c in w0:
        c.wait()

    def w_first(si, carry):
        for br in range(2):
            w_forms(br, 0, si)
        for v in range(pre, 2 * g_init):
            issue(v // 2, v % 2, True, False, si == 0)
        return carry
    jax.lax.fori_loop(0, 8, w_first, 0)

    lead = g_init + dbl // 2
    assert dbl % 2 == 0 and dbl // 2 <= u_main and n_main < lead < ring and w1_at < half

    def ramp(u, carry):
        fast = u < dbl // 2
        g = u + g_init + jnp.minimum(u, dbl // 2)

        def refill(k):
            if k == 0:
                issue(g, 0, True, False)
                issue(g, 1, True, False, fast)
            else:
                g1 = g + fast.astype(jnp.int32)
                issue(g1, 0, True, False, fast)
                issue(g1, 1, True, False)
        block(u, 1, 'ramp', orders[0], refill)

        @pl.when(u + 1 < u_main)
        def _():
            waits_for(u + 1, 1, True)
        return carry

    waits_for(0, 1, True)
    if only in (None, 0):
        jax.lax.fori_loop(0, u_main, ramp, 0)

    def steady(u_start, n, cnt, n_next, lead, extra, kind, order):
        may_end = u_start + cnt * n + lead + extra > n_pos

        def body(j, carry):
            u0 = u_start + j * n

            def refill(k):
                u, h = u0 + k // 2 + lead, k % 2
                if extra and k // 2 < extra:
                    fast = j == 1
                    g = u + jnp.where(j > 1, extra, jnp.where(fast, k // 2 + h, 0))
                    issue(g, 0, False, may_end, fast if h == 1 else True)
                    issue(g, 1, False, may_end, fast if h == 0 else True)
                else:
                    issue(u + (jnp.where(j >= 1, extra, 0) if extra else 0), h, False, may_end)
            block(u0, n, kind, order, refill, emit_prev=(j > 0) if kind == 'last' else False)
            if n == n_next:
                waits_for(u0 + n, n, False)
            else:
                @pl.when(j + 1 < cnt)
                def _():
                    waits_for(u0 + n, n, False)
            return carry
        jax.lax.fori_loop(0, cnt, body, 0)
        if n != n_next:
            waits_for(u_start + cnt * n, n_next, False)

    u_last = n_pos - nb
    waits_for(u_main, n_main, False)
    if u_big is None:
        if only in (None, 1):
            steady(u_main, n_main, (u_last - u_main) // n_main, n_main, lead, 0, 'main', orders[1])
    else:
        n_big = 2 * n_main
        cnt = (u_big - u_main) // n_main
        assert cnt >= 2 and extra <= n_main and n_big < lead + extra < ring and u_big % n_big == 0
        if only in (None, 1):
            steady(u_main, n_main, cnt, n_big, lead, extra, 'main', orders[1])
        lead += extra
        if only in (None, 4):
            steady(u_big, n_big, (u_last - u_big) // n_big, n_main, lead, 0, 'main', orders[4])
    if only in (None, 2):
        steady(u_last, n_main, nb // n_main - 1, n_main, lead, 0, 'last', orders[2])
    if only in (None, 3):
        block(n_pos - n_main, n_main, 'end', orders[3], lambda k: None, emit_prev=True)
    pltpu.make_async_copy(ostage, out, o_sem.at[0]).wait()


def _build(A_x, A_k_cache, A_v_cache, A_wq, A_wo, B_x, B_k_cache, B_v_cache, B_wq, B_wo, *,
           n_main=4, u_main=24, dbl=8, w1_at=7, ring=16, split=(0, 48),
           algq=None, algo=None, olead=3,
           o_ramp="xqdwoabuvf/-/dxqwoabuvf",
           o_main="qdwoabuvf/dqwoabuvf/dqwoabuvf",
           o_last="qdoabuvf/dqoabuvf/dqoabuvf",
           o_end="qoabuvf/qoabuvf/qabuvfo",
           interpret=False, only=None, pv_order=(0, 2, 1), raw=True, u_big=40, extra=4, pre=1, g_init=2, tie_w=4, tie_f=5, tie_f0=4,
           o_big="qdwoabuvf/dqwoabuvf/dqwoabuvf"):
    nb, sq, d = A_x.shape
    n_head, sk = A_k_cache.shape[1], A_k_cache.shape[2]
    n_pair = n_head // 2

    def tr(c):
        return jnp.swapaxes(c, 2, 3).reshape(nb, n_head * _DH, sk)

    aq = _Alg(*(algq or (_ALG_Q, range(len(_ALG_Q)))), split[0])
    ao = _Alg(*(algo or (_ALG_O, range(len(_ALG_O)))), split[1], olead)
    u32 = jnp.uint32
    n_xf = -(-len(aq.a_forms) // 4) * 4
    return pl.pallas_call(
        functools.partial(_kernel, nb=nb, n_pair=n_pair, ring=ring, n_main=n_main,
                          u_main=u_main, dbl=dbl, w1_at=w1_at, aq=aq, ao=ao,
                          orders=(o_ramp, o_main, o_last, o_end, o_big), only=only, pv_order=pv_order, raw=raw, u_big=u_big, extra=extra, pre=pre, g_init=g_init, tie_w=tie_w, tie_f=tie_f, tie_f0=tie_f0),
        in_specs=[pl.BlockSpec(memory_space=pl.ANY)] * 10,
        out_specs=pl.BlockSpec(memory_space=pl.ANY),
        out_shape=jax.ShapeDtypeStruct((nb, sq, 2 * d), A_x.dtype),
        scratch_shapes=[
            pltpu.VMEM((2, nb, 192, d), _BF16),
            pltpu.VMEM((n_pair, 2, d, _PAIR), _BF16),
            pltpu.VMEM((n_pair, 2, _PAIR, d), _BF16),
            pltpu.VMEM((2, nb, sq, d), _F32),
            pltpu.VMEM((nb, sq, 2 * d), _BF16),
            pltpu.VMEM((ring, 4, _PAIR, sk), _BF16),
            pltpu.VMEM((10, sq // 2, 128), _F32),
            pltpu.VMEM((2, nb, n_xf, sq // 4, 128), u32),
            pltpu.VMEM((2, 2, len(aq.b_forms), 64, 128), u32),
            pltpu.VMEM((2, 2, len(ao.b_forms), 64, 128), u32),
            pltpu.VMEM((6, sq // 2, 128), _F32),
            pltpu.SMEM((1,), jnp.int32),
            pltpu.SemaphoreType.DMA((ring + ring // n_main,)),
            pltpu.SemaphoreType.DMA((2,)),
            pltpu.SemaphoreType.DMA((1,)),
            pltpu.SemaphoreType.DMA((1,)),
        ],
        compiler_params=pltpu.CompilerParams(
            vmem_limit_bytes=122 * 1024 * 1024, disable_bounds_checks=True),
        interpret=interpret,
    )(A_x, tr(A_k_cache), tr(A_v_cache), A_wq, A_wo,
      B_x, tr(B_k_cache), tr(B_v_cache), B_wq, B_wo)


@jax.jit
def pallas_concat_heads__gqa_block_cached__mha_block_cached__near_ridge_kernel(
    A_x: jax.Array,
    A_k_cache: jax.Array,
    A_v_cache: jax.Array,
    A_wq: jax.Array,
    A_wo: jax.Array,
    B_x: jax.Array,
    B_k_cache: jax.Array,
    B_v_cache: jax.Array,
    B_wq: jax.Array,
    B_wo: jax.Array,
):
    return _build(A_x, A_k_cache, A_v_cache, A_wq, A_wo,
                  B_x, B_k_cache, B_v_cache, B_wq, B_wo)
```

```python
import functools
import math

import jax
import jax.numpy as jnp
import jax.experimental.pallas as pl
import jax.experimental.pallas.tpu as pltpu

_DH = 192
_PAIR = 2 * _DH
_NT = (((1,), (1,)), ((), ()))
_F32 = jnp.float32
_BF16 = jnp.bfloat16
_SCALE = (_DH ** -0.5) * math.log2(math.e)

_ALG_Q = (
    (((1, 4, 1),), ((3, 2, -1), (4, 0, 1), (4, 1, -1), (4, 2, 1)), ((1, 0, 1), (1, 1, 1), (1, 2, 1))),
    (((1, 1, 1), (1, 2, -1)), ((2, 0, 1),), ((1, 0, -1), (1, 2, -1))),
    (((0, 3, 1), (1, 3, -1), (1, 4, -1)), ((3, 2, -1), (4, 1, -1), (4, 2, 1)), ((0, 2, -1), (1, 0, 1), (1, 1, 1))),
    (((0, 3, -1), (1, 3, 1)), ((3, 1, 1), (3, 2, -1), (4, 1, -1), (4, 2, 1)), ((1, 0, 1), (1, 1, 1))),
    (((1, 1, 1),), ((1, 0, 1), (2, 0, 1)), ((0, 0, 1), (1, 0, 1))),
    (((0, 3, -1), (1, 0, 1)), ((0, 0, 1), (3, 0, 1), (3, 1, -1)), ((0, 1, 1), (1, 0, 1), (1, 1, 1))),
    (((0, 3, 1),), ((0, 0, 1), (3, 0, 1)), ((0, 0, 1), (0, 1, 1), (1, 0, 1), (1, 1, 1))),
    (((1, 0, 1), (1, 3, -1)), ((3, 0, -1), (3, 1, 1)), ((1, 0, 1),)),
    (((0, 3, 1), (0, 4, 1), (1, 3, -1), (1, 4, -1)), ((4, 1, 1), (4, 2, -1)), ((0, 2, -1),)),
    (((1, 3, 1), (1, 4, 1)), ((3, 2, 1),), ((0, 2, 1), (1, 2, 1))),
    (((0, 2, -1), (1, 2, 1)), ((2, 0, -1), (2, 1, -1), (2, 2, 1)), ((1, 2, 1),)),
    (((0, 2, 1),), ((0, 2, -1), (1, 1, -1), (1, 2, 1), (2, 2, 1)), ((0, 2, 1), (1, 2, 1))),
    (((0, 2, 1), (1, 0, 1)), ((0, 2, 1), (2, 1, -1)), ((0, 1, -1), (1, 2, 1))),
    (((1, 0, 1),), ((0, 0, -1), (0, 1, 1), (2, 1, -1), (3, 0, -1), (3, 1, 1)), ((0, 1, 1), (1, 1, 1))),
    (((0, 1, -1), (0, 4, 1)), ((1, 1, 1),), ((0, 1, -1), (0, 2, -1), (1, 1, -1), (1, 2, -1))),
    (((0, 0, 1), (0, 2, 1)), ((0, 2, 1),), ((0, 1, 1), (0, 2, 1))),
    (((1, 0, 1), (1, 2, 1)), ((2, 1, 1),), ((1, 1, 1), (1, 2, 1))),
    (((0, 1, -1), (0, 4, 1), (1, 1, 1), (1, 4, -1)), ((4, 0, 1), (4, 1, -1)), ((1, 1, 1), (1, 2, 1))),
    (((0, 1, -1), (0, 4, 1), (1, 1, 1)), ((1, 1, 1), (4, 0, -1), (4, 1, 1)), ((0, 0, -1), (1, 1, 1), (1, 2, 1))),
    (((0, 2, -1), (1, 1, 1)), ((1, 1, 1), (1, 2, -1), (2, 0, -1)), ((0, 0, 1), (1, 2, -1))),
    (((0, 1, 1), (1, 1, -1)), ((1, 0, 1), (1, 2, -1), (4, 0, 1), (4, 1, -1)), ((0, 0, 1),)),
    (((0, 4, 1),), ((1, 1, 1), (4, 1, 1)), ((0, 0, 1), (0, 1, 1), (0, 2, 1))),
    (((0, 0, 1), (1, 0, -1)), ((0, 1, 1), (0, 2, -1)), ((0, 1, 1),)),
    (((0, 1, 1), (0, 2, -1)), ((1, 1, -1), (1, 2, 1)), ((0, 0, 1), (0, 2, 1))),
    (((0, 0, 1), (0, 3, -1)), ((0, 0, 1),), ((0, 0, 1),)),
)
_ALG_O = (
    (((1, 2, 1),), ((0, 1, -1), (1, 1, 1), (2, 1, 1)), ((0, 1, -1), (1, 1, 1))),
    (((1, 0, 1), (1, 1, 1)), ((1, 1, -1),), ((1, 1, -1), (1, 2, 1))),
    (((0, 2, 1), (1, 2, 1)), ((1, 1, 1), (1, 2, 1), (2, 1, 1), (2, 2, 1), (2, 4, -1)), ((0, 1, 1),)),
    (((1, 1, -1), (1, 2, 1)), ((2, 0, 1), (2, 3, 1)), ((1, 0, 1),)),
    (((0, 0, 1), (0, 1, 1), (0, 2, -1), (1, 0, 1)), ((0, 0, 1), (0, 2, -1), (1, 2, 1)), ((0, 0, 1), (0, 2, 1), (1, 2, -1))),
    (((1, 0, -1),), ((0, 0, -1),), ((0, 0, -1), (0, 2, -1), (1, 0, 1), (1, 2, 1))),
    (((0, 0, 1), (1, 0, 1)), ((0, 2, 1), (1, 2, -1)), ((0, 0, 1), (0, 2, 1))),
    (((0, 2, 1), (1, 2, 1)), ((2, 3, 1),), ((1, 0, -1), (1, 3, 1))),
    (((0, 2, 1),), ((1, 0, 1), (2, 0, 1)), ((0, 0, 1), (0, 3, -1), (1, 0, -1), (1, 3, 1))),
    (((0, 2, 1), (1, 1, 1)), ((1, 0, -1), (2, 0, -1), (2, 3, -1)), ((0, 3, -1), (1, 0, -1), (1, 3, 1))),
    (((0, 1, -1), (0, 2, 1)), ((0, 0, 1), (0, 2, -1), (1, 0, -1), (1, 2, 1)), ((0, 0, 1),)),
    (((0, 0, 1), (0, 1, 1)), ((1, 2, 1), (2, 2, 1)), ((0, 1, -1), (0, 2, 1))),
    (((0, 0, -1), (0, 1, -1), (0, 2, 1)), ((0, 0, 1), (0, 2, -1), (1, 2, 1), (2, 2, 1)), ((0, 2, 1), (1, 2, -1))),
    (((0, 0, -1), (0, 1, -1), (0, 2, 1), (1, 0, -1), (1, 1, -1), (1, 2, 1)), ((1, 1, -1), (1, 2, -1)), ((1, 2, 1),)),
    (((0, 0, -1), (0, 1, -1), (0, 2, 1), (1, 2, 1)), ((1, 1, 1), (1, 2, 1), (2, 2, 1)), ((0, 1, -1), (1, 2, 1))),
    (((1, 0, 1), (1, 1, 1)), ((0, 3, 1),), ((1, 3, 1), (1, 4, 1))),
    (((0, 0, 1), (1, 0, 1)), ((0, 1, -1), (0, 3, -1), (0, 4, 1), (1, 1, 1)), ((1, 4, 1),)),
    (((0, 0, 1), (1, 1, -1)), ((0, 3, 1), (1, 4, -1)), ((0, 3, 1), (1, 4, 1))),
    (((1, 1, 1),), ((0, 3, -1), (1, 0, 1), (1, 3, 1), (2, 0, 1), (2, 3, 1)), ((0, 3, -1), (1, 3, 1))),
    (((0, 0, 1),), ((0, 4, 1), (1, 4, -1), (2, 4, -1)), ((0, 4, 1), (1, 4, -1))),
    (((1, 0, 1), (1, 2, 1)), ((0, 1, 1), (1, 1, -1)), ((1, 1, 1), (1, 4, 1))),
    (((0, 0, -1), (1, 2, 1)), ((0, 1, -1), (1, 1, 1), (2, 4, 1)), ((0, 1, 1), (1, 4, 1))),
    (((0, 0, 1), (0, 2, 1)), ((2, 4, 1),), ((0, 1, 1), (0, 4, 1))),
    (((0, 1, 1), (1, 1, 1)), ((1, 3, 1), (1, 4, -1)), ((0, 3, 1),)),
    (((0, 0, 1), (0, 1, 1)), ((1, 4, 1),), ((0, 3, 1), (0, 4, 1))),
)

_PLAN = {
    "ramp": ("xqdwyoabuvf", "", "dxqwyoabuvf", None, 6, 3),
    "main": ("qdwoabuvf", "dqwoabuvf", "dqwoabuvf", 4, 6, 4),
    "last": ("qdoabuvf", "dqoabuvf", "dqoabuvf", None, 4, 3),
    "end": ("qoabuvf", "qoabuvf", "qabuvfo", None, 6, 3),
}


class _Alg:
    def __init__(self, table, lead):
        def norm(t):
            sg = t[0][2]
            return tuple((i, j, c * sg) for i, j, c in t), sg
        starts = [0] + list(range(lead, len(table), 4)) + [len(table)]
        self.rounds = list(zip(starts[:-1], starts[1:]))
        self.a_forms, self.b_forms, self.prods = [], [], []
        for a, b, c in table:
            (a, sa), (b, sb) = norm(a), norm(b)
            if a not in self.a_forms:
                self.a_forms.append(a)
            if b not in self.b_forms:
                self.b_forms.append(b)
            self.prods.append((a, b, tuple((i, j, v * sa * sb) for i, j, v in c)))


def _dot(a, b):
    return jnp.dot(a, b, preferred_element_type=_F32)


def _nt(a, b):
    return jax.lax.dot_general(a, b, _NT, preferred_element_type=_F32)


def _combine(form, get):
    r = get(form[0][0], form[0][1])
    for i, j, c in form[1:]:
        r = r + get(i, j) if c > 0 else r - get(i, j)
    return r


def _signed_add(d, key, v, sg):
    if key not in d:
        d[key] = (v, sg)
    else:
        w, sw = d[key]
        d[key] = (w + v if sg == sw else w - v, sw)


def _round(prods, out):
    groups, part = {}, {}
    for m, c in prods:
        sg = c[0][2]
        _signed_add(groups, tuple((i, j, v * sg) for i, j, v in c), m, sg)
    for c, (tot, tsg) in groups.items():
        for i, j, v in c:
            _signed_add(part, (i, j), tot, v * tsg)
    for key, (v, sg) in part.items():
        if key not in out:
            out[key] = v if sg > 0 else -v
        else:
            out[key] = out[key] + v if sg > 0 else out[key] - v


def _bilinear(alg, a_of, b_of, out, tie=None, cut=None):
    for rnd, (r0, r1) in enumerate(alg.rounds):
        prods = []
        for a, b, c in alg.prods[r0:r1]:
            av, bv = a_of(a), b_of(b)
            if tie is not None and rnd == tie[0] and not prods:
                bv = _tie(bv, tie[1]())
            if cut is not None and len(alg.prods) - r0 == 2:
                m = jnp.concatenate([_dot(av[0:cut], bv), _dot(av[cut:], bv)], axis=0)
            else:
                m = _dot(av, bv)
            prods.append((m, c))
        _round(prods, out)
    return out


def _pack(v):
    return pltpu.bitcast(v, jnp.uint32)


def _unpack(v):
    return pltpu.bitcast(v, _BF16)


def _tie(v, words):
    u = _pack(v)
    return _unpack(jnp.concatenate([u[0:8] | words, u[8:]], axis=0))


def _lo(n):
    return jax.lax.broadcasted_iota(jnp.int32, (n, 128), 1) < 64


def _q_forms(c):
    a, b = [[c[m, n] * _SCALE for n in range(3)] for m in range(2)]
    lo = _lo(a[0].shape[0])
    rolled = pltpu.roll(b[1], 64, 1)
    forms = []
    for t, own in ((0, lo), (2, jnp.logical_not(lo))):
        t3 = jnp.where(own, a[t], b[t]).astype(_BF16)
        t3f = t3.astype(_F32)
        forms.append((t3,
                      jnp.where(own, a[1], a[t] - t3f).astype(_BF16),
                      jnp.where(own, b[t] - t3f, rolled).astype(_BF16)))
    return forms


def _qk_pass(af, kt, h, i):
    rows = (((0, 64), (128, 64), (0, 128)), ((256, 320), (256, 192), (192, 320)))[h][i]
    if i == 0:
        w = kt[rows[0]:rows[0] + 128]
    else:
        w = jnp.concatenate([kt[r:r + 64] for r in rows], axis=0)
    return _dot(af[i], w)


def _scores(af, kt, h):
    t = [_qk_pass(af, kt, h, i) for i in range(3)]
    return t[1] + t[0], t[2] + t[0]


def _softmax(s, g):
    s = (s[0], s[1] * jnp.concatenate([g] * 4, axis=1))
    es = [jnp.exp2(c - jnp.max(c, axis=-1, keepdims=True)) for c in s]
    parts = [(e[:, 0:128] + e[:, 128:256]) + (e[:, 256:384] + e[:, 384:512]) for e in es]
    return (es[0].astype(_BF16), es[1].astype(_BF16), (es[0] + es[1]).astype(_BF16)), parts


def _pv(p, vt, h, i):
    lo, hi, e = ((0, 64, 128), (256, 320, 192))[h]
    rows = (((e, hi), (lo, e), (lo, hi)), ((lo, e), (e, hi), (lo, hi)))[h][i]
    if rows == (lo, hi):
        w = vt[lo:lo + 128]
    else:
        w = jnp.concatenate([vt[r:r + 64] for r in rows], axis=0)
    return _nt(p[i], w)


def _pv_finish(t0, t1, l0, l1):
    r0, r1 = [[pl.reciprocal(jnp.sum(v, axis=-1, keepdims=True), approx=True) for v in l]
              for l in (l0, l1)]
    lo = _lo(t0[0].shape[0])
    d0 = jnp.where(lo, t0[1], t0[0])
    e0 = t0[2] - d0
    d1 = jnp.where(lo, t1[0], t1[1])
    e1 = t1[2] - d1
    return {(0, 0): jnp.where(lo, e0, d0) * r0[0],
            (1, 0): jnp.where(lo, d0, e0) * r0[1],
            (0, 1): jnp.where(lo, t0[0], t1[0]) * jnp.where(lo, r0[0], r1[0]),
            (1, 1): pltpu.roll(jnp.where(lo, t1[1], t0[1]), 64, 1) * jnp.where(lo, r0[1], r1[1]),
            (0, 2): jnp.where(lo, d1, e1) * r1[0],
            (1, 2): jnp.where(lo, e1, d1) * r1[1]}


def _kernel(xa, ka, va, wqa, woa, xb, kb, vb, wqb, wob, out,
            x_res, wq_res, wo_res, acc, ostage, kv, o_scr, xc, wqc, woc, f_scr, x_scale,
            zero_ref, g_sem, w_sem, p_sem, o_sem, *, aq, ao, plan, cuts, n_main, u_main, lead,
            w1_at, only):
    n_pair, nb, ring = wq_res.shape[0], acc.shape[1], kv.shape[0]
    sq, d = acc.shape[2], acc.shape[3]
    lg = nb.bit_length() - 1
    lg_main = n_main.bit_length() - 1
    half, hm = nb // 2, sq // 2
    n_pos = n_pair * nb
    assert nb == 1 << lg and n_main == 1 << lg_main and half % n_main == 0 and 8 % half == 0
    assert u_main >= nb and u_main % n_main == 0
    assert n_main < lead < ring and lead <= u_main and w1_at < half

    def static(v):
        return isinstance(v, int)

    def shr(v, s):
        return v >> s if static(v) else jax.lax.shift_right_logical(v, s)

    def aligned(v, m):
        return v if static(v) else pl.multiple_of(v, m)

    def clamp(u, hi=n_pos - 1):
        return min(max(u, 0), hi) if static(u) else jnp.clip(u, 0, hi)

    def when(*conds):
        dyn = [c for c in conds if not isinstance(c, bool)]
        if not all(c for c in conds if isinstance(c, bool)):
            return lambda f: None
        if not dyn:
            return lambda f: f()
        return pl.when(functools.reduce(jnp.logical_and, dyn))

    def pair_ds(p):
        return pl.ds(aligned(p * _PAIR, _PAIR), _PAIR)

    def sem_of(u, early):
        late = ring + (shr(u, lg_main) & (ring // n_main - 1))
        if static(u):
            return u & (ring - 1) if u < u_main else late
        return jnp.where(u < u_main, u & (ring - 1), late) if early else late

    def x_copy(br, b, sem):
        return pltpu.make_async_copy((xa, xb)[br].at[b], x_res.at[br, b, 0:sq], sem)

    def issue(u, h, early, may_end, enable=True):
        uc = clamp(u) if may_end else u
        sem = g_sem.at[sem_of(uc, early)]
        if early:
            ux = clamp(u + 1, nb - 1)

            @when(enable, u + 1 < nb)
            def _():
                x_copy(h, ux, sem).start()
        for i, ref in enumerate(((ka, va), (kb, vb))[h]):
            src = ref.at[uc & (nb - 1), pair_ds(shr(uc, lg)), :]

            @when(enable, (u < n_pos) if may_end else True)
            def _():
                pltpu.make_async_copy(src, kv.at[uc & (ring - 1), 2 * h + i], sem).start()
        if early and h == 1:
            @when(enable, u == w1_at)
            def _():
                w_start(1)

    def wq_copy(p, br, sem):
        return pltpu.make_async_copy((wqa, wqb)[br].at[:, pair_ds(p)], wq_res.at[p, br], sem)

    def wo_copy(p, br, sem):
        return pltpu.make_async_copy((woa, wob)[br].at[pair_ds(p), :], wo_res.at[p, br], sem)

    def w_start(p):
        for br in range(2):
            wq_copy(p, br, w_sem.at[p & 1]).start()
            wo_copy(p, br, w_sem.at[p & 1]).start()

    def waits_for(u0, n, early):
        blk = kv.at[pl.ds(aligned(u0 & (ring - 1), n), n)]
        sem = g_sem.at[u0 & (ring - 1) if early else sem_of(u0, False)]
        pltpu.make_async_copy(blk, blk, sem).wait()
        if early:
            @when(u0 + 1 < nb)
            def _():
                for _ in range(2):
                    x_copy(0, 0, sem).wait()
        p1 = shr(u0, lg) + 1

        @when((u0 & (nb - 1)) == half, p1 < n_pair)
        def _():
            for ref in (wq_res, wo_res):
                pltpu.make_async_copy(ref.at[p1], ref.at[p1], w_sem.at[p1 & 1]).wait()

    def tile(ref, i, j, rows):
        return ref[i * rows:(i + 1) * rows, j * 128:(j + 1) * 128]

    def x_balance(br, b):
        m = [jnp.broadcast_to(jnp.max(jnp.abs(x_res[br, b, i * hm:(i + 1) * hm, :].astype(_F32)),
                                      axis=-1, keepdims=True), (hm, 128)) for i in range(2)]
        ratio = m[1] * pl.reciprocal(m[0], approx=True) * math.sqrt(2.0)
        ratio = jnp.where(jnp.logical_and(m[0] > 0, m[1] > 0), ratio, 1.0)
        e = jnp.clip(pltpu.bitcast(ratio, jnp.int32) & 0x7f800000, 0x20000000, 0x5f000000)
        x_scale[br, b, 0:hm] = pltpu.bitcast(e, _F32)

    def x_forms(br, b, g):
        inv = pltpu.bitcast(0x7f000000 - pltpu.bitcast(g, jnp.int32), _F32)
        x = x_res.at[br, b]
        blk = {}
        for j in range(d // 128):
            blk[0, j] = tile(x, 0, j, hm).astype(_F32)
            blk[1, j] = tile(x, 1, j, hm).astype(_F32) * inv
        for r, f in enumerate(aq.a_forms):
            xc[br, b, r] = _pack(tile(x, 0, f[0][1], hm) if len(f) == 1 and f[0][0] == 0
                                 else _combine(f, lambda i, j: blk[i, j]).astype(_BF16))

    def w_forms(br, p, si, lo=0):
        for raw, dst, alg in ((wq_res, wqc, aq), (wo_res, woc, ao)):
            view = raw.at[p, br, pl.ds(aligned(si * 16, 16), raw.shape[2] - 112 + 16 * lo)]
            rows = pl.ds(aligned((si + lo) * 8, 8), 8)
            blk = {}

            def src(i, j):
                return view[i * 128 + lo * 16:i * 128 + lo * 16 + 16, j * 128:(j + 1) * 128]

            def get(i, j):
                if (i, j) not in blk:
                    blk[i, j] = src(i, j).astype(_F32)
                return blk[i, j]
            for r, f in enumerate(alg.b_forms):
                dst[p & 1, br, r, rows, :] = _pack(
                    src(f[0][0], f[0][1]) if len(f) == 1 else _combine(f, get).astype(_BF16))

    def block(u0, n, kind, refill, emit_prev=False):
        T = 2 * n
        last = kind in ("last", "end")
        first_order, mid_order, last_order, tie_w, tie_f, tie_f0 = plan[kind]
        zero_idx = zero_ref[0]
        zero_vec = jnp.full((8, 128), zero_idx, jnp.int32).astype(jnp.uint32)

        def task(k):
            u = u0 + k // 2
            if k == -1 and kind == "ramp":
                u = clamp(u)
            return k % 2, u & (nb - 1), shr(u, lg)

        def kv_ref(k, i):
            return kv.at[(u0 + k // 2) & (ring - 1), 2 * (k % 2) + i]

        def put_o(o):
            for (i, j), v in o.items():
                f_scr[3 * i + j] = v

        Q, S, P, OT, O = {}, {}, {}, {}, {}
        G = {k: x_scale[k % 2, task(k)[1], 0:hm] for k in range(T)} if kind == "ramp" else {}
        put_o(_pv_finish(*[[o_scr[r] for r in rr]
                           for rr in ((0, 1, 2), (3, 4, 5), (6, 7), (8, 9))]))

        def do_q(k):
            br, b, p = task(k)
            tie = (tie_f if k > 0 else tie_f0,
                   lambda: pltpu.bitcast(f_scr[zero_idx, 0:8], jnp.uint32) & zero_vec)
            Q[k, 0], Q[k, 1] = _q_forms(_bilinear(
                aq, lambda f: _unpack(xc[br, b, aq.a_forms.index(f)]),
                lambda f: _unpack(wqc[p & 1, br, aq.b_forms.index(f)]), {}, tie))

        def do_qk(k, h):
            af = Q.pop((k, h))
            if tie_w is not None and tie_w // 3 == h:
                br, _, p = task(k)
                for ref in (wqc, woc):
                    words = ref[p & 1, br, 0, 0:8] & zero_vec
                    af = tuple(_tie(v, words) if i == tie_w % 3 else v for i, v in enumerate(af))
            S[k, h] = _scores(af, kv_ref(k, 0), h)

        def do_pv(k, h):
            br, b, _ = task(k)
            P[k, h] = _softmax(S.pop((k, h)), G[k] if k in G else x_scale[br, b, 0:hm])
            for i in (0, 2, 1):
                OT[k, h, i] = _pv(P[k, h][0], kv_ref(k, 1), h, i)

        def o_forms(o):
            return [_combine(f, lambda i, j: o[i, j]).astype(_BF16) for f in ao.a_forms]

        def do_pf(k):
            t0, t1 = [[OT.pop((k, h, i)) for i in range(3)] for h in range(2)]
            l0, l1 = P.pop((k, 0))[1], P.pop((k, 1))[1]
            if k < T - 1:
                put_o(_pv_finish(t0, t1, l0, l1))
            elif kind == "end":
                O[k] = o_forms(_pv_finish(t0, t1, l0, l1))
            else:
                for r, v in enumerate(t0 + t1 + l0 + l1):
                    o_scr[r] = v

        def do_o(k):
            br, b, p = task(k)
            forms = O.pop(k) if k in O else o_forms(
                {(i, j): f_scr[3 * i + j] for i in range(2) for j in range(3)})
            a = acc.at[br, b]
            c = _bilinear(
                ao, lambda f: forms[ao.a_forms.index(f)],
                lambda f: _unpack(woc[p & 1, br, ao.b_forms.index(f)]),
                {(i, j): tile(a, i, j, hm) for i in range(2) for j in range(d // 128)},
                cut=cuts[br])
            keep, emit = (emit_prev is not True, emit_prev) if k == -1 else (not last, True)
            if keep:
                for (i, j), v in c.items():
                    a[i * hm:(i + 1) * hm, j * 128:(j + 1) * 128] = v
            if last:
                for i in range(2):
                    row = jnp.concatenate([c[i, j] for j in range(d // 128)], axis=1)
                    ostage[b, i * hm:(i + 1) * hm, br * d:(br + 1) * d] = row.astype(ostage.dtype)
                if br == 1:
                    @when(emit)
                    def _():
                        pltpu.make_async_copy(ostage.at[b], out.at[b], o_sem.at[0]).start()

        def do_w(k):
            br, b, p = task(k)
            pc = jnp.minimum(p + shr(b, lg - 1), n_pair - 1)
            if n >= 4 and half == 8:
                w_forms(br, pc, b & 4, (k // 2) & 3)
            else:
                for i in range(8 // half):
                    w_forms(br, pc, (b & (half - 1)) * (8 // half) + i)

        ops = {"q": do_q, "a": lambda k: do_qk(k, 0), "b": lambda k: do_qk(k, 1),
               "u": lambda k: do_pv(k, 0), "v": lambda k: do_pv(k, 1), "f": do_pf,
               "o": lambda k: do_o(k - 1), "d": refill, "w": do_w,
               "x": lambda k: x_forms(*task(k)[:2], G[k]),
               "y": lambda k: x_balance(*task(k + 2)[:2])}
        for k in range(T):
            for c in (last_order if k == T - 1 else first_order if k == 0 else mid_order):
                ops[c](k)
        if kind == "end":
            do_o(T - 1)
        if not last:
            p2 = shr(u0, lg) + 2

            @when((u0 & (nb - 1)) == (3 * nb // 4 // n) * n, p2 < n_pair)
            def _():
                w_start(p2)

    zero_ref[0] = 0
    w0 = [x_copy(0, 0, p_sem.at[0]), x_copy(1, 0, p_sem.at[0]),
          wq_copy(0, 0, p_sem.at[0]), wq_copy(0, 1, p_sem.at[0]),
          wo_copy(0, 0, p_sem.at[0]), wo_copy(0, 1, p_sem.at[0])]
    for c in w0:
        c.start()
    issue(0, 0, True, False)

    def zero(b, carry):
        for br in range(2):
            acc[br, b] = jnp.zeros((sq, d), _F32)
        return carry
    jax.lax.fori_loop(0, nb, zero, 0)
    o_scr[0:6] = jnp.zeros((6,) + o_scr.shape[1:], _F32)
    o_scr[6:10] = jnp.ones((4,) + o_scr.shape[1:], _F32)
    for c in w0:
        c.wait()

    def w_first(si, carry):
        for br in range(2):
            w_forms(br, 0, si)
        issue(0, 1, True, False, si == 0)
        return carry
    jax.lax.fori_loop(0, 8, w_first, 0)

    def x_first(br, carry):
        x_balance(br, 0)
        return carry
    jax.lax.fori_loop(0, 2, x_first, 0)

    def ramp(u, carry):
        fast = u < lead - 1
        g = u + 1 + jnp.minimum(u, lead - 1)

        def refill(k):
            if k == 0:
                issue(g, 0, True, False)
                issue(g, 1, True, False, fast)
            else:
                g1 = g + fast.astype(jnp.int32)
                issue(g1, 0, True, False, fast)
                issue(g1, 1, True, False)
        block(u, 1, "ramp", refill)

        @pl.when(u + 1 < u_main)
        def _():
            waits_for(u + 1, 1, True)
        return carry

    waits_for(0, 1, True)
    jax.lax.fori_loop(0, u_main, ramp, 0)

    def steady(u_start, cnt, kind):
        may_end = u_start + cnt * n_main + lead > n_pos

        def body(j, carry):
            u0 = u_start + j * n_main
            block(u0, n_main, kind, lambda k: issue(u0 + k // 2 + lead, k % 2, False, may_end),
                  emit_prev=(j > 0) if kind == "last" else False)
            waits_for(u0 + n_main, n_main, False)
            return carry
        jax.lax.fori_loop(0, cnt, body, 0)

    waits_for(u_main, n_main, False)
    if 1 in only:
        steady(u_main, (n_pos - nb - u_main) // n_main, "main")
    if 2 in only:
        steady(n_pos - nb, nb // n_main - 1, "last")
    if 3 in only:
        block(n_pos - n_main, n_main, "end", None, emit_prev=True)
    pltpu.make_async_copy(ostage, out, o_sem.at[0]).wait()


def _build(A_x, A_k_cache, A_v_cache, A_wq, A_wo, B_x, B_k_cache, B_v_cache, B_wq, B_wo, *,
           n_main=4, u_main=20, lead=5, w1_at=7, ring=16, interpret=False,
           algq=None, algo=None, cuts=(48, 48), only=(0, 1, 2, 3), **ties):
    nb, sq, d = A_x.shape
    n_head, sk = A_k_cache.shape[1], A_k_cache.shape[2]
    n_pair = n_head // 2

    def tr(c):
        return jnp.swapaxes(c, 2, 3).reshape(nb, n_head * _DH, sk)

    aq = _Alg([algq[0][i] for i in algq[1]] if algq else _ALG_Q, 4)
    ao = _Alg([algo[0][i] for i in algo[1]] if algo else _ALG_O, 3)
    plan = {k: v[:3] + tuple(ties.get(k, v[3:])) for k, v in _PLAN.items()}
    u32 = jnp.uint32
    n_xf = -(-len(aq.a_forms) // 4) * 4
    return pl.pallas_call(
        functools.partial(_kernel, aq=aq, ao=ao, plan=plan, cuts=cuts, n_main=n_main,
                          u_main=u_main, lead=lead, w1_at=w1_at, only=only),
        in_specs=[pl.BlockSpec(memory_space=pl.ANY)] * 10,
        out_specs=pl.BlockSpec(memory_space=pl.ANY),
        out_shape=jax.ShapeDtypeStruct((nb, sq, 2 * d), A_x.dtype),
        scratch_shapes=[
            pltpu.VMEM((2, nb, 192, d), _BF16),
            pltpu.VMEM((n_pair, 2, d, _PAIR), _BF16),
            pltpu.VMEM((n_pair, 2, _PAIR, d), _BF16),
            pltpu.VMEM((2, nb, sq, d), _F32),
            pltpu.VMEM((nb, sq, 2 * d), _BF16),
            pltpu.VMEM((ring, 4, _PAIR, sk), _BF16),
            pltpu.VMEM((10, sq // 2, 128), _F32),
            pltpu.VMEM((2, nb, n_xf, sq // 4, 128), u32),
            pltpu.VMEM((2, 2, len(aq.b_forms), 64, 128), u32),
            pltpu.VMEM((2, 2, len(ao.b_forms), 64, 128), u32),
            pltpu.VMEM((6, sq // 2, 128), _F32),
            pltpu.VMEM((2, nb, 96, 128), _F32),
            pltpu.SMEM((1,), jnp.int32),
            pltpu.SemaphoreType.DMA((ring + ring // n_main,)),
            pltpu.SemaphoreType.DMA((2,)),
            pltpu.SemaphoreType.DMA((1,)),
            pltpu.SemaphoreType.DMA((1,)),
        ],
        compiler_params=pltpu.CompilerParams(
            vmem_limit_bytes=122 * 1024 * 1024, disable_bounds_checks=True),
        interpret=interpret,
    )(A_x, tr(A_k_cache), tr(A_v_cache), A_wq, A_wo,
      B_x, tr(B_k_cache), tr(B_v_cache), B_wq, B_wo)


@jax.jit
def pallas_concat_heads__gqa_block_cached__mha_block_cached__near_ridge_kernel(
    A_x: jax.Array,
    A_k_cache: jax.Array,
    A_v_cache: jax.Array,
    A_wq: jax.Array,
    A_wo: jax.Array,
    B_x: jax.Array,
    B_k_cache: jax.Array,
    B_v_cache: jax.Array,
    B_wq: jax.Array,
    B_wo: jax.Array,
):
    return _build(A_x, A_k_cache, A_v_cache, A_wq, A_wo,
                  B_x, B_k_cache, B_v_cache, B_wq, B_wo)
```

```python
import functools
import math

import jax
import jax.numpy as jnp
import jax.experimental.pallas as pl
import jax.experimental.pallas.tpu as pltpu

_DH = 192
_PAIR = 2 * _DH
_NT = (((1,), (1,)), ((), ()))
_F32 = jnp.float32
_BF16 = jnp.bfloat16
_SCALE = (_DH ** -0.5) * math.log2(math.e)

_ALG_Q = (
    (((1, 4, 1),), ((3, 2, -1), (4, 0, 1), (4, 1, -1), (4, 2, 1)), ((1, 0, 1), (1, 1, 1), (1, 2, 1))),
    (((0, 3, 1), (1, 3, -1), (1, 4, -1)), ((3, 2, -1), (4, 1, -1), (4, 2, 1)), ((0, 2, -1), (1, 0, 1), (1, 1, 1))),
    (((1, 1, 1), (1, 2, -1)), ((2, 0, 1),), ((1, 0, -1), (1, 2, -1))),
    (((0, 3, -1), (1, 3, 1)), ((3, 1, 1), (3, 2, -1), (4, 1, -1), (4, 2, 1)), ((1, 0, 1), (1, 1, 1))),
    (((0, 3, -1), (1, 0, 1)), ((0, 0, 1), (3, 0, 1), (3, 1, -1)), ((0, 1, 1), (1, 0, 1), (1, 1, 1))),
    (((1, 1, 1),), ((1, 0, 1), (2, 0, 1)), ((0, 0, 1), (1, 0, 1))),
    (((0, 3, 1),), ((0, 0, 1), (3, 0, 1)), ((0, 0, 1), (0, 1, 1), (1, 0, 1), (1, 1, 1))),
    (((1, 0, 1), (1, 3, -1)), ((3, 0, -1), (3, 1, 1)), ((1, 0, 1),)),
    (((0, 3, 1), (0, 4, 1), (1, 3, -1), (1, 4, -1)), ((4, 1, 1), (4, 2, -1)), ((0, 2, -1),)),
    (((1, 3, 1), (1, 4, 1)), ((3, 2, 1),), ((0, 2, 1), (1, 2, 1))),
    (((0, 2, -1), (1, 2, 1)), ((2, 0, -1), (2, 1, -1), (2, 2, 1)), ((1, 2, 1),)),
    (((0, 2, 1),), ((0, 2, -1), (1, 1, -1), (1, 2, 1), (2, 2, 1)), ((0, 2, 1), (1, 2, 1))),
    (((0, 2, 1), (1, 0, 1)), ((0, 2, 1), (2, 1, -1)), ((0, 1, -1), (1, 2, 1))),
    (((1, 0, 1),), ((0, 0, -1), (0, 1, 1), (2, 1, -1), (3, 0, -1), (3, 1, 1)), ((0, 1, 1), (1, 1, 1))),
    (((0, 1, -1), (0, 4, 1)), ((1, 1, 1),), ((0, 1, -1), (0, 2, -1), (1, 1, -1), (1, 2, -1))),
    (((0, 0, 1), (1, 0, -1)), ((0, 1, 1), (0, 2, -1)), ((0, 1, 1),)),
    (((1, 0, 1), (1, 2, 1)), ((2, 1, 1),), ((1, 1, 1), (1, 2, 1))),
    (((0, 1, -1), (0, 4, 1), (1, 1, 1)), ((1, 1, 1), (4, 0, -1), (4, 1, 1)), ((0, 0, -1), (1, 1, 1), (1, 2, 1))),
    (((0, 1, -1), (0, 4, 1), (1, 1, 1), (1, 4, -1)), ((4, 0, 1), (4, 1, -1)), ((1, 1, 1), (1, 2, 1))),
    (((0, 2, -1), (1, 1, 1)), ((1, 1, 1), (1, 2, -1), (2, 0, -1)), ((0, 0, 1), (1, 2, -1))),
    (((0, 1, 1), (1, 1, -1)), ((1, 0, 1), (1, 2, -1), (4, 0, 1), (4, 1, -1)), ((0, 0, 1),)),
    (((0, 4, 1),), ((1, 1, 1), (4, 1, 1)), ((0, 0, 1), (0, 1, 1), (0, 2, 1))),
    (((0, 0, 1), (0, 2, 1)), ((0, 2, 1),), ((0, 1, 1), (0, 2, 1))),
    (((0, 1, 1), (0, 2, -1)), ((1, 1, -1), (1, 2, 1)), ((0, 0, 1), (0, 2, 1))),
    (((0, 0, 1), (0, 3, -1)), ((0, 0, 1),), ((0, 0, 1),)),
)
_ALG_O = (
    (((1, 0, 1), (1, 2, -1)), ((0, 0, 1), (1, 0, 1)), ((1, 0, 1), (1, 2, -1))),
    (((0, 0, 1), (1, 0, -1)), ((0, 0, 1), (0, 2, 1), (0, 3, -1), (1, 0, 1)), ((1, 2, -1),)),
    (((0, 1, 1),), ((0, 1, 1), (0, 4, 1), (1, 1, 1), (1, 4, 1)), ((0, 1, 1),)),
    (((0, 0, -1), (0, 1, 1), (1, 0, 1)), ((0, 1, -1), (0, 4, -1), (1, 4, -1)), ((0, 1, 1), (0, 4, -1), (1, 4, -1))),
    (((0, 0, 1), (0, 1, -1)), ((0, 1, 1), (0, 4, 1), (2, 4, 1)), ((0, 4, 1), (1, 4, 1))),
    (((1, 0, 1),), ((0, 1, 1),), ((0, 1, 1), (0, 4, -1), (1, 1, 1), (1, 4, -1))),
    (((1, 1, 1),), ((1, 1, 1), (1, 3, -1), (2, 1, -1), (2, 3, 1)), ((1, 1, 1),)),
    (((0, 2, 1),), ((2, 1, 1),), ((0, 1, 1), (0, 3, 1), (1, 1, 1), (1, 3, 1))),
    (((0, 2, 1), (1, 2, -1)), ((1, 3, 1), (2, 3, -1)), ((1, 1, 1), (1, 3, 1))),
    (((1, 1, 1), (1, 2, 1)), ((0, 3, 1), (2, 1, -1), (2, 3, 1)), ((0, 3, 1), (1, 3, 1))),
    (((0, 2, 1), (1, 1, -1), (1, 2, -1)), ((1, 3, -1), (2, 1, -1), (2, 3, 1)), ((0, 3, 1), (1, 1, 1), (1, 3, 1))),
    (((1, 0, 1), (1, 1, -1), (1, 2, -1)), ((0, 3, 1),), ((1, 2, 1), (1, 3, 1))),
    (((0, 2, 1), (1, 2, -1)), ((1, 2, -1), (2, 0, 1), (2, 2, 1), (2, 4, 1)), ((0, 0, 1),)),
    (((0, 0, -1), (1, 2, 1)), ((0, 0, -1), (1, 0, -1), (1, 2, -1), (2, 2, 1)), ((0, 0, 1), (1, 2, 1))),
    (((0, 0, 1), (0, 2, -1)), ((1, 2, -1), (2, 2, 1)), ((0, 0, 1), (0, 2, -1))),
    (((0, 1, 1), (0, 2, 1), (1, 1, -1), (1, 2, -1)), ((1, 2, -1), (1, 3, 1)), ((0, 3, 1),)),
    (((0, 0, 1), (1, 1, -1), (1, 2, -1)), ((0, 3, -1), (1, 2, -1)), ((0, 3, -1), (1, 2, 1))),
    (((0, 0, 1),), ((0, 2, 1), (2, 2, 1)), ((0, 2, 1), (1, 2, 1))),
    (((0, 0, -1), (0, 1, 1), (0, 2, 1)), ((1, 2, 1),), ((0, 2, 1), (0, 3, 1))),
    (((1, 0, -1), (1, 1, 1), (1, 2, 1)), ((1, 0, -1),), ((1, 0, -1), (1, 4, 1))),
    (((0, 0, 1), (0, 1, -1), (1, 0, -1), (1, 1, 1)), ((1, 0, -1), (1, 4, -1)), ((1, 4, -1),)),
    (((0, 0, 1), (0, 1, -1), (1, 2, -1)), ((1, 0, -1), (2, 4, -1)), ((0, 0, 1), (1, 4, 1))),
    (((1, 2, 1),), ((0, 0, 1), (2, 0, 1)), ((0, 0, 1), (1, 0, 1))),
    (((0, 0, -1), (0, 1, 1), (0, 2, 1)), ((2, 4, 1),), ((0, 0, -1), (0, 4, 1))),
    (((0, 0, -1), (1, 0, 1)), ((0, 4, 1), (1, 4, 1)), ((0, 1, 1), (0, 4, -1))),
)

_PLAN = {
    "ramp": ("xqdwyoabuvf", "", "dxqwyoabuvf", None, 6, 3),
    "main": ("qdwoabuvf", "dqwoabuvf", "dqwoabuvf", 4, 6, 6),
    "last": ("qdoabuvf", "dqoabuvf", "dqoabuvf", None, 6, 6),
    "end": ("qoabuvf", "qoabuvf", "qabuvfo", None, 6, 3),
}


class _Alg:
    def __init__(self, table, lead):
        def norm(t):
            sg = t[0][2]
            return tuple((i, j, c * sg) for i, j, c in t), sg
        starts = [0] + list(range(lead, len(table), 4)) + [len(table)]
        self.rounds = list(zip(starts[:-1], starts[1:]))
        self.a_forms, self.b_forms, self.prods = [], [], []
        for a, b, c in table:
            (a, sa), (b, sb) = norm(a), norm(b)
            if a not in self.a_forms:
                self.a_forms.append(a)
            if b not in self.b_forms:
                self.b_forms.append(b)
            self.prods.append((a, b, tuple((i, j, v * sa * sb) for i, j, v in c)))


def _dot(a, b):
    return jnp.dot(a, b, preferred_element_type=_F32)


def _nt(a, b):
    return jax.lax.dot_general(a, b, _NT, preferred_element_type=_F32)


def _combine(form, get):
    r = get(form[0][0], form[0][1])
    for i, j, c in form[1:]:
        r = r + get(i, j) if c > 0 else r - get(i, j)
    return r


def _signed_add(d, key, v, sg):
    if key not in d:
        d[key] = (v, sg)
    else:
        w, sw = d[key]
        d[key] = (w + v if sg == sw else w - v, sw)


def _round(prods, out):
    groups, part = {}, {}
    for m, c in prods:
        sg = c[0][2]
        _signed_add(groups, tuple((i, j, v * sg) for i, j, v in c), m, sg)
    for c, (tot, tsg) in groups.items():
        for i, j, v in c:
            _signed_add(part, (i, j), tot, v * tsg)
    for key, (v, sg) in part.items():
        if key not in out:
            out[key] = v if sg > 0 else -v
        else:
            out[key] = out[key] + v if sg > 0 else out[key] - v


def _bilinear(alg, a_of, b_of, out, tie=None, cut=None):
    for rnd, (r0, r1) in enumerate(alg.rounds):
        prods = []
        for a, b, c in alg.prods[r0:r1]:
            av, bv = a_of(a), b_of(b)
            if tie is not None and rnd == tie[0] and not prods:
                bv = _tie(bv, tie[1]())
            if cut is not None and len(alg.prods) - r0 == 2:
                m = jnp.concatenate([_dot(av[0:cut], bv), _dot(av[cut:], bv)], axis=0)
            else:
                m = _dot(av, bv)
            prods.append((m, c))
        _round(prods, out)
    return out


def _pack(v):
    return pltpu.bitcast(v, jnp.uint32)


def _unpack(v):
    return pltpu.bitcast(v, _BF16)


def _tie(v, words):
    u = _pack(v)
    return _unpack(jnp.concatenate([u[0:8] | words, u[8:]], axis=0))


def _lo(n):
    return jax.lax.broadcasted_iota(jnp.int32, (n, 128), 1) < 64


def _q_forms(c):
    a, b = [[c[m, n] * _SCALE for n in range(3)] for m in range(2)]
    lo = _lo(a[0].shape[0])
    rolled = pltpu.roll(b[1], 64, 1)
    forms = []
    for t, own in ((0, lo), (2, jnp.logical_not(lo))):
        t3 = jnp.where(own, a[t], b[t]).astype(_BF16)
        t3f = t3.astype(_F32)
        forms.append((t3,
                      jnp.where(own, a[1], a[t] - t3f).astype(_BF16),
                      jnp.where(own, b[t] - t3f, rolled).astype(_BF16)))
    return forms


def _qk_pass(af, kt, h, i):
    rows = (((0, 64), (128, 64), (0, 128)), ((256, 320), (256, 192), (192, 320)))[h][i]
    if i == 0:
        w = kt[rows[0]:rows[0] + 128]
    else:
        w = jnp.concatenate([kt[r:r + 64] for r in rows], axis=0)
    return _dot(af[i], w)


def _scores(af, kt, h):
    t = [_qk_pass(af, kt, h, i) for i in range(3)]
    return t[1] + t[0], t[2] + t[0]


def _softmax(s, g):
    s = (s[0], s[1] * jnp.concatenate([g] * 4, axis=1))
    es = [jnp.exp2(c - jnp.max(c, axis=-1, keepdims=True)) for c in s]
    parts = [(e[:, 0:128] + e[:, 128:256]) + (e[:, 256:384] + e[:, 384:512]) for e in es]
    return (es[0].astype(_BF16), es[1].astype(_BF16), (es[0] + es[1]).astype(_BF16)), parts


def _pv(p, vt, h, i):
    lo, hi, e = ((0, 64, 128), (256, 320, 192))[h]
    rows = (((e, hi), (lo, e), (lo, hi)), ((lo, e), (e, hi), (lo, hi)))[h][i]
    if rows == (lo, hi):
        w = vt[lo:lo + 128]
    else:
        w = jnp.concatenate([vt[r:r + 64] for r in rows], axis=0)
    return _nt(p[i], w)


def _pv_finish(t0, t1, l0, l1):
    r0, r1 = [[pl.reciprocal(jnp.sum(v, axis=-1, keepdims=True), approx=True) for v in l]
              for l in (l0, l1)]
    lo = _lo(t0[0].shape[0])
    d0 = jnp.where(lo, t0[1], t0[0])
    e0 = t0[2] - d0
    d1 = jnp.where(lo, t1[0], t1[1])
    e1 = t1[2] - d1
    return {(0, 0): jnp.where(lo, e0, d0) * r0[0],
            (1, 0): jnp.where(lo, d0, e0) * r0[1],
            (0, 1): jnp.where(lo, t0[0], t1[0]) * jnp.where(lo, r0[0], r1[0]),
            (1, 1): pltpu.roll(jnp.where(lo, t1[1], t0[1]), 64, 1) * jnp.where(lo, r0[1], r1[1]),
            (0, 2): jnp.where(lo, d1, e1) * r1[0],
            (1, 2): jnp.where(lo, e1, d1) * r1[1]}


def _kernel(xa, ka, va, wqa, woa, xb, kb, vb, wqb, wob, out,
            x_res, wq_res, wo_res, acc, ostage, kv, o_scr, xc, wqc, woc, f_scr, x_scale,
            zero_ref, g_sem, w_sem, p_sem, o_sem, *, aq, ao, plan, cuts, n_main, u_main, lead,
            w1_at, only):
    n_pair, nb, ring = wq_res.shape[0], acc.shape[1], kv.shape[0]
    sq, d = acc.shape[2], acc.shape[3]
    lg = nb.bit_length() - 1
    lg_main = n_main.bit_length() - 1
    half, hm = nb // 2, sq // 2
    n_pos = n_pair * nb
    assert nb == 1 << lg and n_main == 1 << lg_main and half % n_main == 0 and 8 % half == 0
    assert u_main >= nb and u_main % n_main == 0
    assert n_main < lead < ring and lead <= u_main and w1_at < half

    def static(v):
        return isinstance(v, int)

    def shr(v, s):
        return v >> s if static(v) else jax.lax.shift_right_logical(v, s)

    def aligned(v, m):
        return v if static(v) else pl.multiple_of(v, m)

    def clamp(u, hi=n_pos - 1):
        return min(max(u, 0), hi) if static(u) else jnp.clip(u, 0, hi)

    def when(*conds):
        dyn = [c for c in conds if not isinstance(c, bool)]
        if not all(c for c in conds if isinstance(c, bool)):
            return lambda f: None
        if not dyn:
            return lambda f: f()
        return pl.when(functools.reduce(jnp.logical_and, dyn))

    def pair_ds(p):
        return pl.ds(aligned(p * _PAIR, _PAIR), _PAIR)

    def sem_of(u, early):
        late = ring + (shr(u, lg_main) & (ring // n_main - 1))
        if static(u):
            return u & (ring - 1) if u < u_main else late
        return jnp.where(u < u_main, u & (ring - 1), late) if early else late

    def x_copy(br, b, sem):
        return pltpu.make_async_copy((xa, xb)[br].at[b], x_res.at[br, b, 0:sq], sem)

    def issue(u, h, early, may_end, enable=True):
        uc = clamp(u) if may_end else u
        sem = g_sem.at[sem_of(uc, early)]
        if early:
            ux = clamp(u + 1, nb - 1)

            @when(enable, u + 1 < nb)
            def _():
                x_copy(h, ux, sem).start()
        for i, ref in enumerate(((ka, va), (kb, vb))[h]):
            src = ref.at[uc & (nb - 1), pair_ds(shr(uc, lg)), :]

            @when(enable, (u < n_pos) if may_end else True)
            def _():
                pltpu.make_async_copy(src, kv.at[uc & (ring - 1), 2 * h + i], sem).start()
        if early and h == 1:
            @when(enable, u == w1_at)
            def _():
                w_start(1)

    def wq_copy(p, br, sem):
        return pltpu.make_async_copy((wqa, wqb)[br].at[:, pair_ds(p)], wq_res.at[p, br], sem)

    def wo_copy(p, br, sem):
        return pltpu.make_async_copy((woa, wob)[br].at[pair_ds(p), :], wo_res.at[p, br], sem)

    def w_start(p):
        for br in range(2):
            wq_copy(p, br, w_sem.at[p & 1]).start()
            wo_copy(p, br, w_sem.at[p & 1]).start()

    def waits_for(u0, n, early):
        blk = kv.at[pl.ds(aligned(u0 & (ring - 1), n), n)]
        sem = g_sem.at[u0 & (ring - 1) if early else sem_of(u0, False)]
        pltpu.make_async_copy(blk, blk, sem).wait()
        if early:
            @when(u0 + 1 < nb)
            def _():
                for br in range(2):
                    x_copy(br, u0 + 1, sem).wait()
        p1 = shr(u0, lg) + 1

        @when((u0 & (nb - 1)) == half, p1 < n_pair)
        def _():
            for ref in (wq_res, wo_res):
                pltpu.make_async_copy(ref.at[p1], ref.at[p1], w_sem.at[p1 & 1]).wait()

    def tile(ref, i, j, rows):
        return ref[i * rows:(i + 1) * rows, j * 128:(j + 1) * 128]

    def x_balance(br, b):
        m = [jnp.broadcast_to(jnp.max(jnp.abs(x_res[br, b, i * hm:(i + 1) * hm, :].astype(_F32)),
                                      axis=-1, keepdims=True), (hm, 128)) for i in range(2)]
        ratio = m[1] * pl.reciprocal(m[0], approx=True) * math.sqrt(2.0)
        ratio = jnp.where(jnp.logical_and(m[0] > 0, m[1] > 0), ratio, 1.0)
        e = jnp.clip(pltpu.bitcast(ratio, jnp.int32) & 0x7f800000, 0x20000000, 0x5f000000)
        x_scale[br, b, 0:hm] = pltpu.bitcast(e, _F32)

    def x_forms(br, b, g):
        inv = pltpu.bitcast(0x7f000000 - pltpu.bitcast(g, jnp.int32), _F32)
        x = x_res.at[br, b]
        blk = {}
        for j in range(d // 128):
            blk[0, j] = tile(x, 0, j, hm).astype(_F32)
            blk[1, j] = tile(x, 1, j, hm).astype(_F32) * inv
        for r, f in enumerate(aq.a_forms):
            xc[br, b, r] = _pack(tile(x, 0, f[0][1], hm) if len(f) == 1 and f[0][0] == 0
                                 else _combine(f, lambda i, j: blk[i, j]).astype(_BF16))

    def w_forms(br, p, si, lo=0):
        for raw, dst, alg in ((wq_res, wqc, aq), (wo_res, woc, ao)):
            view = raw.at[p, br, pl.ds(aligned(si * 16, 16), raw.shape[2] - 112 + 16 * lo)]
            rows = pl.ds(aligned((si + lo) * 8, 8), 8)
            blk = {}

            def src(i, j):
                return view[i * 128 + lo * 16:i * 128 + lo * 16 + 16, j * 128:(j + 1) * 128]

            def get(i, j):
                if (i, j) not in blk:
                    blk[i, j] = src(i, j).astype(_F32)
                return blk[i, j]
            for r, f in enumerate(alg.b_forms):
                dst[p & 1, br, r, rows, :] = _pack(
                    src(f[0][0], f[0][1]) if len(f) == 1 else _combine(f, get).astype(_BF16))

    def block(u0, n, kind, refill, emit_prev=False):
        T = 2 * n
        last = kind in ("last", "end")
        first_order, mid_order, last_order, tie_w, tie_f, tie_f0 = plan[kind]
        zero_idx = zero_ref[0]
        zero_vec = jnp.full((8, 128), zero_idx, jnp.int32).astype(jnp.uint32)

        def task(k):
            u = u0 + k // 2
            if k == -1 and kind == "ramp":
                u = clamp(u)
            return k % 2, u & (nb - 1), shr(u, lg)

        def kv_ref(k, i):
            return kv.at[(u0 + k // 2) & (ring - 1), 2 * (k % 2) + i]

        def put_o(o):
            for (i, j), v in o.items():
                f_scr[3 * i + j] = v

        Q, S, P, OT, O = {}, {}, {}, {}, {}
        G = {k: x_scale[k % 2, task(k)[1], 0:hm] for k in range(T)} if kind == "ramp" else {}
        put_o(_pv_finish(*[[o_scr[r] for r in rr]
                           for rr in ((0, 1, 2), (3, 4, 5), (6, 7), (8, 9))]))

        def do_q(k):
            br, b, p = task(k)
            tie = (tie_f if k > 0 else tie_f0,
                   lambda: pltpu.bitcast(f_scr[zero_idx, 0:8], jnp.uint32) & zero_vec)
            Q[k, 0], Q[k, 1] = _q_forms(_bilinear(
                aq, lambda f: _unpack(xc[br, b, aq.a_forms.index(f)]),
                lambda f: _unpack(wqc[p & 1, br, aq.b_forms.index(f)]), {}, tie))

        def do_qk(k, h):
            af = Q.pop((k, h))
            if tie_w is not None and tie_w // 3 == h:
                br, _, p = task(k)
                for ref in (wqc, woc):
                    words = ref[p & 1, br, 0, 0:8] & zero_vec
                    af = tuple(_tie(v, words) if i == tie_w % 3 else v for i, v in enumerate(af))
            S[k, h] = _scores(af, kv_ref(k, 0), h)

        def do_pv(k, h):
            br, b, _ = task(k)
            P[k, h] = _softmax(S.pop((k, h)), G[k] if k in G else x_scale[br, b, 0:hm])
            for i in (0, 2, 1):
                OT[k, h, i] = _pv(P[k, h][0], kv_ref(k, 1), h, i)

        def o_forms(o):
            return [_combine(f, lambda i, j: o[i, j]).astype(_BF16) for f in ao.a_forms]

        def do_pf(k):
            t0, t1 = [[OT.pop((k, h, i)) for i in range(3)] for h in range(2)]
            l0, l1 = P.pop((k, 0))[1], P.pop((k, 1))[1]
            if k < T - 1:
                put_o(_pv_finish(t0, t1, l0, l1))
            elif kind == "end":
                O[k] = o_forms(_pv_finish(t0, t1, l0, l1))
            else:
                for r, v in enumerate(t0 + t1 + l0 + l1):
                    o_scr[r] = v

        def do_o(k):
            br, b, p = task(k)
            forms = O.pop(k) if k in O else o_forms(
                {(i, j): f_scr[3 * i + j] for i in range(2) for j in range(3)})
            a = acc.at[br, b]
            c = _bilinear(
                ao, lambda f: forms[ao.a_forms.index(f)],
                lambda f: _unpack(woc[p & 1, br, ao.b_forms.index(f)]),
                {(i, j): tile(a, i, j, hm) for i in range(2) for j in range(d // 128)},
                cut=cuts[br])
            keep, emit = (emit_prev is not True, emit_prev) if k == -1 else (not last, True)
            if keep:
                for (i, j), v in c.items():
                    a[i * hm:(i + 1) * hm, j * 128:(j + 1) * 128] = v
            if last:
                for i in range(2):
                    row = jnp.concatenate([c[i, j] for j in range(d // 128)], axis=1)
                    ostage[b, i * hm:(i + 1) * hm, br * d:(br + 1) * d] = row.astype(ostage.dtype)
                if br == 1:
                    @when(emit)
                    def _():
                        pltpu.make_async_copy(ostage.at[b], out.at[b], o_sem.at[0]).start()

        def do_w(k):
            br, b, p = task(k)
            pc = jnp.minimum(p + shr(b, lg - 1), n_pair - 1)
            if n >= 4 and half == 8:
                w_forms(br, pc, b & 4, (k // 2) & 3)
            else:
                for i in range(8 // half):
                    w_forms(br, pc, (b & (half - 1)) * (8 // half) + i)

        ops = {"q": do_q, "a": lambda k: do_qk(k, 0), "b": lambda k: do_qk(k, 1),
               "u": lambda k: do_pv(k, 0), "v": lambda k: do_pv(k, 1), "f": do_pf,
               "o": lambda k: do_o(k - 1), "d": refill, "w": do_w,
               "x": lambda k: x_forms(*task(k)[:2], G[k]),
               "y": lambda k: x_balance(*task(k + 2)[:2])}
        for k in range(T):
            for c in (last_order if k == T - 1 else first_order if k == 0 else mid_order):
                ops[c](k)
        if kind == "end":
            do_o(T - 1)
        if not last:
            p2 = shr(u0, lg) + 2

            @when((u0 & (nb - 1)) == (3 * nb // 4 // n) * n, p2 < n_pair)
            def _():
                w_start(p2)

    zero_ref[0] = 0
    w0 = [x_copy(0, 0, p_sem.at[0]), x_copy(1, 0, p_sem.at[0]),
          wq_copy(0, 0, p_sem.at[0]), wq_copy(0, 1, p_sem.at[0]),
          wo_copy(0, 0, p_sem.at[0]), wo_copy(0, 1, p_sem.at[0])]
    for c in w0:
        c.start()
    issue(0, 0, True, False)

    def zero(b, carry):
        for br in range(2):
            acc[br, b] = jnp.zeros((sq, d), _F32)
        return carry
    jax.lax.fori_loop(0, nb, zero, 0)
    o_scr[0:6] = jnp.zeros((6,) + o_scr.shape[1:], _F32)
    o_scr[6:10] = jnp.ones((4,) + o_scr.shape[1:], _F32)
    for c in w0:
        c.wait()

    def w_first(si, carry):
        for br in range(2):
            w_forms(br, 0, si)
        issue(0, 1, True, False, si == 0)
        return carry
    jax.lax.fori_loop(0, 8, w_first, 0)

    def x_first(br, carry):
        x_balance(br, 0)
        return carry
    jax.lax.fori_loop(0, 2, x_first, 0)

    def ramp(u, carry):
        fast = u < lead - 1
        g = u + 1 + jnp.minimum(u, lead - 1)

        def refill(k):
            if k == 0:
                issue(g, 0, True, False)
                issue(g, 1, True, False, fast)
            else:
                g1 = g + fast.astype(jnp.int32)
                issue(g1, 0, True, False, fast)
                issue(g1, 1, True, False)
        block(u, 1, "ramp", refill)

        @pl.when(u + 1 < u_main)
        def _():
            waits_for(u + 1, 1, True)
        return carry

    waits_for(0, 1, True)
    jax.lax.fori_loop(0, u_main, ramp, 0)

    def steady(u_start, cnt, kind):
        may_end = u_start + cnt * n_main + lead > n_pos

        def body(j, carry):
            u0 = u_start + j * n_main
            block(u0, n_main, kind, lambda k: issue(u0 + k // 2 + lead, k % 2, False, may_end),
                  emit_prev=(j > 0) if kind == "last" else False)
            waits_for(u0 + n_main, n_main, False)
            return carry
        jax.lax.fori_loop(0, cnt, body, 0)

    waits_for(u_main, n_main, False)
    if 1 in only:
        steady(u_main, (n_pos - nb - u_main) // n_main, "main")
    if 2 in only:
        steady(n_pos - nb, nb // n_main - 1, "last")
    if 3 in only:
        block(n_pos - n_main, n_main, "end", None, emit_prev=True)
    pltpu.make_async_copy(ostage, out, o_sem.at[0]).wait()


def _build(A_x, A_k_cache, A_v_cache, A_wq, A_wo, B_x, B_k_cache, B_v_cache, B_wq, B_wo, *,
           n_main=4, u_main=24, lead=6, w1_at=7, ring=16, interpret=False,
           algq=None, algo=None, cuts=(48, 48), only=(0, 1, 2, 3), **ties):
    nb, sq, d = A_x.shape
    n_head, sk = A_k_cache.shape[1], A_k_cache.shape[2]
    n_pair = n_head // 2

    def tr(c):
        return jnp.swapaxes(c, 2, 3).reshape(nb, n_head * _DH, sk)

    aq = _Alg([algq[0][i] for i in algq[1]] if algq else _ALG_Q, 4)
    ao = _Alg([algo[0][i] for i in algo[1]] if algo else _ALG_O, 3)
    plan = {k: v[:3] + tuple(ties.get(k, v[3:])) for k, v in _PLAN.items()}
    u32 = jnp.uint32
    n_xf = -(-len(aq.a_forms) // 4) * 4
    return pl.pallas_call(
        functools.partial(_kernel, aq=aq, ao=ao, plan=plan, cuts=cuts, n_main=n_main,
                          u_main=u_main, lead=lead, w1_at=w1_at, only=only),
        in_specs=[pl.BlockSpec(memory_space=pl.ANY)] * 10,
        out_specs=pl.BlockSpec(memory_space=pl.ANY),
        out_shape=jax.ShapeDtypeStruct((nb, sq, 2 * d), A_x.dtype),
        scratch_shapes=[
            pltpu.VMEM((2, nb, 192, d), _BF16),
            pltpu.VMEM((n_pair, 2, d, _PAIR), _BF16),
            pltpu.VMEM((n_pair, 2, _PAIR, d), _BF16),
            pltpu.VMEM((2, nb, sq, d), _F32),
            pltpu.VMEM((nb, sq, 2 * d), _BF16),
            pltpu.VMEM((ring, 4, _PAIR, sk), _BF16),
            pltpu.VMEM((10, sq // 2, 128), _F32),
            pltpu.VMEM((2, nb, n_xf, sq // 4, 128), u32),
            pltpu.VMEM((2, 2, len(aq.b_forms), 64, 128), u32),
            pltpu.VMEM((2, 2, len(ao.b_forms), 64, 128), u32),
            pltpu.VMEM((6, sq // 2, 128), _F32),
            pltpu.VMEM((2, nb, 96, 128), _F32),
            pltpu.SMEM((1,), jnp.int32),
            pltpu.SemaphoreType.DMA((ring + ring // n_main,)),
            pltpu.SemaphoreType.DMA((2,)),
            pltpu.SemaphoreType.DMA((1,)),
            pltpu.SemaphoreType.DMA((1,)),
        ],
        compiler_params=pltpu.CompilerParams(
            vmem_limit_bytes=122 * 1024 * 1024, disable_bounds_checks=True),
        interpret=interpret,
    )(A_x, tr(A_k_cache), tr(A_v_cache), A_wq, A_wo,
      B_x, tr(B_k_cache), tr(B_v_cache), B_wq, B_wo)


@jax.jit
def pallas_concat_heads__gqa_block_cached__mha_block_cached__near_ridge_kernel(
    A_x: jax.Array,
    A_k_cache: jax.Array,
    A_v_cache: jax.Array,
    A_wq: jax.Array,
    A_wo: jax.Array,
    B_x: jax.Array,
    B_k_cache: jax.Array,
    B_v_cache: jax.Array,
    B_wq: jax.Array,
    B_wo: jax.Array,
):
    return _build(A_x, A_k_cache, A_v_cache, A_wq, A_wo,
                  B_x, B_k_cache, B_v_cache, B_wq, B_wo)
```

```python
import functools
import math

import jax
import jax.numpy as jnp
import jax.experimental.pallas as pl
import jax.experimental.pallas.tpu as pltpu

_DH = 192
_PAIR = 2 * _DH
_NT = (((1,), (1,)), ((), ()))
_F32 = jnp.float32
_BF16 = jnp.bfloat16
_SCALE = (_DH ** -0.5) * math.log2(math.e)

_ALG_Q = (
    (((0, 3, 1), (1, 3, -1), (1, 4, -1)), ((3, 2, -1), (4, 1, -1), (4, 2, 1)), ((0, 2, -1), (1, 0, 1), (1, 1, 1))),
    (((1, 4, 1),), ((3, 2, -1), (4, 0, 1), (4, 1, -1), (4, 2, 1)), ((1, 0, 1), (1, 1, 1), (1, 2, 1))),
    (((1, 1, 1), (1, 2, -1)), ((2, 0, 1),), ((1, 0, -1), (1, 2, -1))),
    (((0, 3, -1), (1, 3, 1)), ((3, 1, 1), (3, 2, -1), (4, 1, -1), (4, 2, 1)), ((1, 0, 1), (1, 1, 1))),
    (((0, 3, -1), (1, 0, 1)), ((0, 0, 1), (3, 0, 1), (3, 1, -1)), ((0, 1, 1), (1, 0, 1), (1, 1, 1))),
    (((1, 1, 1),), ((1, 0, 1), (2, 0, 1)), ((0, 0, 1), (1, 0, 1))),
    (((0, 3, 1),), ((0, 0, 1), (3, 0, 1)), ((0, 0, 1), (0, 1, 1), (1, 0, 1), (1, 1, 1))),
    (((1, 0, 1), (1, 3, -1)), ((3, 0, -1), (3, 1, 1)), ((1, 0, 1),)),
    (((0, 3, 1), (0, 4, 1), (1, 3, -1), (1, 4, -1)), ((4, 1, 1), (4, 2, -1)), ((0, 2, -1),)),
    (((1, 3, 1), (1, 4, 1)), ((3, 2, 1),), ((0, 2, 1), (1, 2, 1))),
    (((0, 2, -1), (1, 2, 1)), ((2, 0, -1), (2, 1, -1), (2, 2, 1)), ((1, 2, 1),)),
    (((0, 2, 1),), ((0, 2, -1), (1, 1, -1), (1, 2, 1), (2, 2, 1)), ((0, 2, 1), (1, 2, 1))),
    (((0, 2, 1), (1, 0, 1)), ((0, 2, 1), (2, 1, -1)), ((0, 1, -1), (1, 2, 1))),
    (((1, 0, 1),), ((0, 0, -1), (0, 1, 1), (2, 1, -1), (3, 0, -1), (3, 1, 1)), ((0, 1, 1), (1, 1, 1))),
    (((0, 1, -1), (0, 4, 1)), ((1, 1, 1),), ((0, 1, -1), (0, 2, -1), (1, 1, -1), (1, 2, -1))),
    (((0, 0, 1), (1, 0, -1)), ((0, 1, 1), (0, 2, -1)), ((0, 1, 1),)),
    (((1, 0, 1), (1, 2, 1)), ((2, 1, 1),), ((1, 1, 1), (1, 2, 1))),
    (((0, 1, -1), (0, 4, 1), (1, 1, 1)), ((1, 1, 1), (4, 0, -1), (4, 1, 1)), ((0, 0, -1), (1, 1, 1), (1, 2, 1))),
    (((0, 1, -1), (0, 4, 1), (1, 1, 1), (1, 4, -1)), ((4, 0, 1), (4, 1, -1)), ((1, 1, 1), (1, 2, 1))),
    (((0, 2, -1), (1, 1, 1)), ((1, 1, 1), (1, 2, -1), (2, 0, -1)), ((0, 0, 1), (1, 2, -1))),
    (((0, 1, 1), (1, 1, -1)), ((1, 0, 1), (1, 2, -1), (4, 0, 1), (4, 1, -1)), ((0, 0, 1),)),
    (((0, 4, 1),), ((1, 1, 1), (4, 1, 1)), ((0, 0, 1), (0, 1, 1), (0, 2, 1))),
    (((0, 0, 1), (0, 2, 1)), ((0, 2, 1),), ((0, 1, 1), (0, 2, 1))),
    (((0, 1, 1), (0, 2, -1)), ((1, 1, -1), (1, 2, 1)), ((0, 0, 1), (0, 2, 1))),
    (((0, 0, 1), (0, 3, -1)), ((0, 0, 1),), ((0, 0, 1),)),
)
_ALG_O = (
    (((1, 0, 1), (1, 2, -1)), ((0, 0, 1), (1, 0, 1)), ((1, 0, 1), (1, 2, -1))),
    (((0, 0, 1), (1, 0, -1)), ((0, 0, 1), (0, 2, 1), (0, 3, -1), (1, 0, 1)), ((1, 2, -1),)),
    (((0, 1, 1),), ((0, 1, 1), (0, 4, 1), (1, 1, 1), (1, 4, 1)), ((0, 1, 1),)),
    (((0, 0, -1), (0, 1, 1), (1, 0, 1)), ((0, 1, -1), (0, 4, -1), (1, 4, -1)), ((0, 1, 1), (0, 4, -1), (1, 4, -1))),
    (((0, 0, -1), (1, 0, 1)), ((0, 4, 1), (1, 4, 1)), ((0, 1, 1), (0, 4, -1))),
    (((1, 0, 1),), ((0, 1, 1),), ((0, 1, 1), (0, 4, -1), (1, 1, 1), (1, 4, -1))),
    (((1, 1, 1),), ((1, 1, 1), (1, 3, -1), (2, 1, -1), (2, 3, 1)), ((1, 1, 1),)),
    (((0, 2, 1),), ((2, 1, 1),), ((0, 1, 1), (0, 3, 1), (1, 1, 1), (1, 3, 1))),
    (((0, 2, 1), (1, 2, -1)), ((1, 3, 1), (2, 3, -1)), ((1, 1, 1), (1, 3, 1))),
    (((1, 1, 1), (1, 2, 1)), ((0, 3, 1), (2, 1, -1), (2, 3, 1)), ((0, 3, 1), (1, 3, 1))),
    (((0, 2, 1), (1, 1, -1), (1, 2, -1)), ((1, 3, -1), (2, 1, -1), (2, 3, 1)), ((0, 3, 1), (1, 1, 1), (1, 3, 1))),
    (((1, 0, 1), (1, 1, -1), (1, 2, -1)), ((0, 3, 1),), ((1, 2, 1), (1, 3, 1))),
    (((0, 2, 1), (1, 2, -1)), ((1, 2, -1), (2, 0, 1), (2, 2, 1), (2, 4, 1)), ((0, 0, 1),)),
    (((0, 0, -1), (1, 2, 1)), ((0, 0, -1), (1, 0, -1), (1, 2, -1), (2, 2, 1)), ((0, 0, 1), (1, 2, 1))),
    (((0, 0, 1), (0, 2, -1)), ((1, 2, -1), (2, 2, 1)), ((0, 0, 1), (0, 2, -1))),
    (((0, 0, 1), (1, 1, -1), (1, 2, -1)), ((0, 3, -1), (1, 2, -1)), ((0, 3, -1), (1, 2, 1))),
    (((0, 1, 1), (0, 2, 1), (1, 1, -1), (1, 2, -1)), ((1, 2, -1), (1, 3, 1)), ((0, 3, 1),)),
    (((0, 0, 1),), ((0, 2, 1), (2, 2, 1)), ((0, 2, 1), (1, 2, 1))),
    (((0, 0, -1), (0, 1, 1), (0, 2, 1)), ((1, 2, 1),), ((0, 2, 1), (0, 3, 1))),
    (((1, 0, -1), (1, 1, 1), (1, 2, 1)), ((1, 0, -1),), ((1, 0, -1), (1, 4, 1))),
    (((0, 0, 1), (0, 1, -1), (1, 0, -1), (1, 1, 1)), ((1, 0, -1), (1, 4, -1)), ((1, 4, -1),)),
    (((0, 0, 1), (0, 1, -1), (1, 2, -1)), ((1, 0, -1), (2, 4, -1)), ((0, 0, 1), (1, 4, 1))),
    (((1, 2, 1),), ((0, 0, 1), (2, 0, 1)), ((0, 0, 1), (1, 0, 1))),
    (((0, 0, -1), (0, 1, 1), (0, 2, 1)), ((2, 4, 1),), ((0, 0, -1), (0, 4, 1))),
    (((0, 0, 1), (0, 1, -1)), ((0, 1, 1), (0, 4, 1), (2, 4, 1)), ((0, 4, 1), (1, 4, 1))),
)

_PLAN = {
    "ramp": ("xqdwyoabuvf", "", "dxqwyoabuvf", None, 6, 3),
    "main": ("qdwoabuvf", "dqwoabuvf", "dqwoabuvf", 4, 6, 6),
    "big": ("qdwoabuvf", "dqwoabuvf", "dqwoabuvf", 4, 6, 6),
    "last": ("qdoabuvf", "dqoabuvf", "dqoabuvf", None, 6, 6),
    "end": ("qoabuvf", "qoabuvf", "qoabuvf", None, 5, 3),
}


class _Alg:
    def __init__(self, table, lead):
        def norm(t):
            sg = t[0][2]
            return tuple((i, j, c * sg) for i, j, c in t), sg
        starts = [0] + list(range(lead, len(table), 4)) + [len(table)]
        self.rounds = list(zip(starts[:-1], starts[1:]))
        self.a_forms, self.b_forms, self.prods = [], [], []
        for a, b, c in table:
            (a, sa), (b, sb) = norm(a), norm(b)
            if a not in self.a_forms:
                self.a_forms.append(a)
            if b not in self.b_forms:
                self.b_forms.append(b)
            self.prods.append((a, b, tuple((i, j, v * sa * sb) for i, j, v in c)))


def _dot(a, b):
    return jnp.dot(a, b, preferred_element_type=_F32)


def _nt(a, b):
    return jax.lax.dot_general(a, b, _NT, preferred_element_type=_F32)


def _combine(form, get):
    r = get(form[0][0], form[0][1])
    for i, j, c in form[1:]:
        r = r + get(i, j) if c > 0 else r - get(i, j)
    return r


def _signed_add(d, key, v, sg):
    if key not in d:
        d[key] = (v, sg)
    else:
        w, sw = d[key]
        d[key] = (w + v if sg == sw else w - v, sw)


def _round(prods, out):
    groups, part = {}, {}
    for m, c in prods:
        sg = c[0][2]
        _signed_add(groups, tuple((i, j, v * sg) for i, j, v in c), m, sg)
    for c, (tot, tsg) in groups.items():
        for i, j, v in c:
            _signed_add(part, (i, j), tot, v * tsg)
    for key, (v, sg) in part.items():
        if key not in out:
            out[key] = v if sg > 0 else -v
        else:
            out[key] = out[key] + v if sg > 0 else out[key] - v


def _bilinear(alg, a_of, b_of, out, tie=None, cut=None):
    for rnd, (r0, r1) in enumerate(alg.rounds):
        prods = []
        for a, b, c in alg.prods[r0:r1]:
            av, bv = a_of(a), b_of(b)
            if tie is not None and rnd == tie[0] and not prods:
                bv = _tie(bv, tie[1]())
            if cut is not None and len(alg.prods) - r0 == 2:
                m = jnp.concatenate([_dot(av[0:cut], bv), _dot(av[cut:], bv)], axis=0)
            else:
                m = _dot(av, bv)
            prods.append((m, c))
        _round(prods, out)
    return out


def _pack(v):
    return pltpu.bitcast(v, jnp.uint32)


def _unpack(v):
    return pltpu.bitcast(v, _BF16)


def _tie(v, words):
    u = _pack(v)
    return _unpack(jnp.concatenate([u[0:8] | words, u[8:]], axis=0))


def _lo(n):
    return jax.lax.broadcasted_iota(jnp.int32, (n, 128), 1) < 64


def _q_forms(c):
    a, b = [[c[m, n] * _SCALE for n in range(3)] for m in range(2)]
    lo = _lo(a[0].shape[0])
    rolled = pltpu.roll(b[1], 64, 1)
    forms = []
    for t, own in ((0, lo), (2, jnp.logical_not(lo))):
        t3 = jnp.where(own, a[t], b[t]).astype(_BF16)
        t3f = t3.astype(_F32)
        forms.append((t3,
                      jnp.where(own, a[1], a[t] - t3f).astype(_BF16),
                      jnp.where(own, b[t] - t3f, rolled).astype(_BF16)))
    return forms


def _qk_pass(af, kt, h, i):
    rows = (((0, 64), (128, 64), (0, 128)), ((256, 320), (256, 192), (192, 320)))[h][i]
    if i == 0:
        w = kt[rows[0]:rows[0] + 128]
    else:
        w = jnp.concatenate([kt[r:r + 64] for r in rows], axis=0)
    return _dot(af[i], w)


def _scores(af, kt, h):
    t = [_qk_pass(af, kt, h, i) for i in range(3)]
    return t[1] + t[0], t[2] + t[0]


def _softmax(s, g):
    s = (s[0], s[1] * jnp.concatenate([g] * 4, axis=1))
    es = [jnp.exp2(c - jnp.max(c, axis=-1, keepdims=True)) for c in s]
    parts = [(e[:, 0:128] + e[:, 128:256]) + (e[:, 256:384] + e[:, 384:512]) for e in es]
    return (es[0].astype(_BF16), es[1].astype(_BF16), (es[0] + es[1]).astype(_BF16)), parts


def _pv(p, vt, h, i):
    lo, hi, e = ((0, 64, 128), (256, 320, 192))[h]
    rows = (((e, hi), (lo, e), (lo, hi)), ((lo, e), (e, hi), (lo, hi)))[h][i]
    if rows == (lo, hi):
        w = vt[lo:lo + 128]
    else:
        w = jnp.concatenate([vt[r:r + 64] for r in rows], axis=0)
    return _nt(p[i], w)


def _pv_finish(t0, t1, l0, l1):
    r0, r1 = [[pl.reciprocal(jnp.sum(v, axis=-1, keepdims=True), approx=True) for v in l]
              for l in (l0, l1)]
    lo = _lo(t0[0].shape[0])
    d0 = jnp.where(lo, t0[1], t0[0])
    e0 = t0[2] - d0
    d1 = jnp.where(lo, t1[0], t1[1])
    e1 = t1[2] - d1
    return {(0, 0): jnp.where(lo, e0, d0) * r0[0],
            (1, 0): jnp.where(lo, d0, e0) * r0[1],
            (0, 1): jnp.where(lo, t0[0], t1[0]) * jnp.where(lo, r0[0], r1[0]),
            (1, 1): pltpu.roll(jnp.where(lo, t1[1], t0[1]), 64, 1) * jnp.where(lo, r0[1], r1[1]),
            (0, 2): jnp.where(lo, d1, e1) * r1[0],
            (1, 2): jnp.where(lo, e1, d1) * r1[1]}


def _kernel(xa, ka, va, wqa, woa, xb, kb, vb, wqb, wob, out,
            x_res, wq_res, wo_res, acc, ostage, kv, o_scr, xc, wqc, woc, f_scr, x_scale,
            zero_ref, g_sem, w_sem, p_sem, o_sem, *, aq, ao, n_main, u_main, lead, u_big,
            extra, w1_at):
    n_pair, nb, ring = wq_res.shape[0], acc.shape[1], kv.shape[0]
    sq, d = acc.shape[2], acc.shape[3]
    lg = nb.bit_length() - 1
    lg_main = n_main.bit_length() - 1
    half, hm = nb // 2, sq // 2
    n_pos = n_pair * nb
    assert nb == 1 << lg and n_main == 1 << lg_main and half % n_main == 0 and 8 % half == 0
    assert u_main >= nb and u_main % n_main == 0
    assert n_main < lead < ring and lead <= u_main and w1_at < half

    def static(v):
        return isinstance(v, int)

    def shr(v, s):
        return v >> s if static(v) else jax.lax.shift_right_logical(v, s)

    def aligned(v, m):
        return v if static(v) else pl.multiple_of(v, m)

    def clamp(u, hi=n_pos - 1):
        return min(max(u, 0), hi) if static(u) else jnp.clip(u, 0, hi)

    def when(*conds):
        dyn = [c for c in conds if not isinstance(c, bool)]
        if not all(c for c in conds if isinstance(c, bool)):
            return lambda f: None
        if not dyn:
            return lambda f: f()
        return pl.when(functools.reduce(jnp.logical_and, dyn))

    def pair_ds(p):
        return pl.ds(aligned(p * _PAIR, _PAIR), _PAIR)

    def sem_of(u, early):
        late = ring + (shr(u, lg_main) & (ring // n_main - 1))
        if static(u):
            return u & (ring - 1) if u < u_main else late
        return jnp.where(u < u_main, u & (ring - 1), late) if early else late

    def x_copy(br, b, sem):
        return pltpu.make_async_copy((xa, xb)[br].at[b], x_res.at[br, b, 0:sq], sem)

    def issue(u, h, early, may_end, enable=True):
        uc = clamp(u) if may_end else u
        sem = g_sem.at[sem_of(uc, early)]
        if early:
            ux = clamp(u + 1, nb - 1)

            @when(enable, u + 1 < nb)
            def _():
                x_copy(h, ux, sem).start()
        for i, ref in enumerate(((ka, va), (kb, vb))[h]):
            src = ref.at[uc & (nb - 1), pair_ds(shr(uc, lg)), :]

            @when(enable, (u < n_pos) if may_end else True)
            def _():
                pltpu.make_async_copy(src, kv.at[uc & (ring - 1), 2 * h + i], sem).start()
        if early and h == 1:
            @when(enable, u == w1_at)
            def _():
                w_start(1)

    def wq_copy(p, br, sem):
        return pltpu.make_async_copy((wqa, wqb)[br].at[:, pair_ds(p)], wq_res.at[p, br], sem)

    def wo_copy(p, br, sem):
        return pltpu.make_async_copy((woa, wob)[br].at[pair_ds(p), :], wo_res.at[p, br], sem)

    def w_start(p):
        for br in range(2):
            wq_copy(p, br, w_sem.at[p & 1]).start()
            wo_copy(p, br, w_sem.at[p & 1]).start()

    def waits_for(u0, n, early, big=False):
        g = min(n, n_main)
        for u in [u0 + i for i in range(0, n, g)]:
            blk = kv.at[pl.ds(aligned(u & (ring - 1), g), g)]
            sem = g_sem.at[u & (ring - 1) if early else sem_of(u, False)]
            pltpu.make_async_copy(blk, blk, sem).wait()
        if early:
            @when(u0 + 1 < nb)
            def _():
                for br in range(2):
                    x_copy(br, u0 + 1, sem).wait()
        p1 = shr(u0, lg) + 1

        @when((u0 & (nb - 1)) == (0 if big else half), p1 < n_pair)
        def _():
            for ref in (wq_res, wo_res):
                pltpu.make_async_copy(ref.at[p1], ref.at[p1], w_sem.at[p1 & 1]).wait()

    def tile(ref, i, j, rows):
        return ref[i * rows:(i + 1) * rows, j * 128:(j + 1) * 128]

    def x_balance(br, b):
        m = [jnp.broadcast_to(jnp.max(jnp.abs(x_res[br, b, i * hm:(i + 1) * hm, :].astype(_F32)),
                                      axis=-1, keepdims=True), (hm, 128)) for i in range(2)]
        ratio = m[1] * pl.reciprocal(m[0], approx=True) * math.sqrt(2.0)
        ratio = jnp.where(jnp.logical_and(m[0] > 0, m[1] > 0), ratio, 1.0)
        e = jnp.clip(pltpu.bitcast(ratio, jnp.int32) & 0x7f800000, 0x20000000, 0x5f000000)
        x_scale[br, b, 0:hm] = pltpu.bitcast(e, _F32)

    def x_forms(br, b, g):
        inv = pltpu.bitcast(0x7f000000 - pltpu.bitcast(g, jnp.int32), _F32)
        x = x_res.at[br, b]
        blk = {}
        for j in range(d // 128):
            blk[0, j] = tile(x, 0, j, hm).astype(_F32)
            blk[1, j] = tile(x, 1, j, hm).astype(_F32) * inv
        for r, f in enumerate(aq.a_forms):
            xc[br, b, r] = _pack(tile(x, 0, f[0][1], hm) if len(f) == 1 and f[0][0] == 0
                                 else _combine(f, lambda i, j: blk[i, j]).astype(_BF16))

    def w_forms(br, p, si, lo=0):
        for raw, dst, alg in ((wq_res, wqc, aq), (wo_res, woc, ao)):
            view = raw.at[p, br, pl.ds(aligned(si * 16, 16), raw.shape[2] - 112 + 16 * lo)]
            rows = pl.ds(aligned((si + lo) * 8, 8), 8)
            blk = {}

            def src(i, j):
                return view[i * 128 + lo * 16:i * 128 + lo * 16 + 16, j * 128:(j + 1) * 128]

            def get(i, j):
                if (i, j) not in blk:
                    blk[i, j] = src(i, j).astype(_F32)
                return blk[i, j]
            for r, f in enumerate(alg.b_forms):
                dst[p & 1, br, r, rows, :] = _pack(
                    src(f[0][0], f[0][1]) if len(f) == 1 else _combine(f, get).astype(_BF16))

    def block(u0, n, kind, refill, emit_prev=False):
        T = 2 * n
        last = kind in ("last", "end")
        first_order, mid_order, last_order, tie_w, tie_f, tie_f0 = _PLAN[kind]
        zero_idx = zero_ref[0]
        zero_vec = jnp.full((8, 128), zero_idx, jnp.int32).astype(jnp.uint32)

        def task(k):
            u = u0 + k // 2
            if k == -1 and kind == "ramp":
                u = clamp(u)
            return k % 2, u & (nb - 1), shr(u, lg)

        def kv_ref(k, i):
            return kv.at[(u0 + k // 2) & (ring - 1), 2 * (k % 2) + i]

        def put_o(o):
            for (i, j), v in o.items():
                f_scr[3 * i + j] = v

        Q, S, P, OT, O = {}, {}, {}, {}, {}
        G = {k: x_scale[k % 2, task(k)[1], 0:hm] for k in range(T)} if kind == "ramp" else {}
        put_o(_pv_finish(*[[o_scr[r] for r in rr]
                           for rr in ((0, 1, 2), (3, 4, 5), (6, 7), (8, 9))]))

        def do_q(k):
            br, b, p = task(k)
            tie = (tie_f if k > 0 else tie_f0,
                   lambda: pltpu.bitcast(f_scr[zero_idx, 0:8], jnp.uint32) & zero_vec)
            Q[k, 0], Q[k, 1] = _q_forms(_bilinear(
                aq, lambda f: _unpack(xc[br, b, aq.a_forms.index(f)]),
                lambda f: _unpack(wqc[p & 1, br, aq.b_forms.index(f)]), {}, tie))

        def do_qk(k, h):
            af = Q.pop((k, h))
            if tie_w is not None and tie_w // 3 == h and (kind != "big" or k < n):
                br, _, p = task(k)
                for ref in (wqc, woc):
                    words = ref[p & 1, br, 0, 0:8] & zero_vec
                    af = tuple(_tie(v, words) if i == tie_w % 3 else v for i, v in enumerate(af))
            S[k, h] = _scores(af, kv_ref(k, 0), h)

        def do_pv(k, h):
            br, b, _ = task(k)
            P[k, h] = _softmax(S.pop((k, h)), G[k] if k in G else x_scale[br, b, 0:hm])
            for i in (0, 2, 1):
                OT[k, h, i] = _pv(P[k, h][0], kv_ref(k, 1), h, i)

        def o_forms(o):
            return [_combine(f, lambda i, j: o[i, j]).astype(_BF16) for f in ao.a_forms]

        def do_pf(k):
            t0, t1 = [[OT.pop((k, h, i)) for i in range(3)] for h in range(2)]
            l0, l1 = P.pop((k, 0))[1], P.pop((k, 1))[1]
            if k < T - 1:
                put_o(_pv_finish(t0, t1, l0, l1))
            elif kind == "end":
                O[k] = o_forms(_pv_finish(t0, t1, l0, l1))
            else:
                for r, v in enumerate(t0 + t1 + l0 + l1):
                    o_scr[r] = v

        def do_o(k):
            br, b, p = task(k)
            forms = O.pop(k) if k in O else o_forms(
                {(i, j): f_scr[3 * i + j] for i in range(2) for j in range(3)})
            a = acc.at[br, b]
            c = _bilinear(
                ao, lambda f: forms[ao.a_forms.index(f)],
                lambda f: _unpack(woc[p & 1, br, ao.b_forms.index(f)]),
                {(i, j): tile(a, i, j, hm) for i in range(2) for j in range(d // 128)},
                cut=48)
            keep, emit = (emit_prev is not True, emit_prev) if k == -1 else (not last, True)
            if keep:
                for (i, j), v in c.items():
                    a[i * hm:(i + 1) * hm, j * 128:(j + 1) * 128] = v
            if last:
                for i in range(2):
                    row = jnp.concatenate([c[i, j] for j in range(d // 128)], axis=1)
                    ostage[b, i * hm:(i + 1) * hm, br * d:(br + 1) * d] = row.astype(ostage.dtype)
                if br == 1:
                    @when(emit)
                    def _():
                        pltpu.make_async_copy(ostage.at[b], out.at[b], o_sem.at[0]).start()

        def do_w(k):
            br, b, p = task(k)
            per = 8 // half
            if kind == "big":
                if k < n:
                    for i in range(per):
                        u = u0 + k // 2 + zero_idx
                        si = shr(u & half, lg - 3) if lg >= 3 else (u & half) * (4 // half)
                        w_forms(br, shr(u, lg) + 1, si, (k // 2) * per + i)
                return
            pc = jnp.minimum(p + shr(b, lg - 1), n_pair - 1)
            if n >= 4 and half == 8:
                w_forms(br, pc, b & 4, (k // 2) & 3)
            else:
                for i in range(per):
                    w_forms(br, pc, (b & (half - 1)) * per + i)

        ops = {"q": do_q, "a": lambda k: do_qk(k, 0), "b": lambda k: do_qk(k, 1),
               "u": lambda k: do_pv(k, 0), "v": lambda k: do_pv(k, 1), "f": do_pf,
               "o": lambda k: do_o(k - 1), "d": refill, "w": do_w,
               "x": lambda k: x_forms(*task(k)[:2], G[k]),
               "y": lambda k: x_balance(*task(k + 2)[:2])}
        for k in range(T):
            for c in (last_order if k == T - 1 else first_order if k == 0 else mid_order):
                ops[c](k)
        if kind == "end":
            do_o(T - 1)
        if not last:
            p2 = shr(u0, lg) + 2

            @when((u0 & (nb - 1)) == {"ramp": 3 * nb // 4, "main": half, "big": 0}[kind],
                  p2 < n_pair)
            def _():
                w_start(p2)

    zero_ref[0] = 0
    w0 = [x_copy(0, 0, p_sem.at[0]), x_copy(1, 0, p_sem.at[0]),
          wq_copy(0, 0, p_sem.at[0]), wq_copy(0, 1, p_sem.at[0]),
          wo_copy(0, 0, p_sem.at[0]), wo_copy(0, 1, p_sem.at[0])]
    for c in w0:
        c.start()
    issue(0, 0, True, False)

    def zero(b, carry):
        for br in range(2):
            acc[br, b] = jnp.zeros((sq, d), _F32)
        return carry
    jax.lax.fori_loop(0, nb, zero, 0)
    o_scr[0:6] = jnp.zeros((6,) + o_scr.shape[1:], _F32)
    o_scr[6:10] = jnp.ones((4,) + o_scr.shape[1:], _F32)
    for c in w0:
        c.wait()

    def w_first(si, carry):
        for br in range(2):
            w_forms(br, 0, si)
        issue(0, 1, True, False, si == 0)
        return carry
    jax.lax.fori_loop(0, 8, w_first, 0)

    def x_first(br, carry):
        x_balance(br, 0)
        return carry
    jax.lax.fori_loop(0, 2, x_first, 0)

    def ramp(u, carry):
        fast = u < lead - 1
        g = u + 1 + jnp.minimum(u, lead - 1)

        def refill(k):
            if k == 0:
                issue(g, 0, True, False)
                issue(g, 1, True, False, fast)
            else:
                g1 = g + fast.astype(jnp.int32)
                issue(g1, 0, True, False, fast)
                issue(g1, 1, True, False)
        block(u, 1, "ramp", refill)

        @pl.when(u + 1 < u_main)
        def _():
            waits_for(u + 1, 1, True)
        return carry

    waits_for(0, 1, True)
    jax.lax.fori_loop(0, u_main, ramp, 0)

    def steady(u_start, n, cnt, n_next, lead, extra, kind):
        may_end = u_start + cnt * n + lead + extra > n_pos

        def body(j, carry):
            u0 = u_start + j * n

            def refill(k):
                u, h = u0 + k // 2 + lead, k % 2
                if k // 2 < extra:
                    fast = j == 1
                    g = u + jnp.where(j > 1, extra, jnp.where(fast, k // 2 + h, 0))
                    issue(g, 0, False, may_end, fast if h == 1 else True)
                    issue(g, 1, False, may_end, fast if h == 0 else True)
                else:
                    issue(u + (jnp.where(j >= 1, extra, 0) if extra else 0), h, False, may_end)
            block(u0, n, kind, refill, emit_prev=(j > 0) if kind == "last" else False)

            @when((j + 1 < cnt) if n != n_next else True)
            def _():
                waits_for(u0 + n, n, False, kind == "big")
            return carry
        jax.lax.fori_loop(0, cnt, body, 0)
        if n != n_next:
            waits_for(u_start + cnt * n, n_next, False, n_next > n)

    n_big = 2 * n_main
    assert n_big == half and u_big % nb == 0 and u_big - u_main >= n_big
    assert extra <= n_main and n_big < lead + extra < ring
    assert not half < (u_main & (nb - 1)) <= 3 * nb // 4 and u_big < n_pos - nb
    waits_for(u_main, n_main, False)
    steady(u_main, n_main, (u_big - u_main) // n_main, n_big, lead, extra, "main")
    steady(u_big, n_big, (n_pos - nb - u_big) // n_big, n_main, lead + extra, 0, "big")
    steady(n_pos - nb, n_main, nb // n_main - 1, n_main, lead + extra, 0, "last")
    block(n_pos - n_main, n_main, "end", None, emit_prev=True)
    pltpu.make_async_copy(ostage, out, o_sem.at[0]).wait()


def _build(A_x, A_k_cache, A_v_cache, A_wq, A_wo, B_x, B_k_cache, B_v_cache, B_wq, B_wo, *,
           n_main=4, u_main=24, lead=6, u_big=48, extra=4, w1_at=7, ring=16,
           interpret=False):
    nb, sq, d = A_x.shape
    n_head, sk = A_k_cache.shape[1], A_k_cache.shape[2]
    n_pair = n_head // 2

    def tr(c):
        return jnp.swapaxes(c, 2, 3).reshape(nb, n_head * _DH, sk)

    aq, ao = _Alg(_ALG_Q, 4), _Alg(_ALG_O, 3)
    u32 = jnp.uint32
    n_xf = -(-len(aq.a_forms) // 4) * 4
    return pl.pallas_call(
        functools.partial(_kernel, aq=aq, ao=ao, n_main=n_main, u_main=u_main, lead=lead,
                          u_big=u_big, extra=extra, w1_at=w1_at),
        in_specs=[pl.BlockSpec(memory_space=pl.ANY)] * 10,
        out_specs=pl.BlockSpec(memory_space=pl.ANY),
        out_shape=jax.ShapeDtypeStruct((nb, sq, 2 * d), A_x.dtype),
        scratch_shapes=[
            pltpu.VMEM((2, nb, 192, d), _BF16),
            pltpu.VMEM((n_pair, 2, d, _PAIR), _BF16),
            pltpu.VMEM((n_pair, 2, _PAIR, d), _BF16),
            pltpu.VMEM((2, nb, sq, d), _F32),
            pltpu.VMEM((nb, sq, 2 * d), _BF16),
            pltpu.VMEM((ring, 4, _PAIR, sk), _BF16),
            pltpu.VMEM((10, sq // 2, 128), _F32),
            pltpu.VMEM((2, nb, n_xf, sq // 4, 128), u32),
            pltpu.VMEM((2, 2, len(aq.b_forms), 64, 128), u32),
            pltpu.VMEM((2, 2, len(ao.b_forms), 64, 128), u32),
            pltpu.VMEM((6, sq // 2, 128), _F32),
            pltpu.VMEM((2, nb, 96, 128), _F32),
            pltpu.SMEM((1,), jnp.int32),
            pltpu.SemaphoreType.DMA((ring + ring // n_main,)),
            pltpu.SemaphoreType.DMA((2,)),
            pltpu.SemaphoreType.DMA((1,)),
            pltpu.SemaphoreType.DMA((1,)),
        ],
        compiler_params=pltpu.CompilerParams(
            vmem_limit_bytes=122 * 1024 * 1024, disable_bounds_checks=True),
        interpret=interpret,
    )(A_x, tr(A_k_cache), tr(A_v_cache), A_wq, A_wo,
      B_x, tr(B_k_cache), tr(B_v_cache), B_wq, B_wo)


@jax.jit
def pallas_concat_heads__gqa_block_cached__mha_block_cached__near_ridge_kernel(
    A_x: jax.Array,
    A_k_cache: jax.Array,
    A_v_cache: jax.Array,
    A_wq: jax.Array,
    A_wo: jax.Array,
    B_x: jax.Array,
    B_k_cache: jax.Array,
    B_v_cache: jax.Array,
    B_wq: jax.Array,
    B_wo: jax.Array,
):
    return _build(A_x, A_k_cache, A_v_cache, A_wq, A_wo,
                  B_x, B_k_cache, B_v_cache, B_wq, B_wo)
```

```python
import functools
import math

import jax
import jax.numpy as jnp
import jax.experimental.pallas as pl
import jax.experimental.pallas.tpu as pltpu

_DH = 192
_PAIR = 2 * _DH
_NT = (((1,), (1,)), ((), ()))
_F32 = jnp.float32
_BF16 = jnp.bfloat16
_SCALE = (_DH ** -0.5) * math.log2(math.e)

_ALG_Q = (
    (((0, 3, 1), (1, 3, -1), (1, 4, -1)), ((3, 2, -1), (4, 1, -1), (4, 2, 1)), ((0, 2, -1), (1, 0, 1), (1, 1, 1))),
    (((1, 4, 1),), ((3, 2, -1), (4, 0, 1), (4, 1, -1), (4, 2, 1)), ((1, 0, 1), (1, 1, 1), (1, 2, 1))),
    (((1, 1, 1), (1, 2, -1)), ((2, 0, 1),), ((1, 0, -1), (1, 2, -1))),
    (((0, 3, -1), (1, 3, 1)), ((3, 1, 1), (3, 2, -1), (4, 1, -1), (4, 2, 1)), ((1, 0, 1), (1, 1, 1))),
    (((0, 3, -1), (1, 0, 1)), ((0, 0, 1), (3, 0, 1), (3, 1, -1)), ((0, 1, 1), (1, 0, 1), (1, 1, 1))),
    (((1, 1, 1),), ((1, 0, 1), (2, 0, 1)), ((0, 0, 1), (1, 0, 1))),
    (((0, 3, 1),), ((0, 0, 1), (3, 0, 1)), ((0, 0, 1), (0, 1, 1), (1, 0, 1), (1, 1, 1))),
    (((1, 0, 1), (1, 3, -1)), ((3, 0, -1), (3, 1, 1)), ((1, 0, 1),)),
    (((0, 3, 1), (0, 4, 1), (1, 3, -1), (1, 4, -1)), ((4, 1, 1), (4, 2, -1)), ((0, 2, -1),)),
    (((1, 3, 1), (1, 4, 1)), ((3, 2, 1),), ((0, 2, 1), (1, 2, 1))),
    (((0, 2, -1), (1, 2, 1)), ((2, 0, -1), (2, 1, -1), (2, 2, 1)), ((1, 2, 1),)),
    (((0, 2, 1),), ((0, 2, -1), (1, 1, -1), (1, 2, 1), (2, 2, 1)), ((0, 2, 1), (1, 2, 1))),
    (((0, 2, 1), (1, 0, 1)), ((0, 2, 1), (2, 1, -1)), ((0, 1, -1), (1, 2, 1))),
    (((1, 0, 1),), ((0, 0, -1), (0, 1, 1), (2, 1, -1), (3, 0, -1), (3, 1, 1)), ((0, 1, 1), (1, 1, 1))),
    (((0, 1, -1), (0, 4, 1)), ((1, 1, 1),), ((0, 1, -1), (0, 2, -1), (1, 1, -1), (1, 2, -1))),
    (((0, 0, 1), (1, 0, -1)), ((0, 1, 1), (0, 2, -1)), ((0, 1, 1),)),
    (((1, 0, 1), (1, 2, 1)), ((2, 1, 1),), ((1, 1, 1), (1, 2, 1))),
    (((0, 1, -1), (0, 4, 1), (1, 1, 1)), ((1, 1, 1), (4, 0, -1), (4, 1, 1)), ((0, 0, -1), (1, 1, 1), (1, 2, 1))),
    (((0, 1, -1), (0, 4, 1), (1, 1, 1), (1, 4, -1)), ((4, 0, 1), (4, 1, -1)), ((1, 1, 1), (1, 2, 1))),
    (((0, 2, -1), (1, 1, 1)), ((1, 1, 1), (1, 2, -1), (2, 0, -1)), ((0, 0, 1), (1, 2, -1))),
    (((0, 1, 1), (1, 1, -1)), ((1, 0, 1), (1, 2, -1), (4, 0, 1), (4, 1, -1)), ((0, 0, 1),)),
    (((0, 4, 1),), ((1, 1, 1), (4, 1, 1)), ((0, 0, 1), (0, 1, 1), (0, 2, 1))),
    (((0, 0, 1), (0, 2, 1)), ((0, 2, 1),), ((0, 1, 1), (0, 2, 1))),
    (((0, 1, 1), (0, 2, -1)), ((1, 1, -1), (1, 2, 1)), ((0, 0, 1), (0, 2, 1))),
    (((0, 0, 1), (0, 3, -1)), ((0, 0, 1),), ((0, 0, 1),)),
)
_ALG_O = (
    (((1, 0, 1), (1, 2, -1)), ((0, 0, 1), (1, 0, 1)), ((1, 0, 1), (1, 2, -1))),
    (((0, 0, 1), (1, 0, -1)), ((0, 0, 1), (0, 2, 1), (0, 3, -1), (1, 0, 1)), ((1, 2, -1),)),
    (((0, 1, 1),), ((0, 1, 1), (0, 4, 1), (1, 1, 1), (1, 4, 1)), ((0, 1, 1),)),
    (((0, 0, -1), (0, 1, 1), (1, 0, 1)), ((0, 1, -1), (0, 4, -1), (1, 4, -1)), ((0, 1, 1), (0, 4, -1), (1, 4, -1))),
    (((0, 0, -1), (1, 0, 1)), ((0, 4, 1), (1, 4, 1)), ((0, 1, 1), (0, 4, -1))),
    (((1, 0, 1),), ((0, 1, 1),), ((0, 1, 1), (0, 4, -1), (1, 1, 1), (1, 4, -1))),
    (((1, 1, 1),), ((1, 1, 1), (1, 3, -1), (2, 1, -1), (2, 3, 1)), ((1, 1, 1),)),
    (((0, 2, 1),), ((2, 1, 1),), ((0, 1, 1), (0, 3, 1), (1, 1, 1), (1, 3, 1))),
    (((0, 2, 1), (1, 2, -1)), ((1, 3, 1), (2, 3, -1)), ((1, 1, 1), (1, 3, 1))),
    (((1, 1, 1), (1, 2, 1)), ((0, 3, 1), (2, 1, -1), (2, 3, 1)), ((0, 3, 1), (1, 3, 1))),
    (((0, 2, 1), (1, 1, -1), (1, 2, -1)), ((1, 3, -1), (2, 1, -1), (2, 3, 1)), ((0, 3, 1), (1, 1, 1), (1, 3, 1))),
    (((1, 0, 1), (1, 1, -1), (1, 2, -1)), ((0, 3, 1),), ((1, 2, 1), (1, 3, 1))),
    (((0, 2, 1), (1, 2, -1)), ((1, 2, -1), (2, 0, 1), (2, 2, 1), (2, 4, 1)), ((0, 0, 1),)),
    (((0, 0, -1), (1, 2, 1)), ((0, 0, -1), (1, 0, -1), (1, 2, -1), (2, 2, 1)), ((0, 0, 1), (1, 2, 1))),
    (((0, 0, 1), (0, 2, -1)), ((1, 2, -1), (2, 2, 1)), ((0, 0, 1), (0, 2, -1))),
    (((0, 0, 1), (1, 1, -1), (1, 2, -1)), ((0, 3, -1), (1, 2, -1)), ((0, 3, -1), (1, 2, 1))),
    (((0, 1, 1), (0, 2, 1), (1, 1, -1), (1, 2, -1)), ((1, 2, -1), (1, 3, 1)), ((0, 3, 1),)),
    (((0, 0, 1),), ((0, 2, 1), (2, 2, 1)), ((0, 2, 1), (1, 2, 1))),
    (((0, 0, -1), (0, 1, 1), (0, 2, 1)), ((1, 2, 1),), ((0, 2, 1), (0, 3, 1))),
    (((1, 0, -1), (1, 1, 1), (1, 2, 1)), ((1, 0, -1),), ((1, 0, -1), (1, 4, 1))),
    (((0, 0, 1), (0, 1, -1), (1, 0, -1), (1, 1, 1)), ((1, 0, -1), (1, 4, -1)), ((1, 4, -1),)),
    (((0, 0, 1), (0, 1, -1), (1, 2, -1)), ((1, 0, -1), (2, 4, -1)), ((0, 0, 1), (1, 4, 1))),
    (((1, 2, 1),), ((0, 0, 1), (2, 0, 1)), ((0, 0, 1), (1, 0, 1))),
    (((0, 0, -1), (0, 1, 1), (0, 2, 1)), ((2, 4, 1),), ((0, 0, -1), (0, 4, 1))),
    (((0, 0, 1), (0, 1, -1)), ((0, 1, 1), (0, 4, 1), (2, 4, 1)), ((0, 4, 1), (1, 4, 1))),
)

_PLAN = {
    "ramp": ("xqdwyoabuvf", "", "dxqwyoabuvf", None, 6, 3),
    "duo": ("qdwoabuvf", "dqwoabuvf", "dqwoabuvf", 4, 6, 6),
    "main": ("qdwoabuvf", "dqwoabuvf", "dqwoabuvf", 4, 6, 6),
    "big": ("qdwoabuvf", "dqwoabuvf", "dqwoabuvf", 4, 6, 6),
    "last": ("qdoabuvf", "dqoabuvf", "dqoabuvf", None, 6, 6),
    "end": ("qoabuvf", "qoabuvf", "qoabuvf", None, 5, 3),
}


class _Alg:
    def __init__(self, table, lead):
        def norm(t):
            sg = t[0][2]
            return tuple((i, j, c * sg) for i, j, c in t), sg
        starts = [0] + list(range(lead, len(table), 4)) + [len(table)]
        self.rounds = list(zip(starts[:-1], starts[1:]))
        self.a_forms, self.b_forms, self.prods = [], [], []
        for a, b, c in table:
            (a, sa), (b, sb) = norm(a), norm(b)
            if a not in self.a_forms:
                self.a_forms.append(a)
            if b not in self.b_forms:
                self.b_forms.append(b)
            self.prods.append((a, b, tuple((i, j, v * sa * sb) for i, j, v in c)))


def _dot(a, b):
    return jnp.dot(a, b, preferred_element_type=_F32)


def _nt(a, b):
    return jax.lax.dot_general(a, b, _NT, preferred_element_type=_F32)


def _combine(form, get):
    r = get(form[0][0], form[0][1])
    for i, j, c in form[1:]:
        r = r + get(i, j) if c > 0 else r - get(i, j)
    return r


def _signed_add(d, key, v, sg):
    if key not in d:
        d[key] = (v, sg)
    else:
        w, sw = d[key]
        d[key] = (w + v if sg == sw else w - v, sw)


def _round(prods, out):
    groups, part = {}, {}
    for m, c in prods:
        sg = c[0][2]
        _signed_add(groups, tuple((i, j, v * sg) for i, j, v in c), m, sg)
    for c, (tot, tsg) in groups.items():
        for i, j, v in c:
            _signed_add(part, (i, j), tot, v * tsg)
    for key, (v, sg) in part.items():
        if key not in out:
            out[key] = v if sg > 0 else -v
        else:
            out[key] = out[key] + v if sg > 0 else out[key] - v


def _bilinear(alg, a_of, b_of, out, tie=None, cut=None):
    for rnd, (r0, r1) in enumerate(alg.rounds):
        prods = []
        for a, b, c in alg.prods[r0:r1]:
            av, bv = a_of(a), b_of(b)
            if tie is not None and rnd == tie[0] and not prods:
                bv = _tie(bv, tie[1]())
            if cut is not None and len(alg.prods) - r0 == 2:
                m = jnp.concatenate([_dot(av[0:cut], bv), _dot(av[cut:], bv)], axis=0)
            else:
                m = _dot(av, bv)
            prods.append((m, c))
        _round(prods, out)
    return out


def _pack(v):
    return pltpu.bitcast(v, jnp.uint32)


def _unpack(v):
    return pltpu.bitcast(v, _BF16)


def _tie(v, words):
    u = _pack(v)
    return _unpack(jnp.concatenate([u[0:8] | words, u[8:]], axis=0))


def _lo(n):
    return jax.lax.broadcasted_iota(jnp.int32, (n, 128), 1) < 64


def _q_forms(c):
    a, b = [[c[m, n] * _SCALE for n in range(3)] for m in range(2)]
    lo = _lo(a[0].shape[0])
    rolled = pltpu.roll(b[1], 64, 1)
    forms = []
    for t, own in ((0, lo), (2, jnp.logical_not(lo))):
        t3 = jnp.where(own, a[t], b[t]).astype(_BF16)
        t3f = t3.astype(_F32)
        forms.append((t3,
                      jnp.where(own, a[1], a[t] - t3f).astype(_BF16),
                      jnp.where(own, b[t] - t3f, rolled).astype(_BF16)))
    return forms


def _qk_pass(af, kt, h, i):
    rows = (((0, 64), (128, 64), (0, 128)), ((256, 320), (256, 192), (192, 320)))[h][i]
    if i == 0:
        w = kt[rows[0]:rows[0] + 128]
    else:
        w = jnp.concatenate([kt[r:r + 64] for r in rows], axis=0)
    return _dot(af[i], w)


def _scores(af, kt, h):
    t = [_qk_pass(af, kt, h, i) for i in range(3)]
    return t[1] + t[0], t[2] + t[0]


def _softmax(s, g):
    s = (s[0], s[1] * jnp.concatenate([g] * 4, axis=1))
    es = [jnp.exp2(c - jnp.max(c, axis=-1, keepdims=True)) for c in s]
    parts = [(e[:, 0:128] + e[:, 128:256]) + (e[:, 256:384] + e[:, 384:512]) for e in es]
    return (es[0].astype(_BF16), es[1].astype(_BF16), (es[0] + es[1]).astype(_BF16)), parts


def _pv(p, vt, h, i):
    lo, hi, e = ((0, 64, 128), (256, 320, 192))[h]
    rows = (((e, hi), (lo, e), (lo, hi)), ((lo, e), (e, hi), (lo, hi)))[h][i]
    if rows == (lo, hi):
        w = vt[lo:lo + 128]
    else:
        w = jnp.concatenate([vt[r:r + 64] for r in rows], axis=0)
    return _nt(p[i], w)


def _pv_finish(t0, t1, l0, l1):
    r0, r1 = [[pl.reciprocal(jnp.sum(v, axis=-1, keepdims=True), approx=True) for v in l]
              for l in (l0, l1)]
    lo = _lo(t0[0].shape[0])
    d0 = jnp.where(lo, t0[1], t0[0])
    e0 = t0[2] - d0
    d1 = jnp.where(lo, t1[0], t1[1])
    e1 = t1[2] - d1
    return {(0, 0): jnp.where(lo, e0, d0) * r0[0],
            (1, 0): jnp.where(lo, d0, e0) * r0[1],
            (0, 1): jnp.where(lo, t0[0], t1[0]) * jnp.where(lo, r0[0], r1[0]),
            (1, 1): pltpu.roll(jnp.where(lo, t1[1], t0[1]), 64, 1) * jnp.where(lo, r0[1], r1[1]),
            (0, 2): jnp.where(lo, d1, e1) * r1[0],
            (1, 2): jnp.where(lo, e1, d1) * r1[1]}


def _kernel(xa, ka, va, wqa, woa, xb, kb, vb, wqb, wob, out,
            x_res, wq_res, wo_res, acc, ostage, kv, o_scr, xc, wqc, woc, f_scr, x_scale,
            zero_ref, g_sem, w_sem, p_sem, o_sem, *, aq, ao, n_main, u_duo, u_main, u_big, lead,
            extra, w1_at):
    n_pair, nb, ring = wq_res.shape[0], acc.shape[1], kv.shape[0]
    sq, d = acc.shape[2], acc.shape[3]
    lg = nb.bit_length() - 1
    lg_main = n_main.bit_length() - 1
    half, hm = nb // 2, sq // 2
    n_pos = n_pair * nb
    assert nb == 1 << lg and n_main == 1 << lg_main and half % n_main == 0 and 8 % half == 0
    assert nb <= u_duo < u_main and u_main % n_main == 0 and u_duo % 2 == 0
    assert n_main < lead < ring and lead <= u_duo and w1_at < half

    def static(v):
        return isinstance(v, int)

    def shr(v, s):
        return v >> s if static(v) else jax.lax.shift_right_logical(v, s)

    def aligned(v, m):
        return v if static(v) else pl.multiple_of(v, m)

    def clamp(u, hi=n_pos - 1):
        return min(max(u, 0), hi) if static(u) else jnp.clip(u, 0, hi)

    def when(*conds):
        dyn = [c for c in conds if not isinstance(c, bool)]
        if not all(c for c in conds if isinstance(c, bool)):
            return lambda f: None
        if not dyn:
            return lambda f: f()
        return pl.when(functools.reduce(jnp.logical_and, dyn))

    def pair_ds(p):
        return pl.ds(aligned(p * _PAIR, _PAIR), _PAIR)

    def sem_of(u, early):
        late = ring + (shr(u, lg_main) & (ring // n_main - 1))
        if static(u):
            return u & (ring - 1) if u < u_main else late
        return late if early is False else jnp.where(u < u_main, u & (ring - 1), late)

    def x_copy(br, b, sem):
        return pltpu.make_async_copy((xa, xb)[br].at[b], x_res.at[br, b, 0:sq], sem)

    def issue(u, h, early, may_end, enable=True):
        uc = clamp(u) if may_end else u
        sem = g_sem.at[sem_of(uc, early)]
        if early:
            ux = clamp(u + 1, nb - 1)

            @when(enable, u + 1 < nb)
            def _():
                x_copy(h, ux, sem).start()
        for i, ref in enumerate(((ka, va), (kb, vb))[h]):
            src = ref.at[uc & (nb - 1), pair_ds(shr(uc, lg)), :]

            @when(enable, (u < n_pos) if may_end else True)
            def _():
                pltpu.make_async_copy(src, kv.at[uc & (ring - 1), 2 * h + i], sem).start()
        if early and h == 1:
            @when(enable, u == w1_at)
            def _():
                w_start(1)

    def wq_copy(p, br, sem):
        return pltpu.make_async_copy((wqa, wqb)[br].at[:, pair_ds(p)], wq_res.at[p, br], sem)

    def wo_copy(p, br, sem):
        return pltpu.make_async_copy((woa, wob)[br].at[pair_ds(p), :], wo_res.at[p, br], sem)

    def w_start(p):
        for br in range(2):
            wq_copy(p, br, w_sem.at[p & 1]).start()
            wo_copy(p, br, w_sem.at[p & 1]).start()

    def waits_for(u0, n, early, big=False):
        g = min(n, n_main) if early is False else 1
        for u in [u0 + i for i in range(0, n, g)]:
            blk = kv.at[pl.ds(aligned(u & (ring - 1), g), g)]
            sem = g_sem.at[sem_of(u, False) if early is False else u & (ring - 1)]
            pltpu.make_async_copy(blk, blk, sem).wait()
        if early:
            @when(u0 + 1 < nb)
            def _():
                for br in range(2):
                    x_copy(br, u0 + 1, sem).wait()
        p1 = shr(u0, lg) + 1

        @when((u0 & (nb - 1)) == (0 if big else half), p1 < n_pair)
        def _():
            for ref in (wq_res, wo_res):
                pltpu.make_async_copy(ref.at[p1], ref.at[p1], w_sem.at[p1 & 1]).wait()

    def tile(ref, i, j, rows):
        return ref[i * rows:(i + 1) * rows, j * 128:(j + 1) * 128]

    def x_balance(br, b):
        m = [jnp.broadcast_to(jnp.max(jnp.abs(x_res[br, b, i * hm:(i + 1) * hm, :].astype(_F32)),
                                      axis=-1, keepdims=True), (hm, 128)) for i in range(2)]
        ratio = m[1] * pl.reciprocal(m[0], approx=True) * math.sqrt(2.0)
        ratio = jnp.where(jnp.logical_and(m[0] > 0, m[1] > 0), ratio, 1.0)
        e = jnp.clip(pltpu.bitcast(ratio, jnp.int32) & 0x7f800000, 0x20000000, 0x5f000000)
        x_scale[br, b, 0:hm] = pltpu.bitcast(e, _F32)

    def x_forms(br, b, g):
        inv = pltpu.bitcast(0x7f000000 - pltpu.bitcast(g, jnp.int32), _F32)
        x = x_res.at[br, b]
        blk = {}
        for j in range(d // 128):
            blk[0, j] = tile(x, 0, j, hm).astype(_F32)
            blk[1, j] = tile(x, 1, j, hm).astype(_F32) * inv
        for r, f in enumerate(aq.a_forms):
            xc[br, b, r] = _pack(tile(x, 0, f[0][1], hm) if len(f) == 1 and f[0][0] == 0
                                 else _combine(f, lambda i, j: blk[i, j]).astype(_BF16))

    def w_forms(br, p, si, lo=0):
        for raw, dst, alg in ((wq_res, wqc, aq), (wo_res, woc, ao)):
            view = raw.at[p, br, pl.ds(aligned(si * 16, 16), raw.shape[2] - 112 + 16 * lo)]
            rows = pl.ds(aligned((si + lo) * 8, 8), 8)
            blk = {}

            def src(i, j):
                return view[i * 128 + lo * 16:i * 128 + lo * 16 + 16, j * 128:(j + 1) * 128]

            def get(i, j):
                if (i, j) not in blk:
                    blk[i, j] = src(i, j).astype(_F32)
                return blk[i, j]
            for r, f in enumerate(alg.b_forms):
                dst[p & 1, br, r, rows, :] = _pack(
                    src(f[0][0], f[0][1]) if len(f) == 1 else _combine(f, get).astype(_BF16))

    def block(u0, n, kind, refill, emit_prev=False):
        T = 2 * n
        last = kind in ("last", "end")
        first_order, mid_order, last_order, tie_w, tie_f, tie_f0 = _PLAN[kind]
        zero_idx = zero_ref[0]
        zero_vec = jnp.full((8, 128), zero_idx, jnp.int32).astype(jnp.uint32)

        def task(k):
            u = u0 + k // 2
            if k == -1 and kind == "ramp":
                u = clamp(u)
            return k % 2, u & (nb - 1), shr(u, lg)

        def kv_ref(k, i):
            return kv.at[(u0 + k // 2) & (ring - 1), 2 * (k % 2) + i]

        def put_o(o):
            for (i, j), v in o.items():
                f_scr[3 * i + j] = v

        Q, S, P, OT, O = {}, {}, {}, {}, {}
        G = {k: x_scale[k % 2, task(k)[1], 0:hm] for k in range(T)} if kind == "ramp" else {}
        put_o(_pv_finish(*[[o_scr[r] for r in rr]
                           for rr in ((0, 1, 2), (3, 4, 5), (6, 7), (8, 9))]))

        def do_q(k):
            br, b, p = task(k)
            tie = (tie_f if k > 0 else tie_f0,
                   lambda: pltpu.bitcast(f_scr[zero_idx, 0:8], jnp.uint32) & zero_vec)
            Q[k, 0], Q[k, 1] = _q_forms(_bilinear(
                aq, lambda f: _unpack(xc[br, b, aq.a_forms.index(f)]),
                lambda f: _unpack(wqc[p & 1, br, aq.b_forms.index(f)]), {}, tie))

        def do_qk(k, h):
            af = Q.pop((k, h))
            if tie_w is not None and tie_w // 3 == h and (kind != "big" or k < n):
                br, _, p = task(k)
                for ref in (wqc, woc):
                    words = ref[p & 1, br, 0, 0:8] & zero_vec
                    af = tuple(_tie(v, words) if i == tie_w % 3 else v for i, v in enumerate(af))
            S[k, h] = _scores(af, kv_ref(k, 0), h)

        def do_pv(k, h):
            br, b, _ = task(k)
            P[k, h] = _softmax(S.pop((k, h)), G[k] if k in G else x_scale[br, b, 0:hm])
            for i in (0, 2, 1):
                OT[k, h, i] = _pv(P[k, h][0], kv_ref(k, 1), h, i)

        def o_forms(o):
            return [_combine(f, lambda i, j: o[i, j]).astype(_BF16) for f in ao.a_forms]

        def do_pf(k):
            t0, t1 = [[OT.pop((k, h, i)) for i in range(3)] for h in range(2)]
            l0, l1 = P.pop((k, 0))[1], P.pop((k, 1))[1]
            if k < T - 1:
                put_o(_pv_finish(t0, t1, l0, l1))
            elif kind == "end":
                O[k] = o_forms(_pv_finish(t0, t1, l0, l1))
            else:
                for r, v in enumerate(t0 + t1 + l0 + l1):
                    o_scr[r] = v

        def do_o(k):
            br, b, p = task(k)
            forms = O.pop(k) if k in O else o_forms(
                {(i, j): f_scr[3 * i + j] for i in range(2) for j in range(3)})
            a = acc.at[br, b]
            fresh = kind == "ramp" or (kind == "duo" and k == -1)
            c = _bilinear(
                ao, lambda f: forms[ao.a_forms.index(f)],
                lambda f: _unpack(woc[p & 1, br, ao.b_forms.index(f)]),
                {(i, j): (jnp.where(p > 0, tile(a, i, j, hm), 0.0) if fresh
                          else tile(a, i, j, hm)) for i in range(2) for j in range(d // 128)},
                cut=48)
            keep, emit = (emit_prev is not True, emit_prev) if k == -1 else (not last, True)
            if keep:
                for (i, j), v in c.items():
                    a[i * hm:(i + 1) * hm, j * 128:(j + 1) * 128] = v
            if last:
                for i in range(2):
                    row = jnp.concatenate([c[i, j] for j in range(d // 128)], axis=1)
                    ostage[b, i * hm:(i + 1) * hm, br * d:(br + 1) * d] = row.astype(ostage.dtype)
                if br == 1:
                    @when(emit)
                    def _():
                        pltpu.make_async_copy(ostage.at[b], out.at[b], o_sem.at[0]).start()

        def do_w(k):
            br, b, p = task(k)
            per = 8 // half
            if kind == "big":
                if k < n:
                    for i in range(per):
                        u = u0 + k // 2 + zero_idx
                        si = shr(u & half, lg - 3) if lg >= 3 else (u & half) * (4 // half)
                        w_forms(br, shr(u, lg) + 1, si, (k // 2) * per + i)
                return
            pc = jnp.minimum(p + shr(b, lg - 1), n_pair - 1)
            if n >= 4 and half == 8:
                w_forms(br, pc, b & 4, (k // 2) & 3)
            else:
                for i in range(per):
                    w_forms(br, pc, (b & (half - 1)) * per + i)

        ops = {"q": do_q, "a": lambda k: do_qk(k, 0), "b": lambda k: do_qk(k, 1),
               "u": lambda k: do_pv(k, 0), "v": lambda k: do_pv(k, 1), "f": do_pf,
               "o": lambda k: do_o(k - 1), "d": refill, "w": do_w,
               "x": lambda k: x_forms(*task(k)[:2], G[k]),
               "y": lambda k: x_balance(*task(k + 2)[:2])}
        for k in range(T):
            for c in (last_order if k == T - 1 else first_order if k == 0 else mid_order):
                ops[c](k)
        if kind == "end":
            do_o(T - 1)
        if not last:
            p2 = shr(u0, lg) + 2

            @when((u0 & (nb - 1)) == {"ramp": 3 * nb // 4, "duo": 3 * nb // 4, "main": half,
                                       "big": 0}[kind],
                  p2 < n_pair)
            def _():
                w_start(p2)

    zero_ref[0] = 0
    w0 = [wq_copy(0, 0, p_sem.at[0]), wq_copy(0, 1, p_sem.at[0]),
          wo_copy(0, 0, p_sem.at[0]), wo_copy(0, 1, p_sem.at[0]),
          x_copy(0, 0, p_sem.at[0]), x_copy(1, 0, p_sem.at[0])]
    for c in w0:
        c.start()

    def o_init(r, carry):
        o_scr[r] = jnp.zeros(o_scr.shape[1:], _F32)
        o_scr[6 + (r & 3)] = jnp.ones(o_scr.shape[1:], _F32)
        return carry
    jax.lax.fori_loop(0, 6, o_init, 0)
    for v in range(4):
        issue(v // 2, v % 2, True, False)
    for c in w0:
        c.wait()

    def w_first(si, carry):
        for br in range(2):
            w_forms(br, 0, si)
        return carry
    jax.lax.fori_loop(0, 8, w_first, 0)

    def x_first(br, carry):
        x_balance(br, 0)
        return carry
    jax.lax.fori_loop(0, 2, x_first, 0)

    def ramp(u, carry):
        fast = u < lead - 2
        g = u + 2 + jnp.minimum(u, lead - 2)

        def refill(k):
            if k == 0:
                issue(g, 0, True, False)
                issue(g, 1, True, False, fast)
            else:
                g1 = g + fast.astype(jnp.int32)
                issue(g1, 0, True, False, fast)
                issue(g1, 1, True, False)
        block(u, 1, "ramp", refill)

        @pl.when(u + 1 < u_duo)
        def _():
            waits_for(u + 1, 1, True)
        return carry

    waits_for(0, 1, True)
    jax.lax.fori_loop(0, u_duo, ramp, 0)

    def duo(j, carry):
        u0 = u_duo + 2 * j
        block(u0, 2, "duo", lambda k: issue(u0 + k // 2 + lead, k % 2, None, False))

        @pl.when(u0 + 2 < u_main)
        def _():
            waits_for(u0 + 2, 2, None)
        return carry

    waits_for(u_duo, 2, None)
    jax.lax.fori_loop(0, (u_main - u_duo) // 2, duo, 0)

    def steady(u_start, n, cnt, n_next, lead, extra, kind):
        may_end = u_start + cnt * n + lead + extra > n_pos

        def body(j, carry):
            u0 = u_start + j * n

            def refill(k):
                u, h = u0 + k // 2 + lead, k % 2
                if k // 2 < extra:
                    fast = j == 1
                    g = u + jnp.where(j > 1, extra, jnp.where(fast, k // 2 + h, 0))
                    issue(g, 0, False, may_end, fast if h == 1 else True)
                    issue(g, 1, False, may_end, fast if h == 0 else True)
                else:
                    issue(u + (jnp.where(j >= 1, extra, 0) if extra else 0), h, False, may_end)
            block(u0, n, kind, refill, emit_prev=(j > 0) if kind == "last" else False)

            @when((j + 1 < cnt) if n != n_next else True)
            def _():
                waits_for(u0 + n, n, False, kind == "big")
            return carry
        jax.lax.fori_loop(0, cnt, body, 0)
        if n != n_next:
            waits_for(u_start + cnt * n, n_next, False, n_next > n)

    n_big = 2 * n_main
    assert n_big == half and u_big % nb == 0 and u_big - u_main >= n_big
    assert extra <= n_main and n_big < lead + extra < ring
    assert not half < (u_main & (nb - 1)) <= 3 * nb // 4 and u_big < n_pos - nb
    waits_for(u_main, n_main, False)
    steady(u_main, n_main, (u_big - u_main) // n_main, n_big, lead, extra, "main")
    steady(u_big, n_big, (n_pos - nb - u_big) // n_big, n_main, lead + extra, 0, "big")
    steady(n_pos - nb, n_main, nb // n_main - 1, n_main, lead + extra, 0, "last")
    block(n_pos - n_main, n_main, "end", None, emit_prev=True)
    pltpu.make_async_copy(ostage, out, o_sem.at[0]).wait()


def _build(A_x, A_k_cache, A_v_cache, A_wq, A_wo, B_x, B_k_cache, B_v_cache, B_wq, B_wo, *,
           n_main=4, u_duo=16, u_main=24, u_big=64, lead=6, extra=4, w1_at=7, ring=16,
           interpret=False):
    nb, sq, d = A_x.shape
    n_head, sk = A_k_cache.shape[1], A_k_cache.shape[2]
    n_pair = n_head // 2

    def tr(c):
        return jnp.swapaxes(c, 2, 3).reshape(nb, n_head * _DH, sk)

    aq, ao = _Alg(_ALG_Q, 4), _Alg(_ALG_O, 3)
    u32 = jnp.uint32
    n_xf = -(-len(aq.a_forms) // 4) * 4
    return pl.pallas_call(
        functools.partial(_kernel, aq=aq, ao=ao, n_main=n_main, u_duo=u_duo, u_main=u_main,
                          u_big=u_big, lead=lead, extra=extra, w1_at=w1_at),
        in_specs=[pl.BlockSpec(memory_space=pl.ANY)] * 10,
        out_specs=pl.BlockSpec(memory_space=pl.ANY),
        out_shape=jax.ShapeDtypeStruct((nb, sq, 2 * d), A_x.dtype),
        scratch_shapes=[
            pltpu.VMEM((2, nb, 192, d), _BF16),
            pltpu.VMEM((n_pair, 2, d, _PAIR), _BF16),
            pltpu.VMEM((n_pair, 2, _PAIR, d), _BF16),
            pltpu.VMEM((2, nb, sq, d), _F32),
            pltpu.VMEM((nb, sq, 2 * d), _BF16),
            pltpu.VMEM((ring, 4, _PAIR, sk), _BF16),
            pltpu.VMEM((10, sq // 2, 128), _F32),
            pltpu.VMEM((2, nb, n_xf, sq // 4, 128), u32),
            pltpu.VMEM((2, 2, len(aq.b_forms), 64, 128), u32),
            pltpu.VMEM((2, 2, len(ao.b_forms), 64, 128), u32),
            pltpu.VMEM((6, sq // 2, 128), _F32),
            pltpu.VMEM((2, nb, 96, 128), _F32),
            pltpu.SMEM((1,), jnp.int32),
            pltpu.SemaphoreType.DMA((ring + ring // n_main,)),
            pltpu.SemaphoreType.DMA((2,)),
            pltpu.SemaphoreType.DMA((1,)),
            pltpu.SemaphoreType.DMA((1,)),
        ],
        compiler_params=pltpu.CompilerParams(
            vmem_limit_bytes=122 * 1024 * 1024, disable_bounds_checks=True),
        interpret=interpret,
    )(A_x, tr(A_k_cache), tr(A_v_cache), A_wq, A_wo,
      B_x, tr(B_k_cache), tr(B_v_cache), B_wq, B_wo)


@jax.jit
def pallas_concat_heads__gqa_block_cached__mha_block_cached__near_ridge_kernel(
    A_x: jax.Array,
    A_k_cache: jax.Array,
    A_v_cache: jax.Array,
    A_wq: jax.Array,
    A_wo: jax.Array,
    B_x: jax.Array,
    B_k_cache: jax.Array,
    B_v_cache: jax.Array,
    B_wq: jax.Array,
    B_wo: jax.Array,
):
    return _build(A_x, A_k_cache, A_v_cache, A_wq, A_wo,
                  B_x, B_k_cache, B_v_cache, B_wq, B_wo)
```

```python
import functools
import math

import jax
import jax.numpy as jnp
import jax.experimental.pallas as pl
import jax.experimental.pallas.tpu as pltpu

_DH = 192
_PAIR = 2 * _DH
_NT = (((1,), (1,)), ((), ()))
_F32 = jnp.float32
_BF16 = jnp.bfloat16
_SCALE = (_DH ** -0.5) * math.log2(math.e)

_ALG_Q = (
    (((0, 3, 1), (1, 3, -1), (1, 4, -1)), ((3, 2, -1), (4, 1, -1), (4, 2, 1)), ((0, 2, -1), (1, 0, 1), (1, 1, 1))),
    (((1, 4, 1),), ((3, 2, -1), (4, 0, 1), (4, 1, -1), (4, 2, 1)), ((1, 0, 1), (1, 1, 1), (1, 2, 1))),
    (((1, 1, 1), (1, 2, -1)), ((2, 0, 1),), ((1, 0, -1), (1, 2, -1))),
    (((0, 3, -1), (1, 3, 1)), ((3, 1, 1), (3, 2, -1), (4, 1, -1), (4, 2, 1)), ((1, 0, 1), (1, 1, 1))),
    (((0, 3, -1), (1, 0, 1)), ((0, 0, 1), (3, 0, 1), (3, 1, -1)), ((0, 1, 1), (1, 0, 1), (1, 1, 1))),
    (((1, 1, 1),), ((1, 0, 1), (2, 0, 1)), ((0, 0, 1), (1, 0, 1))),
    (((0, 3, 1),), ((0, 0, 1), (3, 0, 1)), ((0, 0, 1), (0, 1, 1), (1, 0, 1), (1, 1, 1))),
    (((1, 0, 1), (1, 3, -1)), ((3, 0, -1), (3, 1, 1)), ((1, 0, 1),)),
    (((0, 3, 1), (0, 4, 1), (1, 3, -1), (1, 4, -1)), ((4, 1, 1), (4, 2, -1)), ((0, 2, -1),)),
    (((1, 3, 1), (1, 4, 1)), ((3, 2, 1),), ((0, 2, 1), (1, 2, 1))),
    (((0, 2, -1), (1, 2, 1)), ((2, 0, -1), (2, 1, -1), (2, 2, 1)), ((1, 2, 1),)),
    (((0, 2, 1),), ((0, 2, -1), (1, 1, -1), (1, 2, 1), (2, 2, 1)), ((0, 2, 1), (1, 2, 1))),
    (((0, 2, 1), (1, 0, 1)), ((0, 2, 1), (2, 1, -1)), ((0, 1, -1), (1, 2, 1))),
    (((1, 0, 1),), ((0, 0, -1), (0, 1, 1), (2, 1, -1), (3, 0, -1), (3, 1, 1)), ((0, 1, 1), (1, 1, 1))),
    (((0, 1, -1), (0, 4, 1)), ((1, 1, 1),), ((0, 1, -1), (0, 2, -1), (1, 1, -1), (1, 2, -1))),
    (((0, 0, 1), (1, 0, -1)), ((0, 1, 1), (0, 2, -1)), ((0, 1, 1),)),
    (((1, 0, 1), (1, 2, 1)), ((2, 1, 1),), ((1, 1, 1), (1, 2, 1))),
    (((0, 1, -1), (0, 4, 1), (1, 1, 1)), ((1, 1, 1), (4, 0, -1), (4, 1, 1)), ((0, 0, -1), (1, 1, 1), (1, 2, 1))),
    (((0, 1, -1), (0, 4, 1), (1, 1, 1), (1, 4, -1)), ((4, 0, 1), (4, 1, -1)), ((1, 1, 1), (1, 2, 1))),
    (((0, 2, -1), (1, 1, 1)), ((1, 1, 1), (1, 2, -1), (2, 0, -1)), ((0, 0, 1), (1, 2, -1))),
    (((0, 1, 1), (1, 1, -1)), ((1, 0, 1), (1, 2, -1), (4, 0, 1), (4, 1, -1)), ((0, 0, 1),)),
    (((0, 4, 1),), ((1, 1, 1), (4, 1, 1)), ((0, 0, 1), (0, 1, 1), (0, 2, 1))),
    (((0, 0, 1), (0, 2, 1)), ((0, 2, 1),), ((0, 1, 1), (0, 2, 1))),
    (((0, 1, 1), (0, 2, -1)), ((1, 1, -1), (1, 2, 1)), ((0, 0, 1), (0, 2, 1))),
    (((0, 0, 1), (0, 3, -1)), ((0, 0, 1),), ((0, 0, 1),)),
)
_ALG_O = (
    (((1, 0, 1), (1, 2, -1)), ((0, 0, 1), (1, 0, 1)), ((1, 0, 1), (1, 2, -1))),
    (((0, 0, 1), (1, 0, -1)), ((0, 0, 1), (0, 2, 1), (0, 3, -1), (1, 0, 1)), ((1, 2, -1),)),
    (((0, 1, 1),), ((0, 1, 1), (0, 4, 1), (1, 1, 1), (1, 4, 1)), ((0, 1, 1),)),
    (((0, 0, -1), (0, 1, 1), (1, 0, 1)), ((0, 1, -1), (0, 4, -1), (1, 4, -1)), ((0, 1, 1), (0, 4, -1), (1, 4, -1))),
    (((0, 0, -1), (1, 0, 1)), ((0, 4, 1), (1, 4, 1)), ((0, 1, 1), (0, 4, -1))),
    (((1, 0, 1),), ((0, 1, 1),), ((0, 1, 1), (0, 4, -1), (1, 1, 1), (1, 4, -1))),
    (((1, 1, 1),), ((1, 1, 1), (1, 3, -1), (2, 1, -1), (2, 3, 1)), ((1, 1, 1),)),
    (((0, 2, 1),), ((2, 1, 1),), ((0, 1, 1), (0, 3, 1), (1, 1, 1), (1, 3, 1))),
    (((0, 2, 1), (1, 2, -1)), ((1, 3, 1), (2, 3, -1)), ((1, 1, 1), (1, 3, 1))),
    (((1, 1, 1), (1, 2, 1)), ((0, 3, 1), (2, 1, -1), (2, 3, 1)), ((0, 3, 1), (1, 3, 1))),
    (((0, 2, 1), (1, 1, -1), (1, 2, -1)), ((1, 3, -1), (2, 1, -1), (2, 3, 1)), ((0, 3, 1), (1, 1, 1), (1, 3, 1))),
    (((1, 0, 1), (1, 1, -1), (1, 2, -1)), ((0, 3, 1),), ((1, 2, 1), (1, 3, 1))),
    (((0, 2, 1), (1, 2, -1)), ((1, 2, -1), (2, 0, 1), (2, 2, 1), (2, 4, 1)), ((0, 0, 1),)),
    (((0, 0, -1), (1, 2, 1)), ((0, 0, -1), (1, 0, -1), (1, 2, -1), (2, 2, 1)), ((0, 0, 1), (1, 2, 1))),
    (((0, 0, 1), (0, 2, -1)), ((1, 2, -1), (2, 2, 1)), ((0, 0, 1), (0, 2, -1))),
    (((0, 0, 1), (1, 1, -1), (1, 2, -1)), ((0, 3, -1), (1, 2, -1)), ((0, 3, -1), (1, 2, 1))),
    (((0, 1, 1), (0, 2, 1), (1, 1, -1), (1, 2, -1)), ((1, 2, -1), (1, 3, 1)), ((0, 3, 1),)),
    (((0, 0, 1),), ((0, 2, 1), (2, 2, 1)), ((0, 2, 1), (1, 2, 1))),
    (((0, 0, -1), (0, 1, 1), (0, 2, 1)), ((1, 2, 1),), ((0, 2, 1), (0, 3, 1))),
    (((1, 0, -1), (1, 1, 1), (1, 2, 1)), ((1, 0, -1),), ((1, 0, -1), (1, 4, 1))),
    (((0, 0, 1), (0, 1, -1), (1, 0, -1), (1, 1, 1)), ((1, 0, -1), (1, 4, -1)), ((1, 4, -1),)),
    (((0, 0, 1), (0, 1, -1), (1, 2, -1)), ((1, 0, -1), (2, 4, -1)), ((0, 0, 1), (1, 4, 1))),
    (((1, 2, 1),), ((0, 0, 1), (2, 0, 1)), ((0, 0, 1), (1, 0, 1))),
    (((0, 0, -1), (0, 1, 1), (0, 2, 1)), ((2, 4, 1),), ((0, 0, -1), (0, 4, 1))),
    (((0, 0, 1), (0, 1, -1)), ((0, 1, 1), (0, 4, 1), (2, 4, 1)), ((0, 4, 1), (1, 4, 1))),
)

_PLAN = {
    "ramp": ("xqdwyoabuvf", "", "dxqwyoabuvf", None, 6, 3),
    "duo": ("qdwoabuvf", "dqwoabuvf", "dqwoabuvf", 4, 6, 6),
    "main": ("qdwoabuvf", "dqwoabuvf", "dqwoabuvf", 4, 6, 6),
    "big": ("qdwoabuvf", "dqwoabuvf", "dqwoabuvf", 4, 6, 6),
    "last": ("qdoabuvf", "dqoabuvf", "dqoabuvf", None, 6, 6),
    "end": ("qoabuvf", "qoabuvf", "qoabuvf", None, 5, 3),
}


class _Alg:
    def __init__(self, table, lead):
        def norm(t):
            sg = t[0][2]
            return tuple((i, j, c * sg) for i, j, c in t), sg
        starts = [0] + list(range(lead, len(table), 4)) + [len(table)]
        self.rounds = list(zip(starts[:-1], starts[1:]))
        self.a_forms, self.b_forms, self.prods = [], [], []
        for a, b, c in table:
            (a, sa), (b, sb) = norm(a), norm(b)
            if a not in self.a_forms:
                self.a_forms.append(a)
            if b not in self.b_forms:
                self.b_forms.append(b)
            self.prods.append((a, b, tuple((i, j, v * sa * sb) for i, j, v in c)))


def _dot(a, b):
    return jnp.dot(a, b, preferred_element_type=_F32)


def _nt(a, b):
    return jax.lax.dot_general(a, b, _NT, preferred_element_type=_F32)


def _combine(form, get):
    r = get(form[0][0], form[0][1])
    for i, j, c in form[1:]:
        r = r + get(i, j) if c > 0 else r - get(i, j)
    return r


def _signed_add(d, key, v, sg):
    if key not in d:
        d[key] = (v, sg)
    else:
        w, sw = d[key]
        d[key] = (w + v if sg == sw else w - v, sw)


def _round(prods, out):
    groups, part = {}, {}
    for m, c in prods:
        sg = c[0][2]
        _signed_add(groups, tuple((i, j, v * sg) for i, j, v in c), m, sg)
    for c, (tot, tsg) in groups.items():
        for i, j, v in c:
            _signed_add(part, (i, j), tot, v * tsg)
    for key, (v, sg) in part.items():
        if key not in out:
            out[key] = v if sg > 0 else -v
        else:
            out[key] = out[key] + v if sg > 0 else out[key] - v


def _bilinear(alg, a_of, b_of, out, tie=None, cut=None):
    for rnd, (r0, r1) in enumerate(alg.rounds):
        prods = []
        for a, b, c in alg.prods[r0:r1]:
            av, bv = a_of(a), b_of(b)
            if tie is not None and rnd == tie[0] and not prods:
                bv = _tie(bv, tie[1]())
            if cut is not None and len(alg.prods) - r0 == 2:
                m = jnp.concatenate([_dot(av[0:cut], bv), _dot(av[cut:], bv)], axis=0)
            else:
                m = _dot(av, bv)
            prods.append((m, c))
        _round(prods, out)
    return out


def _pack(v):
    return pltpu.bitcast(v, jnp.uint32)


def _unpack(v):
    return pltpu.bitcast(v, _BF16)


def _tie(v, words):
    u = _pack(v)
    return _unpack(jnp.concatenate([u[0:8] | words, u[8:]], axis=0))


def _lo(n):
    return jax.lax.broadcasted_iota(jnp.int32, (n, 128), 1) < 64


def _q_forms(c):
    a, b = [[c[m, n] * _SCALE for n in range(3)] for m in range(2)]
    lo = _lo(a[0].shape[0])
    rolled = pltpu.roll(b[1], 64, 1)
    forms = []
    for t, own in ((0, lo), (2, jnp.logical_not(lo))):
        t3 = jnp.where(own, a[t], b[t]).astype(_BF16)
        t3f = t3.astype(_F32)
        forms.append((t3,
                      jnp.where(own, a[1], a[t] - t3f).astype(_BF16),
                      jnp.where(own, b[t] - t3f, rolled).astype(_BF16)))
    return forms


def _qk_pass(af, kt, h, i):
    rows = (((0, 64), (128, 64), (0, 128)), ((256, 320), (256, 192), (192, 320)))[h][i]
    if i == 0:
        w = kt[rows[0]:rows[0] + 128]
    else:
        w = jnp.concatenate([kt[r:r + 64] for r in rows], axis=0)
    return _dot(af[i], w)


def _scores(af, kt, h):
    t = [_qk_pass(af, kt, h, i) for i in range(3)]
    return t[1] + t[0], t[2] + t[0]


def _softmax(s, g):
    s = (s[0], s[1] * jnp.concatenate([g] * 4, axis=1))
    es = [jnp.exp2(c - jnp.max(c, axis=-1, keepdims=True)) for c in s]
    parts = [(e[:, 0:128] + e[:, 128:256]) + (e[:, 256:384] + e[:, 384:512]) for e in es]
    return (es[0].astype(_BF16), es[1].astype(_BF16), (es[0] + es[1]).astype(_BF16)), parts


def _pv(p, vt, h, i):
    lo, hi, e = ((0, 64, 128), (256, 320, 192))[h]
    rows = (((e, hi), (lo, e), (lo, hi)), ((lo, e), (e, hi), (lo, hi)))[h][i]
    if rows == (lo, hi):
        w = vt[lo:lo + 128]
    else:
        w = jnp.concatenate([vt[r:r + 64] for r in rows], axis=0)
    return _nt(p[i], w)


def _pv_finish(t0, t1, l0, l1):
    r0, r1 = [[pl.reciprocal(jnp.sum(v, axis=-1, keepdims=True), approx=True) for v in l]
              for l in (l0, l1)]
    lo = _lo(t0[0].shape[0])
    d0 = jnp.where(lo, t0[1], t0[0])
    e0 = t0[2] - d0
    d1 = jnp.where(lo, t1[0], t1[1])
    e1 = t1[2] - d1
    return {(0, 0): jnp.where(lo, e0, d0) * r0[0],
            (1, 0): jnp.where(lo, d0, e0) * r0[1],
            (0, 1): jnp.where(lo, t0[0], t1[0]) * jnp.where(lo, r0[0], r1[0]),
            (1, 1): pltpu.roll(jnp.where(lo, t1[1], t0[1]), 64, 1) * jnp.where(lo, r0[1], r1[1]),
            (0, 2): jnp.where(lo, d1, e1) * r1[0],
            (1, 2): jnp.where(lo, e1, d1) * r1[1]}


def _kernel(xa, ka, va, wqa, woa, xb, kb, vb, wqb, wob, out,
            x_res, wq_res, wo_res, acc, ostage, kv, o_scr, xc, wqc, woc, f_scr, x_scale,
            zero_ref, g_sem, w_sem, p_sem, o_sem, *, aq, ao, n_main, u_duo, u_main, u_big, lead,
            extra, w1_at):
    n_pair, nb, ring = wq_res.shape[0], acc.shape[1], kv.shape[0]
    sq, d = acc.shape[2], acc.shape[3]
    lg = nb.bit_length() - 1
    lg_main = n_main.bit_length() - 1
    half, hm = nb // 2, sq // 2
    n_pos = n_pair * nb
    assert nb == 1 << lg and n_main == 1 << lg_main and half % n_main == 0 and 8 % half == 0
    assert nb <= u_duo < u_main and u_main % n_main == 0 and u_duo % 2 == 0
    assert n_main < lead < ring and lead <= u_duo and w1_at < half

    def static(v):
        return isinstance(v, int)

    def shr(v, s):
        return v >> s if static(v) else jax.lax.shift_right_logical(v, s)

    def aligned(v, m):
        return v if static(v) else pl.multiple_of(v, m)

    def clamp(u, hi=n_pos - 1):
        return min(max(u, 0), hi) if static(u) else jnp.clip(u, 0, hi)

    def when(*conds):
        dyn = [c for c in conds if not isinstance(c, bool)]
        if not all(c for c in conds if isinstance(c, bool)):
            return lambda f: None
        if not dyn:
            return lambda f: f()
        return pl.when(functools.reduce(jnp.logical_and, dyn))

    def pair_ds(p):
        return pl.ds(aligned(p * _PAIR, _PAIR), _PAIR)

    def sem_of(u, early):
        late = ring + (shr(u, lg_main) & (ring // n_main - 1))
        if static(u):
            return u & (ring - 1) if u < u_main else late
        return late if early is False else jnp.where(u < u_main, u & (ring - 1), late)

    def x_copy(br, b, sem):
        return pltpu.make_async_copy((xa, xb)[br].at[b], x_res.at[br, b, 0:sq], sem)

    def issue(u, h, early, may_end, enable=True):
        uc = clamp(u) if may_end else u
        sem = g_sem.at[sem_of(uc, early)]
        if early:
            ux = clamp(u + 1, nb - 1)

            @when(enable, u + 1 < nb)
            def _():
                x_copy(h, ux, sem).start()
        for i, ref in enumerate(((ka, va), (kb, vb))[h]):
            src = ref.at[uc & (nb - 1), pair_ds(shr(uc, lg)), :]

            @when(enable, (u < n_pos) if may_end else True)
            def _():
                pltpu.make_async_copy(src, kv.at[uc & (ring - 1), 2 * h + i], sem).start()
        if early and h == 1:
            @when(enable, u == w1_at)
            def _():
                w_start(1)

    def wq_copy(p, br, sem):
        return pltpu.make_async_copy((wqa, wqb)[br].at[:, pair_ds(p)], wq_res.at[p, br], sem)

    def wo_copy(p, br, sem):
        return pltpu.make_async_copy((woa, wob)[br].at[pair_ds(p), :], wo_res.at[p, br], sem)

    def w_start(p):
        for br in range(2):
            wq_copy(p, br, w_sem.at[p & 1]).start()
            wo_copy(p, br, w_sem.at[p & 1]).start()

    def waits_for(u0, n, early, big=False):
        g = min(n, n_main) if early is False else 1
        for u in [u0 + i for i in range(0, n, g)]:
            blk = kv.at[pl.ds(aligned(u & (ring - 1), g), g)]
            sem = g_sem.at[sem_of(u, False) if early is False else u & (ring - 1)]
            pltpu.make_async_copy(blk, blk, sem).wait()
        if early:
            @when(u0 + 1 < nb)
            def _():
                for br in range(2):
                    x_copy(br, u0 + 1, sem).wait()
        p1 = shr(u0, lg) + 1

        @when((u0 & (nb - 1)) == (0 if big else half), p1 < n_pair)
        def _():
            for ref in (wq_res, wo_res):
                pltpu.make_async_copy(ref.at[p1], ref.at[p1], w_sem.at[p1 & 1]).wait()

    def tile(ref, i, j, rows):
        return ref[i * rows:(i + 1) * rows, j * 128:(j + 1) * 128]

    def x_balance(br, b):
        m = [jnp.broadcast_to(jnp.max(jnp.abs(x_res[br, b, i * hm:(i + 1) * hm, :].astype(_F32)),
                                      axis=-1, keepdims=True), (hm, 128)) for i in range(2)]
        ratio = m[1] * pl.reciprocal(m[0], approx=True) * math.sqrt(2.0)
        ratio = jnp.where(jnp.logical_and(m[0] > 0, m[1] > 0), ratio, 1.0)
        e = jnp.clip(pltpu.bitcast(ratio, jnp.int32) & 0x7f800000, 0x20000000, 0x5f000000)
        x_scale[br, b, 0:hm] = pltpu.bitcast(e, _F32)

    def x_forms(br, b, g):
        inv = pltpu.bitcast(0x7f000000 - pltpu.bitcast(g, jnp.int32), _F32)
        x = x_res.at[br, b]
        blk = {}
        for j in range(d // 128):
            blk[0, j] = tile(x, 0, j, hm).astype(_F32)
            blk[1, j] = tile(x, 1, j, hm).astype(_F32) * inv
        for r, f in enumerate(aq.a_forms):
            xc[br, b, r] = _pack(tile(x, 0, f[0][1], hm) if len(f) == 1 and f[0][0] == 0
                                 else _combine(f, lambda i, j: blk[i, j]).astype(_BF16))

    def w_forms(br, p, si, lo=0):
        for raw, dst, alg in ((wq_res, wqc, aq), (wo_res, woc, ao)):
            view = raw.at[p, br, pl.ds(aligned(si * 16, 16), raw.shape[2] - 112 + 16 * lo)]
            rows = pl.ds(aligned((si + lo) * 8, 8), 8)
            blk = {}

            def src(i, j):
                return view[i * 128 + lo * 16:i * 128 + lo * 16 + 16, j * 128:(j + 1) * 128]

            def get(i, j):
                if (i, j) not in blk:
                    blk[i, j] = src(i, j).astype(_F32)
                return blk[i, j]
            for r, f in enumerate(alg.b_forms):
                dst[p & 1, br, r, rows, :] = _pack(
                    src(f[0][0], f[0][1]) if len(f) == 1 else _combine(f, get).astype(_BF16))

    def block(u0, n, kind, refill, emit_prev=False):
        T = 2 * n
        last = kind in ("last", "end")
        first_order, mid_order, last_order, tie_w, tie_f, tie_f0 = _PLAN[kind]
        zero_idx = zero_ref[0]
        zero_vec = jnp.full((8, 128), zero_idx, jnp.int32).astype(jnp.uint32)

        def task(k):
            u = u0 + k // 2
            if k == -1 and kind == "ramp":
                u = clamp(u)
            return k % 2, u & (nb - 1), shr(u, lg)

        def kv_ref(k, i):
            return kv.at[(u0 + k // 2) & (ring - 1), 2 * (k % 2) + i]

        def put_o(o):
            for (i, j), v in o.items():
                f_scr[3 * i + j] = v

        Q, S, P, OT, O = {}, {}, {}, {}, {}
        G = {k: x_scale[k % 2, task(k)[1], 0:hm] for k in range(T)} if kind == "ramp" else {}
        put_o(_pv_finish(*[[o_scr[r] for r in rr]
                           for rr in ((0, 1, 2), (3, 4, 5), (6, 7), (8, 9))]))

        def do_q(k):
            br, b, p = task(k)
            tie = (tie_f if k > 0 else tie_f0,
                   lambda: pltpu.bitcast(f_scr[zero_idx, 0:8], jnp.uint32) & zero_vec)
            Q[k, 0], Q[k, 1] = _q_forms(_bilinear(
                aq, lambda f: _unpack(xc[br, b, aq.a_forms.index(f)]),
                lambda f: _unpack(wqc[p & 1, br, aq.b_forms.index(f)]), {}, tie))

        def do_qk(k, h):
            af = Q.pop((k, h))
            if tie_w is not None and tie_w // 3 == h and (kind != "big" or k < n):
                br, _, p = task(k)
                for ref in (wqc, woc):
                    words = ref[p & 1, br, 0, 0:8] & zero_vec
                    af = tuple(_tie(v, words) if i == tie_w % 3 else v for i, v in enumerate(af))
            S[k, h] = _scores(af, kv_ref(k, 0), h)

        def do_pv(k, h):
            br, b, _ = task(k)
            P[k, h] = _softmax(S.pop((k, h)), G[k] if k in G else x_scale[br, b, 0:hm])
            for i in (0, 2, 1):
                OT[k, h, i] = _pv(P[k, h][0], kv_ref(k, 1), h, i)

        def o_forms(o):
            return [_combine(f, lambda i, j: o[i, j]).astype(_BF16) for f in ao.a_forms]

        def do_pf(k):
            t0, t1 = [[OT.pop((k, h, i)) for i in range(3)] for h in range(2)]
            l0, l1 = P.pop((k, 0))[1], P.pop((k, 1))[1]
            if k < T - 1:
                put_o(_pv_finish(t0, t1, l0, l1))
            elif kind == "end":
                O[k] = o_forms(_pv_finish(t0, t1, l0, l1))
            else:
                for r, v in enumerate(t0 + t1 + l0 + l1):
                    o_scr[r] = v

        def do_o(k):
            br, b, p = task(k)
            forms = O.pop(k) if k in O else o_forms(
                {(i, j): f_scr[3 * i + j] for i in range(2) for j in range(3)})
            a = acc.at[br, b]
            fresh = kind == "ramp" or (kind == "duo" and k == -1)
            c = _bilinear(
                ao, lambda f: forms[ao.a_forms.index(f)],
                lambda f: _unpack(woc[p & 1, br, ao.b_forms.index(f)]),
                {(i, j): (jnp.where(p > 0, tile(a, i, j, hm), 0.0) if fresh
                          else tile(a, i, j, hm)) for i in range(2) for j in range(d // 128)},
                cut=48)
            keep, emit = (emit_prev is not True, emit_prev) if k == -1 else (not last, True)
            if keep:
                for (i, j), v in c.items():
                    a[i * hm:(i + 1) * hm, j * 128:(j + 1) * 128] = v
            if last:
                for i in range(2):
                    row = jnp.concatenate([c[i, j] for j in range(d // 128)], axis=1)
                    ostage[b, i * hm:(i + 1) * hm, br * d:(br + 1) * d] = row.astype(ostage.dtype)
                if kind == "end" and k >= T - 2:
                    cols = pl.ds(br * d, d)
                    pltpu.make_async_copy(ostage.at[b, :, cols], out.at[b, :, cols],
                                          o_sem.at[0]).start()
                elif br == 1:
                    @when(emit)
                    def _():
                        pltpu.make_async_copy(ostage.at[b], out.at[b], o_sem.at[0]).start()

        def do_w(k):
            br, b, p = task(k)
            per = 8 // half
            if kind == "big":
                if k < n:
                    for i in range(per):
                        u = u0 + k // 2 + zero_idx
                        si = shr(u & half, lg - 3) if lg >= 3 else (u & half) * (4 // half)
                        w_forms(br, shr(u, lg) + 1, si, (k // 2) * per + i)
                return
            pc = jnp.minimum(p + shr(b, lg - 1), n_pair - 1)
            if n >= 4 and half == 8:
                w_forms(br, pc, b & 4, (k // 2) & 3)
            else:
                for i in range(per):
                    w_forms(br, pc, (b & (half - 1)) * per + i)

        ops = {"q": do_q, "a": lambda k: do_qk(k, 0), "b": lambda k: do_qk(k, 1),
               "u": lambda k: do_pv(k, 0), "v": lambda k: do_pv(k, 1), "f": do_pf,
               "o": lambda k: do_o(k - 1), "d": refill, "w": do_w,
               "x": lambda k: x_forms(*task(k)[:2], G[k]),
               "y": lambda k: x_balance(*task(k + 2)[:2])}
        for k in range(T):
            for c in (last_order if k == T - 1 else first_order if k == 0 else mid_order):
                ops[c](k)
        if kind == "end":
            do_o(T - 1)
        if not last:
            p2 = shr(u0, lg) + 2

            @when((u0 & (nb - 1)) == {"ramp": 3 * nb // 4, "duo": 3 * nb // 4, "main": half,
                                       "big": 0}[kind],
                  p2 < n_pair)
            def _():
                w_start(p2)

    zero_ref[0] = 0
    w0 = [wq_copy(0, 0, p_sem.at[0]), wq_copy(0, 1, p_sem.at[0]),
          wo_copy(0, 0, p_sem.at[0]), wo_copy(0, 1, p_sem.at[0]),
          x_copy(0, 0, p_sem.at[0]), x_copy(1, 0, p_sem.at[0])]
    for c in w0:
        c.start()

    def o_init(r, carry):
        o_scr[r] = jnp.zeros(o_scr.shape[1:], _F32)
        o_scr[6 + (r & 3)] = jnp.ones(o_scr.shape[1:], _F32)
        return carry
    jax.lax.fori_loop(0, 6, o_init, 0)
    for v in range(4):
        issue(v // 2, v % 2, True, False)
    for c in w0:
        c.wait()

    def w_first(si, carry):
        for br in range(2):
            w_forms(br, 0, si)
        return carry
    jax.lax.fori_loop(0, 8, w_first, 0)

    def x_first(br, carry):
        x_balance(br, 0)
        return carry
    jax.lax.fori_loop(0, 2, x_first, 0)

    def ramp(u, carry):
        fast = u < lead - 2
        g = u + 2 + jnp.minimum(u, lead - 2)

        def refill(k):
            if k == 0:
                issue(g, 0, True, False)
                issue(g, 1, True, False, fast)
            else:
                g1 = g + fast.astype(jnp.int32)
                issue(g1, 0, True, False, fast)
                issue(g1, 1, True, False)
        block(u, 1, "ramp", refill)

        @pl.when(u + 1 < u_duo)
        def _():
            waits_for(u + 1, 1, True)
        return carry

    waits_for(0, 1, True)
    jax.lax.fori_loop(0, u_duo, ramp, 0)

    def duo(j, carry):
        u0 = u_duo + 2 * j
        block(u0, 2, "duo", lambda k: issue(u0 + k // 2 + lead, k % 2, None, False))

        @pl.when(u0 + 2 < u_main)
        def _():
            waits_for(u0 + 2, 2, None)
        return carry

    waits_for(u_duo, 2, None)
    jax.lax.fori_loop(0, (u_main - u_duo) // 2, duo, 0)

    def steady(u_start, n, cnt, n_next, lead, extra, kind):
        may_end = u_start + cnt * n + lead + extra > n_pos

        def body(j, carry):
            u0 = u_start + j * n

            def refill(k):
                u, h = u0 + k // 2 + lead, k % 2
                if k // 2 < extra:
                    fast = j == 1
                    g = u + jnp.where(j > 1, extra, jnp.where(fast, k // 2 + h, 0))
                    issue(g, 0, False, may_end, fast if h == 1 else True)
                    issue(g, 1, False, may_end, fast if h == 0 else True)
                else:
                    issue(u + (jnp.where(j >= 1, extra, 0) if extra else 0), h, False, may_end)
            block(u0, n, kind, refill, emit_prev=(j > 0) if kind == "last" else False)

            @when((j + 1 < cnt) if n != n_next else True)
            def _():
                waits_for(u0 + n, n, False, kind == "big")
            return carry
        jax.lax.fori_loop(0, cnt, body, 0)
        if n != n_next:
            waits_for(u_start + cnt * n, n_next, False, n_next > n)

    n_big = 2 * n_main
    assert n_big == half and u_big % nb == 0 and u_big - u_main >= n_big
    assert extra <= n_main and n_big < lead + extra < ring
    assert not half < (u_main & (nb - 1)) <= 3 * nb // 4 and u_big < n_pos - nb
    waits_for(u_main, n_main, False)
    steady(u_main, n_main, (u_big - u_main) // n_main, n_big, lead, extra, "main")
    steady(u_big, n_big, (n_pos - nb - u_big) // n_big, n_main, lead + extra, 0, "big")
    steady(n_pos - nb, n_main, nb // n_main - 1, n_main, lead + extra, 0, "last")
    block(n_pos - n_main, n_main, "end", None, emit_prev=True)
    pltpu.make_async_copy(ostage, out, o_sem.at[0]).wait()


def _build(A_x, A_k_cache, A_v_cache, A_wq, A_wo, B_x, B_k_cache, B_v_cache, B_wq, B_wo, *,
           n_main=4, u_duo=16, u_main=24, u_big=64, lead=6, extra=4, w1_at=7, ring=16,
           interpret=False):
    nb, sq, d = A_x.shape
    n_head, sk = A_k_cache.shape[1], A_k_cache.shape[2]
    n_pair = n_head // 2

    def tr(c):
        return jnp.swapaxes(c, 2, 3).reshape(nb, n_head * _DH, sk)

    aq, ao = _Alg(_ALG_Q, 4), _Alg(_ALG_O, 3)
    u32 = jnp.uint32
    n_xf = -(-len(aq.a_forms) // 4) * 4
    return pl.pallas_call(
        functools.partial(_kernel, aq=aq, ao=ao, n_main=n_main, u_duo=u_duo, u_main=u_main,
                          u_big=u_big, lead=lead, extra=extra, w1_at=w1_at),
        in_specs=[pl.BlockSpec(memory_space=pl.ANY)] * 10,
        out_specs=pl.BlockSpec(memory_space=pl.ANY),
        out_shape=jax.ShapeDtypeStruct((nb, sq, 2 * d), A_x.dtype),
        scratch_shapes=[
            pltpu.VMEM((2, nb, 192, d), _BF16),
            pltpu.VMEM((n_pair, 2, d, _PAIR), _BF16),
            pltpu.VMEM((n_pair, 2, _PAIR, d), _BF16),
            pltpu.VMEM((2, nb, sq, d), _F32),
            pltpu.VMEM((nb, sq, 2 * d), _BF16),
            pltpu.VMEM((ring, 4, _PAIR, sk), _BF16),
            pltpu.VMEM((10, sq // 2, 128), _F32),
            pltpu.VMEM((2, nb, n_xf, sq // 4, 128), u32),
            pltpu.VMEM((2, 2, len(aq.b_forms), 64, 128), u32),
            pltpu.VMEM((2, 2, len(ao.b_forms), 64, 128), u32),
            pltpu.VMEM((6, sq // 2, 128), _F32),
            pltpu.VMEM((2, nb, 96, 128), _F32),
            pltpu.SMEM((1,), jnp.int32),
            pltpu.SemaphoreType.DMA((ring + ring // n_main,)),
            pltpu.SemaphoreType.DMA((2,)),
            pltpu.SemaphoreType.DMA((1,)),
            pltpu.SemaphoreType.DMA((1,)),
        ],
        compiler_params=pltpu.CompilerParams(
            vmem_limit_bytes=122 * 1024 * 1024, disable_bounds_checks=True),
        interpret=interpret,
    )(A_x, tr(A_k_cache), tr(A_v_cache), A_wq, A_wo,
      B_x, tr(B_k_cache), tr(B_v_cache), B_wq, B_wo)


@jax.jit
def pallas_concat_heads__gqa_block_cached__mha_block_cached__near_ridge_kernel(
    A_x: jax.Array,
    A_k_cache: jax.Array,
    A_v_cache: jax.Array,
    A_wq: jax.Array,
    A_wo: jax.Array,
    B_x: jax.Array,
    B_k_cache: jax.Array,
    B_v_cache: jax.Array,
    B_wq: jax.Array,
    B_wo: jax.Array,
):
    return _build(A_x, A_k_cache, A_v_cache, A_wq, A_wo,
                  B_x, B_k_cache, B_v_cache, B_wq, B_wo)
```
